```python
import jax
import jax.numpy as jnp

def _softmax(x, axis=-1):
    return jax.nn.softmax(x, axis=axis)

def _gelu(x):
    return jax.nn.gelu(x, approximate=True)

def _silu(x):
    return jax.nn.silu(x)

def _sigmoid(x):
    return jax.nn.sigmoid(x)

def _layernorm(x, axis=-1, eps=1e-05):
    m = jnp.mean(x, axis=axis, keepdims=True)
    v = jnp.var(x, axis=axis, keepdims=True)
    return (x - m) / jnp.sqrt(v + eps)

def _scatter_add(tgt, idx, src, axis=0):
    return tgt.at[idx].add(src)

def _segment_sum(src, seg, n):
    return jax.ops.segment_sum(src, seg, n)

class _Rng:

    def __init__(self, key):
        self._k = key

    def _next(self):
        self._k, sub = jax.random.split(self._k)
        return sub

    def normal(self, shape):
        return jax.random.normal(self._next(), shape, dtype=jnp.bfloat16)

    def randint(self, lo, hi, shape):
        return jax.random.randint(self._next(), shape, lo, hi, dtype=jnp.int32)

    def uniform(self, shape, lo=0.0, hi=1.0):
        return jax.random.uniform(self._next(), shape, jnp.bfloat16, lo, hi)

    def permutation(self, n):
        return jax.random.permutation(self._next(), n)
kernel_name = 'concat_heads__ssm_conv_h3__memory_aug_recurrent_mem_tr__prompt'

def setup_inputs():
    _rng = _Rng(jax.random.key(int.from_bytes(__import__("os").urandom(4), "little")))
    _w = lambda a: (lambda t: t.astype(jnp.bfloat16) if jnp.issubdtype(t.dtype, jnp.floating) else t)(jnp.asarray(a))

    def _A_setup():
        B, S, D = (1, 2048, 1024)
        ks = 4
        return {'q': _w((lambda *s: _rng.normal(s) * 0.05)(B, S, D)), 'k': _w((lambda *s: _rng.normal(s) * 0.05)(B, S, D)), 'v': _w((lambda *s: _rng.normal(s) * 0.05)(B, S, D)), 'shift_k': _w((lambda *s: _rng.normal(s) * 0.05)(D, ks) * 0.5), 'ssm_k': _w((lambda *s: _rng.normal(s) * 0.05)(D, S) * (1.0 / S ** 0.5)), 'ssm_D': _w((lambda *s: _rng.normal(s) * 0.05)(D))}
    _A_in = _A_setup()

    def _B_setup():
        B, S, Dm = (1, 2048, 1024)
        H, Dh = (32, 128)
        M, seg = (8, 32)
        seg = min(seg, S)
        S = S // seg * seg
        return {'x': _w((lambda *s: _rng.normal(s) * 0.05)(B, S, Dm)), 'mem0': _w((lambda *s: _rng.normal(s) * 0.05)(B, M, Dm)), 'Wq': _w((lambda *s: _rng.normal(s) * 0.05)(Dm, H, Dh) * Dm ** (-0.5)), 'Wk': _w((lambda *s: _rng.normal(s) * 0.05)(Dm, H, Dh) * Dm ** (-0.5)), 'Wv': _w((lambda *s: _rng.normal(s) * 0.05)(Dm, H, Dh) * Dm ** (-0.5)), 'Wo': _w((lambda *s: _rng.normal(s) * 0.05)(H, Dh, Dm) * (H * Dh) ** (-0.5)), 'seg_len': seg}
    _B_in = _B_setup()
    return {'A_q': _A_in['q'], 'A_k': _A_in['k'], 'A_v': _A_in['v'], 'A_shift_k': _A_in['shift_k'], 'A_ssm_k': _A_in['ssm_k'], 'A_ssm_D': _A_in['ssm_D'], 'B_x': _B_in['x'], 'B_mem0': _B_in['mem0'], 'B_Wq': _B_in['Wq'], 'B_Wk': _B_in['Wk'], 'B_Wv': _B_in['Wv'], 'B_Wo': _B_in['Wo'], 'B_seg_len': _B_in['seg_len']}

def reference(A_q, A_k, A_v, A_shift_k, A_ssm_k, A_ssm_D, B_x, B_mem0, B_Wq, B_Wk, B_Wv, B_Wo, B_seg_len):

    def _A_ref(q, k, v, shift_k, ssm_k, ssm_D):
        B, S, D = q.shape
        ks = shift_k.shape[-1]
        k_pad = jnp.pad(k, ((0, 0), (ks - 1, 0), (0, 0)))
        k_shift = jnp.zeros_like(k)
        for t in range(ks):
            k_shift = k_shift + k_pad[:, t:t + S, :] * shift_k[:, ks - 1 - t][None, None, :]
        kv = k_shift * v
        L = 2 * S
        kv_pad = jnp.pad(kv, ((0, 0), (0, S), (0, 0)))
        kf_pad = jnp.pad(ssm_k, ((0, 0), (0, S)))
        kv_f = (lambda x, axes=(-2, -1): jnp.fft.rfft2(x.astype(jnp.float32), axes=axes))(kv_pad[:, None, :, :], axes=(1, 2))
        kf_f = (lambda x, axes=(-2, -1): jnp.fft.rfft2(x.astype(jnp.float32), axes=axes))(kf_pad[:, None, :], axes=(1, 2))
        kf_f = (lambda x, *d: x.transpose(*d))(kf_f, 1, 2, 0)
        y_f = kv_f * kf_f[None, :, :, :]
        y = (lambda x, s, axes=(-2, -1): jnp.fft.irfft2(x, s=s, axes=axes).astype(jnp.bfloat16))(y_f, (1, L), axes=(1, 2))[:, 0, :S, :]
        y = y + kv * ssm_D[None, None, :]
        return q * y

    def _B_ref(x, mem0, Wq, Wk, Wv, Wo, seg_len):
        B, S, Dm = x.shape
        H, Dh = (Wq.shape[1], Wq.shape[2])
        M = mem0.shape[1]
        scale = Dh ** (-0.5)
        n_seg = S // seg_len
        L = M + seg_len
        idx = jnp.arange(L)
        mask = (idx[:, None] < M) | (idx[:, None] >= idx[None, :])
        mem = mem0
        outs = []
        for s in range(n_seg):
            xs = x[:, s * seg_len:(s + 1) * seg_len, :].copy()
            h = jnp.concatenate([mem, xs], axis=1)
            q = jnp.einsum('btd,dhe->bhte', h, Wq)
            k = jnp.einsum('btd,dhe->bhte', h, Wk)
            v = jnp.einsum('btd,dhe->bhte', h, Wv)
            scores = jnp.einsum('bhqe,bhke->bhqk', q, k) * scale
            scores = jnp.where(mask[None, None], scores, -1000000000.0)
            p = _softmax(scores, axis=-1)
            o = jnp.einsum('bhqk,bhke->bhqe', p, v)
            o = jnp.einsum('bhte,hed->btd', o, Wo)
            mem = o[:, :M, :].copy()
            outs.append(o[:, M:, :])
        return jnp.concatenate(outs, axis=1)
    a = _A_ref(A_q, A_k, A_v, A_shift_k, A_ssm_k, A_ssm_D)
    b = _B_ref(B_x, B_mem0, B_Wq, B_Wk, B_Wv, B_Wo, B_seg_len)
    return jnp.concatenate([a, b], axis=-1)
```

```python
import functools
import math

import jax
import jax.numpy as jnp
from jax import lax
import jax.experimental.pallas as pl
import jax.experimental.pallas.tpu as pltpu

bf16, f32, u32, i32 = jnp.bfloat16, jnp.float32, jnp.uint32, jnp.int32

S = 2048
D = 1024
H, DH = 32, 128
M, SEG = 8, 32
NSEG = S // SEG
KS = 4

XR = 24
PRE = S - NSEG * XR
RING = 576
QOFF, OOFF = 64, 192
HS = 514
NPAIR = H // 2
L2 = 2 * (M + SEG)
LAGQK, LAGPV, K1 = 1, 3, 24

C = 128
NC = S // C
NB = D // 128
KPAD = 16


def _bf(x):
    return pltpu.bitcast(x, bf16)


def _kernel(q_hbm, k_hbm, v_hbm, skt_hbm, h_hbm, dd_hbm, x_hbm, mem0_hbm,
            wq_hbm, wk_hbm, wv_hbm, wo_hbm, out_hbm,
            st0, st1, wo_st, wo_p, x_buf, mem_ref, fill_ref, outb, oute,
            skt_buf, dd_buf, coef, k_buf, v_buf, q_buf, h_buf, kvo,
            u_buf, hs_buf, y_buf, kf, f_p, g_p,
            sem_w, sem_wo, sem_x, sem_small, sem_k, sem_v, sem_h, sem_q, sem_out,
            *bufs):
    wp = bufs[0:6]
    qkv = bufs[6:54]
    ob = bufs[54:70]
    om = bufs[70:86]
    stage = (st0, st1)
    w_hbm = (wq_hbm, wk_hbm, wv_hbm)
    scale = DH ** -0.5

    def w_copy(g, c):
        r0 = c * 256
        return pltpu.make_async_copy(
            w_hbm[g // 2].at[pl.ds(r0, 256), pl.ds(16 * (g % 2), 16), :],
            stage[g % 2].at[pl.ds(r0, 256)],
            sem_w.at[(g % 2) * 4 + c])

    def wo_copy(n):
        return pltpu.make_async_copy(
            wo_hbm.at[:, :, pl.ds(n * 128, 128)], wo_st.at[pl.ds(n * 256, 256)],
            sem_wo.at[n])

    def x_copy(part):
        r0, n = (0, PRE) if part == 0 else (PRE, S - PRE)
        return pltpu.make_async_copy(
            x_hbm.at[pl.ds(r0, n)], x_buf.at[pl.ds(r0, n)], sem_x.at[part])

    def small_copies():
        return [pltpu.make_async_copy(skt_hbm, skt_buf, sem_small.at[0]),
                pltpu.make_async_copy(dd_hbm, dd_buf, sem_small.at[1]),
                pltpu.make_async_copy(mem0_hbm, mem_ref, sem_small.at[2])]

    def col(b):
        return pl.ds(pl.multiple_of(b * 128, 128), 128)

    def kvh_copies(b):
        sl = b % 2
        return [pltpu.make_async_copy(k_hbm.at[:, col(b)],
                                      k_buf.at[sl, pl.ds(KPAD, S)], sem_k.at[sl]),
                pltpu.make_async_copy(v_hbm.at[:, col(b)], v_buf.at[sl], sem_v.at[sl]),
                pltpu.make_async_copy(h_hbm.at[col(b)], h_buf.at[sl], sem_h.at[sl])]

    def q_copy(b):
        sl = b % 2
        return pltpu.make_async_copy(q_hbm.at[:, col(b)], q_buf.at[sl], sem_q.at[sl])

    def outa_copy(b):
        return pltpu.make_async_copy(kvo.at[b], out_hbm.at[:, col(b)], sem_out.at[0])

    def outa_piece(b, j):
        rows = pl.ds(pl.multiple_of(j * 2 * C, 2 * C), 2 * C)
        return pltpu.make_async_copy(kvo.at[b, rows], out_hbm.at[rows, col(b)],
                                     sem_out.at[1])

    def outb_copy(cb):
        rows = pl.ds(pl.multiple_of(cb * 8 * XR, 8 * XR), 8 * XR)
        return pltpu.make_async_copy(outb.at[rows], out_hbm.at[rows, pl.ds(D, D)],
                                     sem_out.at[2])

    def oute_copy(n):
        return pltpu.make_async_copy(
            oute.at[n], out_hbm.at[pl.ds(S - PRE, PRE), col(NB + n)], sem_out.at[3])

    def relayout(g, c):
        src, dst = stage[g % 2], wp[g]
        d0 = c * 256
        for i in range(128):
            a = pltpu.bitcast(src[d0 + 2 * i], u32)
            b = pltpu.bitcast(src[d0 + 2 * i + 1], u32)
            lo = (a & jnp.uint32(0xFFFF)) | (b << 16)
            hi = (a >> 16) | (b & jnp.uint32(0xFFFF0000))
            row = c * 128 + i
            dst[pl.ds(row, 8, stride=2 * HS), :] = lo
            dst[pl.ds(row + HS, 8, stride=2 * HS), :] = hi

    def wo_pack(n):
        for r in range(0, 256, 8):
            blk = pltpu.bitcast(wo_st[pl.ds(n * 256 + r, 8)], u32)
            wo_p[n, r * 8:(r + 8) * 8, :] = blk.reshape(64, 128)

    def wqkv(m, h):
        g, hh = 2 * m + h // 16, h % 16
        return _bf(wp[g][hh * HS:hh * HS + D // 2, :])

    def s1_h(sl, j):
        fm = _bf(f_p[...])
        for t in range(2):
            a = 2 * j + t
            hh = h_buf[sl, :, pl.ds(pl.multiple_of(a * C, C), C)]
            hs_buf[sl, a] = lax.dot_general(fm, hh, (((1,), (1,)), ((), ())),
                                            preferred_element_type=f32)

    def s1_u(sl, b, slot, j):
        t0 = pl.multiple_of(j * 2 * C, 2 * C)
        kf[...] = k_buf[sl, pl.ds(t0, 2 * C + KPAD), :].astype(f32)
        acc = None
        for tap in range(KS):
            term = kf[KPAD - tap:KPAD - tap + 2 * C, :] * coef[b, tap:tap + 1, :]
            acc = term if acc is None else acc + term
        kv = (acc * v_buf[sl, pl.ds(t0, 2 * C), :].astype(f32)).astype(bf16)
        kvo[slot, pl.ds(t0, 2 * C), :] = kv
        fm = _bf(f_p[...])
        for t in range(2):
            u_buf[sl, 2 * j + t] = jnp.dot(fm, kv[t * C:(t + 1) * C],
                                           preferred_element_type=f32)

    def s2_parts(sl, j):
        re = pl.ds(pl.multiple_of(j * 16, 16), 16)
        im = pl.ds(pl.multiple_of(C + j * 16, 16), 16)
        yre = pl.ds(pl.multiple_of(j * 8, 8), 8)
        yim = pl.ds(pl.multiple_of(C // 2 + j * 8, 8), 8)
        sgn = (1 - 2 * (lax.broadcasted_iota(i32, (16, 128), 0) % 2)).astype(f32)
        prev = []

        def one(a):
            yr = yi = None
            for b in range(a + 1):
                ur, ui = u_buf[sl, b, re, :], u_buf[sl, b, im, :]
                hr, hi = hs_buf[sl, a - b, re, :], hs_buf[sl, a - b, im, :]
                pr, pi = ur * hr - ui * hi, ur * hi + ui * hr
                yr = pr if yr is None else yr + pr
                yi = pi if yi is None else yi + pi
            if prev:
                zr, zi = yr - prev[1], yi + prev[0]
            else:
                zr, zi = yr, yi
            prev[:] = [yr * sgn, yi * sgn]
            y_buf[sl, a, yre, :] = pltpu.bitcast(zr.astype(bf16), u32)
            y_buf[sl, a, yim, :] = pltpu.bitcast(zi.astype(bf16), u32)
        return one

    def s3(sl, b, slot, j):
        gm = _bf(g_p[...])
        for t in range(2):
            a = 2 * j + t
            rows = pl.ds(pl.multiple_of(a * C, C), C)
            y = jnp.dot(gm, _bf(y_buf[sl, a]), preferred_element_type=f32)
            y = y + kvo[slot, rows, :].astype(f32) * coef[b, KS:KS + 1, :]
            kvo[slot, rows, :] = (q_buf[sl, rows, :].astype(f32) * y).astype(bf16)

    x_copy(0).start()
    for c in range(4):
        w_copy(0, c).start()
    for cp in small_copies():
        cp.start()
    for c in range(4):
        w_copy(1, c).start()

    r = lax.broadcasted_iota(i32, (L2, L2), 0)
    c_ = lax.broadcasted_iota(i32, (L2, L2), 1)
    head = lambda i: jnp.where(i < 2 * M, i // M, (i - 2 * M) // SEG)
    ok = (r < 2 * M) | (c_ < 2 * M) | (c_ <= r)
    fill_ref[...] = jnp.where(head(r) == head(c_),
                              jnp.where(ok, 0.0, -1e9 / scale), -jnp.inf).astype(f32)

    def trig(kdim):
        kk = lax.broadcasted_iota(i32, (C, C), kdim)
        nn = lax.broadcasted_iota(i32, (C, C), 1 - kdim)
        ang = (((2 * kk + 1) * nn) % (4 * C)).astype(f32) * (math.pi / (2 * C))
        return jnp.cos(ang), -jnp.sin(ang)
    cs, sn = trig(0)
    f_p[...] = pltpu.bitcast(jnp.concatenate([cs, sn], axis=0).astype(bf16), u32)
    cs, sn = trig(1)
    g_p[...] = pltpu.bitcast(
        (jnp.concatenate([cs, sn], axis=1) * (1.0 / C)).astype(bf16), u32)
    for sl in range(2):
        k_buf[sl, 0:KPAD, :] = jnp.zeros((KPAD, 128), bf16)

    for cp in small_copies():
        cp.wait()
    skt = skt_buf[...].astype(f32)
    ddv = dd_buf[...].astype(f32)
    for b in range(NB):
        coef[b, 0:KS, :] = skt[:, b * 128:(b + 1) * 128]
        coef[b, KS:KS + 1, :] = ddv[b:b + 1, :]

    def first(c, carry):
        w_copy(0, c).wait()
        relayout(0, c)
        return carry
    lax.fori_loop(0, 4, first, 0)
    x_copy(0).wait()

    for g in range(6):
        if g + 2 < 6:
            for c in range(4):
                w_copy(g + 2, c).start()
        if g in (1, 2):
            for n in range(4 * (g - 1), 4 * g):
                wo_copy(n).start()
        if g == 3:
            for cp in kvh_copies(0):
                cp.start()
            x_copy(1).start()
        if g == 4:
            for cp in kvh_copies(0):
                cp.wait()
            for cp in kvh_copies(1):
                cp.start()
            for n in range(8):
                wo_copy(n).wait()

        def pro(i, carry, g=g):
            if g + 1 < 6:
                w_copy(g + 1, i).wait()
            r0 = pl.multiple_of(i * 128, 128)
            x = x_buf[pl.ds(r0, 128), :]
            for p in range(8):
                ys = [jnp.dot(x, wqkv(g // 2, 16 * (g % 2) + 2 * p + t),
                              preferred_element_type=f32) for t in range(2)]
                qkv[8 * g + p][pl.ds(pl.multiple_of(QOFF + r0, 64), 128), :] = (
                    jnp.concatenate(ys, axis=1).astype(bf16))
                if g >= 4 and p == 0:
                    s1_h(0, 4 * (g - 4) + i)
                if g >= 4 and p == 2:
                    s1_u(0, 0, 0, 4 * (g - 4) + i)
            if g + 1 < 6:
                relayout(g + 1, i)
            if g >= 4:
                wo_pack(4 * (g - 4) + i)
            return carry
        lax.fori_loop(0, 4, pro, 0)
    x_copy(1).wait()

    def step(cb, j):
        s = cb * 8 + j
        x0 = pl.multiple_of(PRE + XR * s, 8)
        wpos = pl.multiple_of((XR * s) % RING, 8)
        rpos = pl.multiple_of((SEG * s + QOFF) % RING, 32)
        owpos = pl.multiple_of((SEG * s + OOFF) % RING, 32)
        orpos = pl.multiple_of((XR * s + OOFF) % RING, 8)
        lhs = jnp.concatenate([mem_ref[...], x_buf[pl.ds(x0, XR), :]], axis=0)

        def proj(p):
            res = []
            for m in range(3):
                ys = [jnp.dot(lhs, wqkv(m, 2 * p + t), preferred_element_type=f32)
                      for t in range(2)]
                qkv[m * NPAIR + p][pl.ds(wpos, XR), :] = jnp.concatenate(
                    [y[M:] for y in ys], axis=1).astype(bf16)
                res.append(jnp.concatenate([y[:M] for y in ys], axis=0).astype(bf16))
            return res

        def gather(m, p, mm):
            xx = qkv[m * NPAIR + p][pl.ds(rpos, SEG), :]
            return jnp.concatenate([mm, xx[:, :DH], xx[:, DH:]], axis=0)

        def qk(p, mems):
            q2, k2 = gather(0, p, mems[0]), gather(1, p, mems[1])
            sc = lax.dot_general(q2, k2, (((1,), (1,)), ((), ())),
                                 preferred_element_type=f32)
            fill = fill_ref[...]
            sc = jnp.where(fill == 0.0, sc, fill)
            mx = jnp.max(sc, axis=1, keepdims=True)
            e = jnp.exp((sc - mx) * scale)
            l = jnp.sum(e, axis=1, keepdims=True)
            rc = pl.reciprocal(l, approx=True)
            rc = rc * (2.0 - l * rc)
            return (e * rc).astype(bf16)

        def pv(p, pr, mems):
            o = jnp.dot(pr, gather(2, p, mems[2]), preferred_element_type=f32)
            om[p][...] = jnp.concatenate([o[0:M], o[M:2 * M]], axis=1).astype(bf16)
            ob[p][pl.ds(owpos, SEG), :] = jnp.concatenate(
                [o[2 * M:2 * M + SEG], o[2 * M + SEG:]], axis=1).astype(bf16)

        def oproj(k0, k1, ns):
            l = jnp.concatenate(
                [jnp.concatenate([om[p][...], ob[p][pl.ds(orpos, XR), :]], axis=0)
                 for p in range(k0 // 2, k1 // 2)], axis=1)
            return [jnp.dot(l, _bf(wo_p[n, k0 * 64:k1 * 64, :]),
                            preferred_element_type=f32) for n in ns]

        sl1 = (cb + 1) % 2
        b1 = jnp.minimum(cb + 1, NB - 1)
        slot1 = cb + 1
        b3 = jnp.maximum(cb - 1, 0)
        slot3 = jnp.where(cb == 0, NB, cb - 1)
        s2 = s2_parts(cb % 2, j)

        mems, prs, parts = {}, {}, []
        for t in range(NPAIR + LAGPV):
            if t < NPAIR:
                mems[t] = proj(t)
            else:
                parts += oproj(0, K1, range(len(parts), len(parts) + 2))
            if t == 0:
                s1_h(sl1, j)
                s3(sl1, b3, slot3, j)
            if t == 1:
                s1_u(sl1, b1, slot1, j)
            p = t - LAGPV
            if 0 <= p < NPAIR:
                pv(p, prs.pop(p), mems.pop(p))
            p = t - LAGQK
            if 0 <= p < NPAIR:
                prs[p] = qk(p, mems[p])
            if 2 <= t < 2 + NC:
                s2(t - 2)
        parts += oproj(0, K1, range(len(parts), 8))
        rest = oproj(K1, H, range(8))
        out = jnp.concatenate([b + a for a, b in zip(parts, rest)], axis=1).astype(bf16)
        mem_ref[...] = out[:M]
        outb[pl.ds(pl.multiple_of(XR * s, 8), XR), :] = out[M:]

    def outer(cb, carry):
        @pl.when(cb + 1 < NB)
        def _():
            for cp in kvh_copies(cb + 1):
                cp.wait()

        @pl.when(cb + 2 < NB)
        def _():
            for cp in kvh_copies(cb + 2):
                cp.start()

        @pl.when(cb >= 1)
        def _():
            q_copy(cb - 1).wait()
            outb_copy(cb - 1).start()

        q_copy(cb).start()

        @pl.when(cb >= 2)
        def _():
            outa_copy(cb - 2).start()

        def inner(j, c2):
            step(cb, j)
            return c2
        lax.fori_loop(0, 8, inner, 0)
        return carry
    lax.fori_loop(0, NB, outer, 0)

    q_copy(NB - 1).wait()
    outb_copy(NB - 1).start()
    outa_copy(NB - 2).start()

    def epi(n, carry):
        s3((NB - 1) % 2, NB - 1, NB - 1, n)
        l = jnp.concatenate([ob[p][0:PRE, :] for p in range(NPAIR)], axis=1)
        y = jnp.dot(l, _bf(wo_p[n]), preferred_element_type=f32)
        oute[n] = y.astype(bf16)
        outa_piece(NB - 1, n).start()
        oute_copy(n).start()
        return carry
    lax.fori_loop(0, 8, epi, 0)

    for b in range(NB - 1):
        outa_copy(b).wait()
    for n in range(8):
        outb_copy(n).wait()
        outa_piece(NB - 1, n).wait()
        oute_copy(n).wait()


@functools.partial(jax.jit, static_argnames=("B_seg_len",))
def pallas_concat_heads__ssm_conv_h3__memory_aug_recurrent_mem_tr__prompt_kernel(
    A_q, A_k, A_v, A_shift_k, A_ssm_k, A_ssm_D, B_x, B_mem0, B_Wq, B_Wk, B_Wv, B_Wo,
    B_seg_len=SEG,
):
    assert B_seg_len == SEG
    assert A_q.shape == (1, S, D) and B_x.shape == (1, S, D)
    assert B_Wq.shape == (D, H, DH) and B_mem0.shape == (1, M, D)
    vm = pltpu.VMEM
    dma = pltpu.SemaphoreType.DMA
    scratch = [
        vm((D, 16, DH), bf16), vm((D, 16, DH), bf16),
        vm((2048, 16, 128), bf16),
        vm((8, H * DH // 2, 128), u32),
        vm((S, D), bf16),
        vm((M, D), bf16),
        vm((L2, L2), f32),
        vm((NSEG * XR, D), bf16),
        vm((8, PRE, 128), bf16),
        vm((KS, D), bf16), vm((NB, 128), bf16),
        vm((NB, 8, 128), f32),
        vm((2, S + KPAD, 128), bf16),
        vm((2, S, 128), bf16), vm((2, S, 128), bf16),
        vm((2, 128, S), bf16),
        vm((NB + 1, S, 128), bf16),
        vm((2, NC, 2 * C, 128), f32), vm((2, NC, 2 * C, 128), f32),
        vm((2, NC, C, 128), u32),
        vm((2 * C + KPAD, 128), f32),
        vm((C, C), u32), vm((C // 2, 2 * C), u32),
        dma((8,)), dma((8,)), dma((2,)), dma((3,)),
        dma((2,)), dma((2,)), dma((2,)), dma((2,)), dma((4,)),
    ]
    scratch += [vm((16 * HS, 128), u32)] * 6
    scratch += [vm((RING, 2 * DH), bf16)] * (3 * NPAIR)
    scratch += [vm((RING, 2 * DH), bf16)] * NPAIR
    scratch += [vm((M, 2 * DH), bf16)] * NPAIR

    out = pl.pallas_call(
        _kernel,
        out_shape=jax.ShapeDtypeStruct((S, 2 * D), bf16),
        in_specs=[pl.BlockSpec(memory_space=pl.ANY)] * 12,
        out_specs=pl.BlockSpec(memory_space=pl.ANY),
        scratch_shapes=scratch,
        compiler_params=pltpu.CompilerParams(vmem_limit_bytes=120 * 1024 * 1024),
        name="ssm_memtr",
    )(A_q.reshape(S, D), A_k.reshape(S, D), A_v.reshape(S, D), A_shift_k.T, A_ssm_k,
      A_ssm_D.reshape(NB, 128), B_x.reshape(S, D), B_mem0.reshape(M, D),
      B_Wq, B_Wk, B_Wv, B_Wo.reshape(H * DH // 16, 16, D))
    return out.reshape(1, S, 2 * D)
```

```python
import functools
import math

import jax
import jax.numpy as jnp
from jax import lax
import jax.experimental.pallas as pl
import jax.experimental.pallas.tpu as pltpu

bf16, f32, u32, i32 = jnp.bfloat16, jnp.float32, jnp.uint32, jnp.int32

S = 2048
D = 1024
H, DH = 32, 128
M, SEG = 8, 32
NSEG = S // SEG
KS = 4

XR = 24
PRE = S - NSEG * XR
RING = 576
QOFF, OOFF = 64, 192
HS = 514
NPAIR = H // 2
L2 = 2 * (M + SEG)
LAGQK, LAGPV, K1 = 1, 3, 24

C = 128
NC = S // C
NB = D // 128
KPAD = 16
S2_AT = list(range(14, 46))


def _bf(x):
    return pltpu.bitcast(x, bf16)


def _kernel(q_hbm, k_hbm, v_hbm, skt_hbm, h_hbm, dd_hbm, x_hbm, mem0_hbm,
            wq_hbm, wk_hbm, wv_hbm, wo_hbm, out_hbm,
            st0, st1, wo_st, wo_p, x_buf, mem_ref, outb, oute,
            coef, k_buf, v_buf, q_buf, h_buf, kvo,
            uh, y_buf, kf, f_p, g_p,
            sem_w, sem_wo, sem_x, sem_small, sem_k, sem_v, sem_h, sem_q, sem_out,
            *bufs):
    wp = bufs[0:6]
    ring = bufs[6:22]
    om = bufs[22:38]
    fill_ref, skt_buf, dd_buf = bufs[38:41]
    stage = (st0, st1)
    w_hbm = (wq_hbm, wk_hbm, wv_hbm)
    scale = DH ** -0.5

    def w_copy(g, c):
        r0 = c * 256
        return pltpu.make_async_copy(
            w_hbm[g // 2].at[pl.ds(r0, 256), pl.ds(16 * (g % 2), 16), :],
            stage[g % 2].at[pl.ds(r0, 256)],
            sem_w.at[(g % 2) * 4 + c])

    def wo_copy(n):
        return pltpu.make_async_copy(
            wo_hbm.at[:, :, pl.ds(n * 128, 128)], wo_st.at[pl.ds(n * 256, 256)],
            sem_wo.at[n])

    def x_copy(part):
        r0, n = (0, PRE) if part == 0 else (PRE, S - PRE)
        return pltpu.make_async_copy(
            x_hbm.at[pl.ds(r0, n)], x_buf.at[pl.ds(r0, n)], sem_x.at[part])

    def small_copies():
        return [pltpu.make_async_copy(skt_hbm, skt_buf, sem_small.at[0]),
                pltpu.make_async_copy(dd_hbm, dd_buf, sem_small.at[1]),
                pltpu.make_async_copy(mem0_hbm, mem_ref, sem_small.at[2])]

    def col(b):
        return pl.ds(pl.multiple_of(b * 128, 128), 128)

    def kvh_copies(b):
        sl = b % 2
        return [pltpu.make_async_copy(k_hbm.at[:, col(b)],
                                      k_buf.at[sl, pl.ds(KPAD, S)], sem_k.at[sl]),
                pltpu.make_async_copy(v_hbm.at[:, col(b)], v_buf.at[sl], sem_v.at[sl]),
                pltpu.make_async_copy(h_hbm.at[col(b)], h_buf.at[sl], sem_h.at[sl])]

    def q_copy(b):
        sl = b % 2
        return pltpu.make_async_copy(q_hbm.at[:, col(b)], q_buf.at[sl], sem_q.at[sl])

    def outa_copy(b):
        return pltpu.make_async_copy(kvo.at[b], out_hbm.at[:, col(b)], sem_out.at[0])

    def outa_piece(b, j):
        rows = pl.ds(pl.multiple_of(j * 2 * C, 2 * C), 2 * C)
        return pltpu.make_async_copy(kvo.at[b, rows], out_hbm.at[rows, col(b)],
                                     sem_out.at[1])

    def outb_copy(cb):
        rows = pl.ds(pl.multiple_of(cb * 8 * XR, 8 * XR), 8 * XR)
        return pltpu.make_async_copy(outb.at[rows], out_hbm.at[rows, pl.ds(D, D)],
                                     sem_out.at[2])

    def oute_copy(n):
        return pltpu.make_async_copy(
            oute.at[n], out_hbm.at[pl.ds(S - PRE, PRE), col(NB + n)], sem_out.at[3])

    def relayout(g, c, lo_i=0, hi_i=128):
        src, dst = stage[g % 2], wp[g]
        d0 = c * 256
        for i in range(lo_i, hi_i):
            a = pltpu.bitcast(src[d0 + 2 * i], u32)
            b = pltpu.bitcast(src[d0 + 2 * i + 1], u32)
            lo = (a & jnp.uint32(0xFFFF)) | (b << 16)
            hi = (a >> 16) | (b & jnp.uint32(0xFFFF0000))
            row = c * 128 + i
            dst[pl.ds(row, 8, stride=2 * HS), :] = lo
            dst[pl.ds(row + HS, 8, stride=2 * HS), :] = hi

    def wo_pack(n, r0, r1):
        for r in range(r0, r1, 8):
            blk = pltpu.bitcast(wo_st[pl.ds(n * 256 + r, 8)], u32)
            wo_p[n, r * 8:(r + 8) * 8, :] = blk.reshape(64, 128)

    def wqkv(m, h):
        g, hh = 2 * m + h // 16, h % 16
        return _bf(wp[g][hh * HS:hh * HS + D // 2, :])

    def s1_h(sl, j):
        for t in range(2):
            a = 2 * j + t
            hh = h_buf[sl, :, pl.ds(pl.multiple_of(a * C, C), C)]
            for half in range(2):
                fm = _bf(f_p[half * 64:(half + 1) * 64, :])
                uh[sl * 2 * NC + NC + a, half * C:(half + 1) * C, :] = lax.dot_general(
                    fm, hh, (((1,), (1,)), ((), ())), preferred_element_type=f32)

    def s0_kv(sl, b, slot, j, i):
        t0 = pl.multiple_of(j * 2 * C, 2 * C)
        kw = k_buf.at[sl, pl.ds(t0, 2 * C + KPAD)]
        vw = v_buf.at[sl, pl.ds(t0, 2 * C)]
        ow = kvo.at[slot, pl.ds(t0, 2 * C)]
        kf[i] = kw[32 * i:32 * i + 32 + KPAD, :].astype(f32)
        acc = None
        for tap in range(KS):
            term = kf[i, KPAD - tap:KPAD - tap + 32, :] * coef[b, tap:tap + 1, :]
            acc = term if acc is None else acc + term
        ow[32 * i:32 * i + 32, :] = (acc * vw[32 * i:32 * i + 32, :].astype(f32)).astype(bf16)

    def s1_u(sl, slot, j):
        for t in range(2):
            a = 2 * j + t
            kv = kvo[slot, pl.ds(pl.multiple_of(a * C, C), C), :]
            for half in range(2):
                fm = _bf(f_p[half * 64:(half + 1) * 64, :])
                uh[sl * 2 * NC + a, half * C:(half + 1) * C, :] = jnp.dot(
                    fm, kv, preferred_element_type=f32)

    def s2_parts(sl, j):
        sgn = (1 - 2 * (lax.broadcasted_iota(i32, (8, 128), 0) % 2)).astype(f32)
        u0 = sl * 2 * NC
        h0 = u0 + NC
        r0 = pl.multiple_of(j * 32, 32)
        prev = []

        def one(idx, pace):
            grp, a = divmod(idx, NC)
            re, im = pl.ds(r0 + 16 * grp, 8), pl.ds(r0 + 16 * grp + 8, 8)
            yr = yi = None
            for b in range(a + 1):
                if b == a:
                    uh[4 * NC, 0:8, :] = pace
                ur, ui = uh[u0 + b, re, :], uh[u0 + b, im, :]
                hr, hi = uh[h0 + a - b, re, :], uh[h0 + a - b, im, :]
                yr = ur * hr if yr is None else yr + ur * hr
                yi = ur * hi if yi is None else yi + ur * hi
                yr = yr - ui * hi
                yi = yi + ui * hr
            if a > 0:
                zr, zi = yr - prev[1], yi + prev[0]
            else:
                zr, zi = yr, yi
            prev[:] = [yr * sgn, yi * sgn]
            z = jnp.concatenate([zr, zi], axis=0).astype(bf16)
            r = (a % 2) * 16 + 8 * grp
            y_buf[sl, j, a // 2, r:r + 8, :] = pltpu.bitcast(z, u32)
        return one

    def s3(sl, b, slot, j):
        gm = _bf(g_p[...])
        for t in range(2):
            a = 2 * j + t
            rows = pl.ds(pl.multiple_of(a * C, C), C)
            yp = y_buf[sl, :, j, 16 * t:16 * t + 16, :].reshape(C, 128)
            y = jnp.dot(gm, _bf(yp), preferred_element_type=f32)
            y = y + kvo[slot, rows, :].astype(f32) * coef[b, KS:KS + 1, :]
            kvo[slot, rows, :] = (q_buf[sl, rows, :].astype(f32) * y).astype(bf16)

    x_copy(0).start()
    for c in range(4):
        w_copy(0, c).start()
    for cp in small_copies():
        cp.start()
    for c in range(4):
        w_copy(1, c).start()

    r = lax.broadcasted_iota(i32, (L2, L2), 0)
    c_ = lax.broadcasted_iota(i32, (L2, L2), 1)
    head = lambda i: jnp.where(i < 2 * M, i // M, (i - 2 * M) // SEG)
    ok = (r < 2 * M) | (c_ < 2 * M) | (c_ <= r)
    fill_ref[...] = jnp.where(head(r) == head(c_),
                              jnp.where(ok, 0.0, -1e9 / scale), -jnp.inf).astype(f32)

    def dft(shape, kdim):
        rr = lax.broadcasted_iota(i32, shape, kdim)
        nn = lax.broadcasted_iota(i32, shape, 1 - kdim)
        kk = 8 * (rr // 16) + rr % 8
        m = ((2 * kk + 1) * nn + C * ((rr // 8) % 2)) % (4 * C)
        return jnp.cos(m.astype(f32) * (math.pi / (2 * C)))
    f_p[...] = pltpu.bitcast(dft((2 * C, C), 0).astype(bf16), u32)
    g_p[...] = pltpu.bitcast((dft((C, 2 * C), 1) * (1.0 / C)).astype(bf16), u32)
    for sl in range(2):
        k_buf[sl, 0:KPAD, :] = jnp.zeros((KPAD, 128), bf16)

    for cp in small_copies():
        cp.wait()
    skt = skt_buf[...].astype(f32)
    ddv = dd_buf[...].astype(f32)
    for b in range(NB):
        coef[b, 0:KS, :] = skt[:, b * 128:(b + 1) * 128]
        coef[b, KS:KS + 1, :] = ddv[b:b + 1, :]

    def first(c, carry):
        w_copy(0, c).wait()
        relayout(0, c)
        return carry
    with jax.named_scope('first'):
        lax.fori_loop(0, 4, first, 0)
    x_copy(0).wait()

    for g in range(6):
        if g + 2 < 6:
            for c in range(4):
                w_copy(g + 2, c).start()
        if g in (1, 2):
            for n in range(4 * (g - 1), 4 * g):
                wo_copy(n).start()
        if g == 3:
            for cp in kvh_copies(0):
                cp.start()
            x_copy(1).start()
        if g == 4:
            for cp in kvh_copies(0):
                cp.wait()
            for cp in kvh_copies(1):
                cp.start()
            for n in range(8):
                wo_copy(n).wait()

        def pro(i, carry, g=g):
            if g + 1 < 6:
                w_copy(g + 1, i).wait()
            r0 = pl.multiple_of(i * 128, 128)
            x = x_buf[pl.ds(r0, 128), :]
            jj = 4 * (g - 4) + i
            for p in range(8):
                ys = []
                for t in range(2):
                    y = jnp.dot(x, wqkv(g // 2, 16 * (g % 2) + 2 * p + t),
                                preferred_element_type=f32)
                    ys.append(y)
                    u = 2 * p + t
                    if u < 15:
                        pace = y[0:16].astype(bf16)
                        if g + 1 < 6:
                            stage[(g + 1) % 2][D] = pace
                            relayout(g + 1, i, (128 * u) // 15, (128 * (u + 1)) // 15)
                        if g >= 4 and u >= 7:
                            wo_st[2048] = pace
                            wo_pack(jj, 32 * (u - 7), 32 * (u - 6))
                    if g >= 4 and u < 8:
                        coef[NB, 0:8, :] = y[0:8]
                        s0_kv(0, 0, 0, jj, u)
                ring[8 * (g % 2) + p][pl.ds(pl.multiple_of(QOFF + r0, 64), 128),
                                      (g // 2) * 256:(g // 2 + 1) * 256] = (
                    jnp.concatenate(ys, axis=1).astype(bf16))
                if g >= 4 and p == 0:
                    s1_h(0, jj)
                if g >= 4 and p == 5:
                    s1_u(0, 0, jj)
            return carry
        with jax.named_scope('pro%d' % g):
            lax.fori_loop(0, 4, pro, 0)
    x_copy(1).wait()

    def step(cb, j):
        s = cb * 8 + j
        x0 = pl.multiple_of(PRE + XR * s, 8)
        wpos = pl.multiple_of(lax.rem(s, RING // XR) * XR, 8)
        rpos = pl.multiple_of(lax.rem(s + QOFF // SEG, RING // SEG) * SEG, 32)
        owpos = pl.multiple_of(lax.rem(s + OOFF // SEG, RING // SEG) * SEG, 32)
        orpos = pl.multiple_of(lax.rem(s + OOFF // XR, RING // XR) * XR, 8)
        lhs = jnp.concatenate([mem_ref[...], x_buf[pl.ds(x0, XR), :]], axis=0)

        def proj(p, bg):
            res = []
            for m in range(3):
                ys = [jnp.dot(lhs, wqkv(m, 2 * p + t), preferred_element_type=f32)
                      for t in range(2)]
                ring[p][pl.ds(wpos, XR), m * 256:(m + 1) * 256] = jnp.concatenate(
                    [y[M:] for y in ys], axis=1).astype(bf16)
                res.append(jnp.concatenate([y[:M] for y in ys], axis=0).astype(bf16))
                bg(3 * p + m, ys[0][:M])
            return res

        def gather(m, p, mm):
            xx = ring[p][pl.ds(rpos, SEG), m * 256:(m + 1) * 256]
            return jnp.concatenate([mm, xx[:, :DH], xx[:, DH:]], axis=0)

        def qk(p, mems):
            q2, k2 = gather(0, p, mems[0]), gather(1, p, mems[1])
            sc = lax.dot_general(q2, k2, (((1,), (1,)), ((), ())),
                                 preferred_element_type=f32)
            fill = fill_ref[...]
            sc = jnp.where(fill == 0.0, sc, fill)
            mx = jnp.max(sc, axis=1, keepdims=True)
            e = jnp.exp((sc - mx) * scale)
            l = jnp.sum(e, axis=1, keepdims=True)
            rc = pl.reciprocal(l, approx=True)
            rc = rc * (2.0 - l * rc)
            return (e * rc).astype(bf16)

        def pv(p, pr, mems):
            o = jnp.dot(pr, gather(2, p, mems[2]), preferred_element_type=f32)
            om[p][...] = jnp.concatenate([o[0:M], o[M:2 * M]], axis=1).astype(bf16)
            ring[p][pl.ds(owpos, SEG), 768:1024] = jnp.concatenate(
                [o[2 * M:2 * M + SEG], o[2 * M + SEG:]], axis=1).astype(bf16)

        def oproj(k0, k1, ns):
            l = jnp.concatenate(
                [jnp.concatenate([om[p][...], ring[p][pl.ds(orpos, XR), 768:1024]], axis=0)
                 for p in range(k0 // 2, k1 // 2)], axis=1)
            return [jnp.dot(l, _bf(wo_p[n, k0 * 64:k1 * 64, :]),
                            preferred_element_type=f32) for n in ns]

        sl1 = (cb + 1) % 2
        b1 = jnp.minimum(cb + 1, NB - 1)
        slot1 = cb + 1
        b3 = jnp.maximum(cb - 1, 0)
        slot3 = jnp.where(cb == 0, NB, cb - 1)
        s2 = s2_parts(cb % 2, j)

        def bg(u, pace):
            if 2 <= u < 10:
                coef[NB, 0:8, :] = pace
                s0_kv(sl1, b1, slot1, j, u - 2)
            if u in S2_AT:
                s2(S2_AT.index(u), pace)

        mems, prs, parts = {}, {}, []
        for t in range(NPAIR + LAGPV):
            if t < NPAIR:
                mems[t] = proj(t, bg)
            else:
                parts += oproj(0, K1, range(len(parts), len(parts) + 2))
                bg(48 + t - NPAIR, parts[-1][:M])
            if t == 0:
                s3(sl1, b3, slot3, j)
            if t == 1:
                s1_h(sl1, j)
            if t == 3:
                s1_u(sl1, slot1, j)
            p = t - LAGPV
            if 0 <= p < NPAIR:
                pv(p, prs.pop(p), mems.pop(p))
            p = t - LAGQK
            if 0 <= p < NPAIR:
                prs[p] = qk(p, mems[p])
        parts += oproj(0, K1, range(len(parts), 8))
        rest = oproj(K1, H, range(8))
        out = jnp.concatenate([b + a for a, b in zip(parts, rest)], axis=1).astype(bf16)
        mem_ref[...] = out[:M]
        outb[pl.ds(pl.multiple_of(XR * s, 8), XR), :] = out[M:]

    def outer(cb, carry):
        @pl.when(cb + 1 < NB)
        def _():
            for cp in kvh_copies(cb + 1):
                cp.wait()

        @pl.when(cb + 2 < NB)
        def _():
            for cp in kvh_copies(cb + 2):
                cp.start()

        @pl.when(cb >= 1)
        def _():
            q_copy(cb - 1).wait()
            outb_copy(cb - 1).start()

        q_copy(cb).start()

        @pl.when(cb >= 2)
        def _():
            outa_copy(cb - 2).start()

        def inner(j, c2):
            step(cb, j)
            return c2
        with jax.named_scope('inner'):
            lax.fori_loop(0, 8, inner, 0)
        return carry
    with jax.named_scope('main'):
        lax.fori_loop(0, NB, outer, 0)

    q_copy(NB - 1).wait()
    outb_copy(NB - 1).start()
    outa_copy(NB - 2).start()

    def epi(n, carry):
        s3((NB - 1) % 2, NB - 1, NB - 1, n)
        l = jnp.concatenate([ring[p][0:PRE, 768:1024] for p in range(NPAIR)], axis=1)
        y = jnp.dot(l, _bf(wo_p[n]), preferred_element_type=f32)
        oute[n] = y.astype(bf16)
        outa_piece(NB - 1, n).start()
        oute_copy(n).start()
        return carry
    with jax.named_scope('epi'):
        lax.fori_loop(0, 8, epi, 0)

    for b in range(NB - 1):
        outa_copy(b).wait()
    for n in range(8):
        outb_copy(n).wait()
        outa_piece(NB - 1, n).wait()
        oute_copy(n).wait()


@functools.partial(jax.jit, static_argnames=("B_seg_len",))
def pallas_concat_heads__ssm_conv_h3__memory_aug_recurrent_mem_tr__prompt_kernel(
    A_q, A_k, A_v, A_shift_k, A_ssm_k, A_ssm_D, B_x, B_mem0, B_Wq, B_Wk, B_Wv, B_Wo,
    B_seg_len=SEG,
):
    assert B_seg_len == SEG
    assert A_q.shape == (1, S, D) and B_x.shape == (1, S, D)
    assert B_Wq.shape == (D, H, DH) and B_mem0.shape == (1, M, D)
    vm = pltpu.VMEM
    dma = pltpu.SemaphoreType.DMA
    scratch = [
        vm((D + 4, 16, DH), bf16), vm((D + 4, 16, DH), bf16),
        vm((2048 + 4, 16, 128), bf16),
        vm((8, H * DH // 2, 128), u32),
        vm((S, D), bf16),
        vm((M, D), bf16),
        vm((NSEG * XR, D), bf16),
        vm((8, PRE, 128), bf16),
        vm((NB + 1, 32, 128), f32),
        vm((2, S + 64, 128), bf16),
        vm((2, S, 128), bf16), vm((2, S, 128), bf16),
        vm((2, 128, S), bf16),
        vm((NB + 1, S, 128), bf16),
        vm((4 * NC + 1, 2 * C, 128), f32),
        vm((2, 8, 8, 32, 128), u32),
        vm((8, 32 + KPAD, 128), f32),
        vm((C, C), u32), vm((C // 2, 2 * C), u32),
        dma((8,)), dma((8,)), dma((2,)), dma((3,)),
        dma((2,)), dma((2,)), dma((2,)), dma((2,)), dma((4,)),
    ]
    scratch += [vm((16 * HS, 128), u32)] * 6
    scratch += [vm((RING, 8 * DH), bf16)] * NPAIR
    scratch += [vm((M, 2 * DH), bf16)] * NPAIR
    scratch += [vm((L2, L2), f32), vm((KS, D), bf16), vm((NB, 128), bf16)]

    out = pl.pallas_call(
        _kernel,
        out_shape=jax.ShapeDtypeStruct((S, 2 * D), bf16),
        in_specs=[pl.BlockSpec(memory_space=pl.ANY)] * 12,
        out_specs=pl.BlockSpec(memory_space=pl.ANY),
        scratch_shapes=scratch,
        compiler_params=pltpu.CompilerParams(vmem_limit_bytes=120 * 1024 * 1024),
        name="ssm_memtr",
    )(A_q.reshape(S, D), A_k.reshape(S, D), A_v.reshape(S, D), A_shift_k.T, A_ssm_k,
      A_ssm_D.reshape(NB, 128), B_x.reshape(S, D), B_mem0.reshape(M, D),
      B_Wq, B_Wk, B_Wv, B_Wo.reshape(H * DH // 16, 16, D))
    return out.reshape(1, S, 2 * D)
```

```python
import functools
import math

import jax
import jax.numpy as jnp
from jax import lax
import jax.experimental.pallas as pl
import jax.experimental.pallas.tpu as pltpu

bf16, f32, u32, i32 = jnp.bfloat16, jnp.float32, jnp.uint32, jnp.int32

S = 2048
D = 1024
H, DH = 32, 128
M, SEG = 8, 32
NSEG = S // SEG
KS = 4

XR = 24
PRE = S - NSEG * XR
RING = 576
QOFF = 64
HS = 514
NPAIR = H // 2
L2 = 2 * (M + SEG)

C = 128
NC = S // C
NB = D // 128
KPAD = 16

CFG = dict(
    lagqk=1, lagpv=3, k1=24, och=8, op_per=2,
    s2_at=[list(range(0, 32)), list(range(62, 94))],
    s0_at=[list(range(0, 4)) + list(range(16, 20)), list(range(62, 66)) + list(range(78, 82))],
    nopro=False,
)


def _bf(x):
    return pltpu.bitcast(x, bf16)


def _kernel(q_hbm, k_hbm, v_hbm, skt_hbm, h_hbm, dd_hbm, x_hbm, mem0_hbm,
            wq_hbm, wk_hbm, wv_hbm, wo_hbm, out_hbm,
            st0, st1, st2, wo_st, wo_p, x_buf, mem_ref, outb,
            coef, k_buf, v_buf, q_buf, h_buf, kvo,
            uh, y_buf, kf, f_p, g_p, xp, sems,
            *bufs):
    wp = bufs[0:6]
    ring = bufs[6:14]
    o_sc = bufs[14:30]
    q_sc = bufs[30:46]
    fill_ref, skt_buf, dd_buf = bufs[46:49]
    stage = (st0, st1, st2)
    w_hbm = (wk_hbm, wv_hbm, wq_hbm)
    scale = DH ** -0.5
    cfg = CFG
    SW, SWO, SX, SSM, SK, SV, SH, SQ, SOUT = 0, 12, 20, 26, 29, 31, 33, 35, 37

    def w_copy(g, c):
        r0 = c * 256
        return pltpu.make_async_copy(
            w_hbm[g // 2].at[pl.ds(r0, 256), pl.ds(16 * (g % 2), 16), :],
            stage[g % 3].at[pl.ds(r0, 256)],
            sems.at[SW + (g % 3) * 4 + c])

    def wo_copy(n):
        return pltpu.make_async_copy(
            wo_hbm.at[:, :, pl.ds(pl.multiple_of(n * 128, 128), 128)],
            wo_st.at[pl.ds(n * 256, 256)], sems.at[SWO + n])

    def xc_copy(c):
        cols = pl.ds(pl.multiple_of(c * 256, 256), 256)
        return pltpu.make_async_copy(x_hbm.at[pl.ds(0, PRE), cols],
                                     x_buf.at[pl.ds(0, PRE), cols], sems.at[SX + c])

    def x_copy(part):
        r0, n = ((PRE, 256), (PRE + 256, S - PRE - 256))[part]
        return pltpu.make_async_copy(
            x_hbm.at[pl.ds(r0, n)], x_buf.at[pl.ds(r0, n)], sems.at[SX + 4 + part])

    def small_copies():
        return [pltpu.make_async_copy(skt_hbm, skt_buf, sems.at[SSM + 0]),
                pltpu.make_async_copy(dd_hbm, dd_buf, sems.at[SSM + 1]),
                pltpu.make_async_copy(mem0_hbm, mem_ref, sems.at[SSM + 2])]

    def col(b):
        return pl.ds(pl.multiple_of(b * 128, 128), 128)

    def kvh_copies(b):
        sl = b % 2
        return [pltpu.make_async_copy(k_hbm.at[:, col(b)],
                                      k_buf.at[sl, pl.ds(KPAD, S)], sems.at[SK + sl]),
                pltpu.make_async_copy(v_hbm.at[:, col(b)], v_buf.at[sl], sems.at[SV + sl]),
                pltpu.make_async_copy(h_hbm.at[col(b)], h_buf.at[sl], sems.at[SH + sl])]

    def q_copy(b):
        sl = b % 2
        return pltpu.make_async_copy(q_hbm.at[:, col(b)], q_buf.at[sl], sems.at[SQ + sl])

    def outa_copy(b):
        return pltpu.make_async_copy(kvo.at[b], out_hbm.at[:, col(b)], sems.at[SOUT + 0])

    def outa_piece(b, r0, n):
        return pltpu.make_async_copy(kvo.at[b, pl.ds(r0, n)],
                                     out_hbm.at[pl.ds(r0, n), col(b)], sems.at[SOUT + 1])

    def outb_piece(r0, n):
        return pltpu.make_async_copy(outb.at[pl.ds(r0, n)],
                                     out_hbm.at[pl.ds(r0, n), pl.ds(D, D)], sems.at[SOUT + 3])

    def outb_copy(cb):
        rows = pl.ds(pl.multiple_of(cb * 8 * SEG, 8 * SEG), 8 * SEG)
        return pltpu.make_async_copy(outb.at[rows], out_hbm.at[rows, pl.ds(D, D)],
                                     sems.at[SOUT + 2])

    def relayout(g, c, lo_i=0, hi_i=128):
        src, dst = stage[g % 3], wp[g]
        d0 = c * 256
        for i in range(lo_i, hi_i):
            a = pltpu.bitcast(src[d0 + 2 * i], u32)
            b = pltpu.bitcast(src[d0 + 2 * i + 1], u32)
            lo = (a & jnp.uint32(0xFFFF)) | (b << 16)
            hi = (a >> 16) | (b & jnp.uint32(0xFFFF0000))
            row = c * 128 + i
            dst[pl.ds(row, 8, stride=2 * HS), :] = lo
            dst[pl.ds(row + HS, 8, stride=2 * HS), :] = hi

    def wo_pack(n, r0=0, r1=256):
        for r in range(r0, r1, 8):
            blk = pltpu.bitcast(wo_st[pl.ds(n * 256 + r, 8)], u32)
            wo_p[n, r * 8:(r + 8) * 8, :] = blk.reshape(64, 128)

    def wt(m, h):
        g, hh = 2 * m + h // 16, h % 16
        return _bf(wp[g][hh * HS:hh * HS + D // 2, :])

    def ring_cols(m, p):
        c0 = 512 * m + 256 * (p % 2)
        return slice(c0, c0 + 256)

    def s0_kv(sl, b, slot, j, i):
        t0 = pl.multiple_of(j * 2 * C, 2 * C)
        kw = k_buf.at[sl, pl.ds(t0, 2 * C + KPAD)]
        vw = v_buf.at[sl, pl.ds(t0, 2 * C)]
        ow = kvo.at[slot, pl.ds(t0, 2 * C)]
        kf[i] = kw[32 * i:32 * i + 32 + KPAD, :].astype(f32)
        acc = None
        for tap in range(KS):
            term = kf[i, KPAD - tap:KPAD - tap + 32, :] * coef[b, tap:tap + 1, :]
            acc = term if acc is None else acc + term
        ow[32 * i:32 * i + 32, :] = (acc * vw[32 * i:32 * i + 32, :].astype(f32)).astype(bf16)

    def s1_h(sl, j):
        for t in range(2):
            a = 2 * j + t
            hh = h_buf[sl, :, pl.ds(pl.multiple_of(a * C, C), C)]
            for half in range(2):
                fm = _bf(f_p[half * 64:(half + 1) * 64, :])
                uh[sl * 2 * NC + NC + a, half * C:(half + 1) * C, :] = lax.dot_general(
                    fm, hh, (((1,), (1,)), ((), ())), preferred_element_type=f32)

    def s1_u(sl, slot, j):
        for t in range(2):
            a = 2 * j + t
            kv = kvo[slot, pl.ds(pl.multiple_of(a * C, C), C), :]
            for half in range(2):
                fm = _bf(f_p[half * 64:(half + 1) * 64, :])
                uh[sl * 2 * NC + a, half * C:(half + 1) * C, :] = jnp.dot(
                    fm, kv, preferred_element_type=f32)

    def s2_parts(sl, j):
        sgn = (1 - 2 * (lax.broadcasted_iota(i32, (8, 128), 0) % 2)).astype(f32)
        u0 = sl * 2 * NC
        h0 = u0 + NC
        r0 = pl.multiple_of(j * 32, 32)
        prev = []

        def one(idx, pace):
            grp, a = divmod(idx, NC)
            re, im = pl.ds(r0 + 16 * grp, 8), pl.ds(r0 + 16 * grp + 8, 8)
            yr = yi = None
            for b in range(a + 1):
                if b == a:
                    uh[4 * NC, 0:8, :] = pace
                ur, ui = uh[u0 + b, re, :], uh[u0 + b, im, :]
                hr, hi = uh[h0 + a - b, re, :], uh[h0 + a - b, im, :]
                yr = ur * hr if yr is None else yr + ur * hr
                yi = ur * hi if yi is None else yi + ur * hi
                yr = yr - ui * hi
                yi = yi + ui * hr
            if a > 0:
                zr, zi = yr - prev[1], yi + prev[0]
            else:
                zr, zi = yr, yi
            prev[:] = [yr * sgn, yi * sgn]
            z = jnp.concatenate([zr, zi], axis=0).astype(bf16)
            r = (a % 2) * 16 + 8 * grp
            y_buf[sl, j, a // 2, r:r + 8, :] = pltpu.bitcast(z, u32)
        return one

    def s3(sl, b, slot, j):
        gm = _bf(g_p[...])
        for t in range(2):
            a = 2 * j + t
            rows = pl.ds(pl.multiple_of(a * C, C), C)
            yp = y_buf[sl, :, j, 16 * t:16 * t + 16, :].reshape(C, 128)
            y = jnp.dot(gm, _bf(yp), preferred_element_type=f32)
            y = y + kvo[slot, rows, :].astype(f32) * coef[b, KS:KS + 1, :]
            kvo[slot, rows, :] = (q_buf[sl, rows, :].astype(f32) * y).astype(bf16)

    for cp in small_copies():
        cp.start()
    for c in range(4):
        xc_copy(c).start()
        w_copy(0, c).start()
        if c > 0:
            w_copy(1, c - 1).start()

    r = lax.broadcasted_iota(i32, (L2, L2), 0)
    c_ = lax.broadcasted_iota(i32, (L2, L2), 1)
    head = lambda i: jnp.where(i < 2 * M, i // M, (i - 2 * M) // SEG)
    ok = (r < 2 * M) | (c_ < 2 * M) | (c_ <= r)
    fill_ref[...] = jnp.where(head(r) == head(c_),
                              jnp.where(ok, 0.0, -1e9 / scale), -jnp.inf).astype(f32)

    rr = lax.broadcasted_iota(i32, (2 * C, C), 0)
    nn = lax.broadcasted_iota(i32, (2 * C, C), 1)
    kk = 8 * (rr // 16) + rr % 8
    mm = ((2 * kk + 1) * nn + C * ((rr // 8) % 2)) % (4 * C)
    fm = jnp.cos(mm.astype(f32) * (math.pi / (2 * C)))
    f_p[...] = pltpu.bitcast(fm.astype(bf16), u32)
    g_p[...] = pltpu.bitcast((fm.T * (1.0 / C)).astype(bf16), u32)
    for sl in range(2):
        k_buf[sl, 0:KPAD, :] = jnp.zeros((KPAD, 128), bf16)
    uh[0:32] = jnp.zeros((32, 2 * C, 128), f32)

    for cp in small_copies():
        cp.wait()
    skt = skt_buf[...].astype(f32)
    ddv = dd_buf[...].astype(f32)
    for b in range(NB):
        coef[b, 0:KS, :] = skt[:, b * 128:(b + 1) * 128]
        coef[b, KS:KS + 1, :] = ddv[b:b + 1, :]

    def pro_body(g, i, tasks):
        r0 = pl.multiple_of(i * 128, 128)
        x = x_buf[pl.ds(r0, 128), :]
        for p in range(8):
            ys = []
            for t in range(2):
                y = jnp.dot(x, wt(g // 2, 16 * (g % 2) + 2 * p + t),
                            preferred_element_type=f32)
                ys.append(y)
                for fn in tasks.get(2 * p + t, ()):
                    fn(y)
            pp = 8 * (g % 2) + p
            ring[pp // 2][pl.ds(pl.multiple_of(QOFF + r0, 64), 128),
                          ring_cols(g // 2, pp)] = jnp.concatenate(ys, axis=1).astype(bf16)

    def add_relayout(tasks, g, c, r):
        for u in range(15):
            def fn(y, u=u):
                stage[g % 3][D] = y[r:r + 16].astype(bf16)
                relayout(g, c, (128 * u) // 15, (128 * (u + 1)) // 15)
            tasks.setdefault(u, []).append(fn)

    def add_wo(tasks, n0):
        for u in range(15):
            def fn(y, u=u):
                wo_st[2048] = y[96:112].astype(bf16)
                for r in range((64 * u) // 15, (64 * (u + 1)) // 15):
                    wo_pack(n0 + r // 32, 8 * (r % 32), 8 * (r % 32) + 8)
            tasks.setdefault(u, []).append(fn)

    def add_s01(tasks, j):
        for k in range(8):
            def fn(y, k=k):
                coef[NB, 0:8, :] = y[48:56]
                s0_kv(0, 0, 0, j, k)
            tasks.setdefault(k, []).append(fn)
        tasks.setdefault(3, []).append(lambda y: s1_h(0, j))
        tasks.setdefault(11, []).append(lambda y: s1_u(0, 0, j))

    def period(g, body):
        if cfg['nopro']:
            return
        with jax.named_scope('pro%d' % g):
            lax.fori_loop(0, 4, lambda i, c: (body(i), c)[1], 0)

    def p0(c):
        @pl.when(c == 1)
        def _():
            w_copy(1, 3).start()
            for i in range(4):
                w_copy(2, i).start()

        @pl.when(c > 0)
        def _():
            w_copy(1, c - 1).wait()
        xc_copy(c).wait()
        w_copy(0, c).wait()
        relayout(0, c)
        xp[...] = pltpu.bitcast(
            x_buf[0:PRE, pl.ds(pl.multiple_of(c * 256, 256), 256)], u32)
        tasks = {}
        add_relayout(tasks, 1, (c + 3) % 4, 0)
        k0 = pl.multiple_of(c * 128, 128)
        for p in range(8):
            ys = []
            for t in range(2):
                hh = 2 * p + t
                w = _bf(wp[0][pl.ds(k0 + hh * HS, 128), :])
                y = (jnp.dot(_bf(xp[...]), w, preferred_element_type=f32)
                     + uh[2 * hh:2 * hh + 2].reshape(PRE, 128))
                uh[2 * hh:2 * hh + 2] = y.reshape(2, 2 * C, 128)
                ys.append(y)
                for fn in tasks.get(hh, ()):
                    fn(y[256 * t:])
            ring[p // 2][QOFF:QOFF + PRE, ring_cols(0, p)] = (
                jnp.concatenate(ys, axis=1).astype(bf16))
    period(0, p0)
    w_copy(1, 3).wait()
    relayout(1, 3)

    def p1(i):
        @pl.when(i == 0)
        def _():
            w_copy(3, 0).start()
            w_copy(3, 1).start()
            for cp in kvh_copies(0):
                cp.start()
            w_copy(4, 0).start()
            w_copy(4, 1).start()
            for c in range(2, 4):
                w_copy(3, c).start()
                w_copy(4, c).start()
        w_copy(2, i).wait()
        tasks = {}
        add_relayout(tasks, 2, i, 0)
        pro_body(1, i, tasks)
    period(1, p1)

    def p2(i):
        @pl.when(i == 0)
        def _():
            for c in range(4):
                w_copy(5, c).start()
                wo_copy(2 * c).start()
                wo_copy(2 * c + 1).start()
            x_copy(0).start()
            for cp in kvh_copies(1):
                cp.start()
            x_copy(1).start()
            for cp in kvh_copies(0):
                cp.wait()
        w_copy(3, i).wait()
        w_copy(4, i).wait()
        tasks = {}
        add_relayout(tasks, 3, i, 0)
        add_relayout(tasks, 4, i, 96)
        add_s01(tasks, i)
        pro_body(2, i, tasks)
    period(2, p2)

    def p3(i):
        w_copy(5, i).wait()
        wo_copy(2 * i).wait()
        wo_copy(2 * i + 1).wait()
        tasks = {}
        add_relayout(tasks, 5, i, 0)
        add_wo(tasks, 2 * i)
        add_s01(tasks, 4 + i)
        pro_body(3, i, tasks)
    period(3, p3)
    x_copy(0).wait()

    def step(cb, j, mem, par):
        s = cb * 8 + j
        x0 = pl.multiple_of(PRE + XR * s, 8)
        wpos = pl.multiple_of(lax.rem(s, RING // XR) * XR, 8)
        rpos = pl.multiple_of(lax.rem(s + QOFF // SEG, RING // SEG) * SEG, 32)
        rbase = pl.multiple_of((s - par) * SEG, 64)
        m0 = 0 if par == 0 else 72
        x8 = 8 + SEG * par

        sl1 = (cb + 1) % 2
        b1 = jnp.minimum(cb + 1, NB - 1)
        slot1 = cb + 1
        b3 = jnp.maximum(cb - 1, 0)
        slot3 = jnp.where(cb == 0, NB, cb - 1)
        s2 = s2_parts(cb % 2, j)
        nu = [0]

        def unit(pace):
            u = nu[0]
            nu[0] += 1
            if u in cfg['s0_at'][par]:
                coef[NB, 0:8, :] = pace
                s0_kv(sl1, b1, slot1, j, cfg['s0_at'][par].index(u))
            if u in cfg['s2_at'][par]:
                s2(cfg['s2_at'][par].index(u), pace)

        def proj_q(p, lq):
            ys = []
            for t in range(2):
                ys.append(jnp.dot(lq, wt(2, 2 * p + t), preferred_element_type=f32))
                unit(ys[-1][:M])
            r0, r1 = (0, 48) if par == 0 else (48, 80)
            q_sc[p][r0:r1, :] = jnp.concatenate(ys, axis=1).astype(bf16)

        def proj_kv(p, m, lhs):
            ys = [jnp.dot(lhs, wt(m, 2 * p + t), preferred_element_type=f32)
                  for t in range(2)]
            ring[p // 2][pl.ds(wpos, XR), ring_cols(m, p)] = jnp.concatenate(
                [y[M:] for y in ys], axis=1).astype(bf16)
            unit(ys[0][:M])
            return jnp.concatenate([y[:M] for y in ys], axis=0).astype(bf16)

        def gather(m, p, mm):
            xx = ring[p // 2][pl.ds(rpos, SEG), ring_cols(m, p)]
            return jnp.concatenate([mm, xx[:, :DH], xx[:, DH:]], axis=0)

        def qk(p, mems):
            b = q_sc[p]
            q2 = jnp.concatenate([b[m0:m0 + M, :DH], b[m0:m0 + M, DH:],
                                  b[x8:x8 + SEG, :DH], b[x8:x8 + SEG, DH:]], axis=0)
            sc = lax.dot_general(q2, gather(0, p, mems[0]), (((1,), (1,)), ((), ())),
                                 preferred_element_type=f32)
            fill = fill_ref[...]
            sc = jnp.where(fill == 0.0, sc, fill)
            mx = jnp.max(sc, axis=1, keepdims=True)
            e = jnp.exp((sc - mx) * scale)
            l = jnp.sum(e, axis=1, keepdims=True)
            rc = pl.reciprocal(l, approx=True)
            rc = rc * (2.0 - l * rc)
            return (e * rc).astype(bf16)

        def pv(p, pr, mems):
            o = jnp.dot(pr, gather(1, p, mems[1]), preferred_element_type=f32)
            o_sc[p][m0:m0 + M, :] = jnp.concatenate([o[0:M], o[M:2 * M]], axis=1).astype(bf16)
            o_sc[p][x8:x8 + SEG, :] = jnp.concatenate(
                [o[2 * M:2 * M + SEG], o[2 * M + SEG:]], axis=1).astype(bf16)

        def ochain(n, k0, k1, acc):
            r0, r1 = (0, 32) if par == 0 else (32, 80)
            for k in range(k0, k1, cfg['och']):
                ke = min(k + cfg['och'], k1)
                l = jnp.concatenate([o_sc[p][r0:r1, :] for p in range(k // 2, ke // 2)], axis=1)
                y = jnp.dot(l, _bf(wo_p[n, k * 64:ke * 64, :]), preferred_element_type=f32)
                acc = y if acc is None else y + acc
                unit(acc[:M])
            return acc

        n1 = s + 7
        s1_u((n1 // 8) % 2, n1 // 8, n1 % 8)
        s1_h(sl1, j)
        s3(sl1, b3, slot3, j)

        if par == 0:
            lq = jnp.concatenate([mem, x_buf[pl.ds(rbase, 40), :]], axis=0)
        else:
            lq = jnp.concatenate([x_buf[pl.ds(rbase + 40, 24), :], mem], axis=0)
        for p in range(NPAIR):
            proj_q(p, lq)

        lhs = jnp.concatenate([mem, x_buf[pl.ds(x0, XR), :]], axis=0)
        mems, prs, parts = {}, {}, []
        for t in range(NPAIR + cfg['lagpv']):
            if t < NPAIR:
                mems[t] = [proj_kv(t, m, lhs) for m in range(2)]
            else:
                for _ in range(cfg['op_per']):
                    parts.append(ochain(len(parts), 0, cfg['k1'], None))
            if t % 2 == 0:
                for p in (t - cfg['lagpv'] - 1, t - cfg['lagpv']):
                    if 0 <= p < NPAIR:
                        pv(p, prs.pop(p), mems.pop(p))
                for p in (t - cfg['lagqk'] - 1, t - cfg['lagqk']):
                    if 0 <= p < NPAIR:
                        prs[p] = qk(p, mems[p])
        while len(parts) < 8:
            parts.append(ochain(len(parts), 0, cfg['k1'], None))
        out = jnp.concatenate([ochain(n, cfg['k1'], H, parts[n]) for n in range(8)],
                              axis=1).astype(bf16)
        if par == 0:
            outb[pl.ds(rbase, 24), :] = out[M:]
            return out[:M]
        outb[pl.ds(rbase + 24, 40), :] = out[:40]
        return out[40:]

    def outer(cb, carry):
        @pl.when(cb + 2 < NB)
        def _():
            for cp in kvh_copies(cb + 2):
                cp.start()

        q_copy(cb).start()

        @pl.when(cb >= 2)
        def _():
            outa_copy(cb - 2).start()

        @pl.when(cb >= 1)
        def _():
            outb_copy(cb - 1).start()
            q_copy(cb - 1).wait()

        @pl.when(cb == 1)
        def _():
            x_copy(1).wait()

        @pl.when(cb + 1 < NB)
        def _():
            for cp in kvh_copies(cb + 1):
                cp.wait()

        def inner(jj, c2):
            @pl.when(jnp.logical_and(cb == NB - 1, jj > 0))
            def _():
                outa_piece(NB - 2, pl.multiple_of((jj - 1) * 4 * C, 4 * C), 4 * C).start()
                outb_piece(pl.multiple_of(S - 5 * 64 + jj * 64, 64), 64).start()
            mem = mem_ref[...]
            for u in range(2):
                mem = step(cb, jj * 2 + u, mem, u)
            mem_ref[...] = mem
            return c2
        with jax.named_scope('inner'):
            lax.fori_loop(0, 4, inner, 0)
        return carry
    with jax.named_scope('main'):
        lax.fori_loop(0, NB, outer, 0)

    outb_piece(S - 64, 64).start()
    outa_piece(NB - 2, 12 * C, 4 * C).start()
    q_copy(NB - 1).wait()
    with jax.named_scope('epi'):
        for j in range(8):
            s3((NB - 1) % 2, NB - 1, NB - 1, j)
            if j % 2 == 1:
                outa_piece(NB - 1, (j - 1) * 2 * C, 4 * C).start()

    for b in range(NB - 2):
        outa_copy(b).wait()
    for n in range(NB - 1):
        outb_copy(n).wait()
    for j in range(4):
        outb_piece(S - 256 + 64 * j, 64).wait()
        outa_piece(NB - 2, j * 4 * C, 4 * C).wait()
        outa_piece(NB - 1, j * 4 * C, 4 * C).wait()


@functools.partial(jax.jit, static_argnames=("B_seg_len",))
def pallas_concat_heads__ssm_conv_h3__memory_aug_recurrent_mem_tr__prompt_kernel(
    A_q, A_k, A_v, A_shift_k, A_ssm_k, A_ssm_D, B_x, B_mem0, B_Wq, B_Wk, B_Wv, B_Wo,
    B_seg_len=SEG,
):
    assert B_seg_len == SEG
    assert A_q.shape == (1, S, D) and B_x.shape == (1, S, D)
    assert B_Wq.shape == (D, H, DH) and B_mem0.shape == (1, M, D)
    vm = pltpu.VMEM
    dma = pltpu.SemaphoreType.DMA
    scratch = [
        vm((D + 4, 16, DH), bf16), vm((D + 4, 16, DH), bf16),
        vm((D + 4, 16, DH), bf16),
        vm((2048 + 4, 16, 128), bf16),
        vm((8, H * DH // 2, 128), u32),
        vm((S, D), bf16),
        vm((M, D), bf16),
        vm((S, D), bf16),
        vm((NB + 1, 32, 128), f32),
        vm((2, S + 64, 128), bf16),
        vm((2, S, 128), bf16), vm((2, S, 128), bf16),
        vm((2, 128, S), bf16),
        vm((NB + 1, S, 128), bf16),
        vm((4 * NC + 1, 2 * C, 128), f32),
        vm((2, 8, 8, 32, 128), u32),
        vm((8, 32 + KPAD, 128), f32),
        vm((C, C), u32), vm((C // 2, 2 * C), u32),
        vm((PRE // 2, 256), u32),
        dma((41,)),
    ]
    scratch += [vm((16 * HS, 128), u32)] * 6
    scratch += [vm((RING, 8 * DH), bf16)] * 8
    scratch += [vm((L2, 2 * DH), bf16)] * (2 * NPAIR)
    scratch += [vm((L2, L2), f32), vm((KS, D), bf16), vm((NB, 128), bf16)]

    out = pl.pallas_call(
        _kernel,
        out_shape=jax.ShapeDtypeStruct((S, 2 * D), bf16),
        in_specs=[pl.BlockSpec(memory_space=pl.ANY)] * 12,
        out_specs=pl.BlockSpec(memory_space=pl.ANY),
        scratch_shapes=scratch,
        compiler_params=pltpu.CompilerParams(vmem_limit_bytes=120 * 1024 * 1024,
                                             disable_bounds_checks=True,
                                             disable_semaphore_checks=True),
        name="ssm_memtr",
    )(A_q.reshape(S, D), A_k.reshape(S, D), A_v.reshape(S, D), A_shift_k.T, A_ssm_k,
      A_ssm_D.reshape(NB, 128), B_x.reshape(S, D), B_mem0.reshape(M, D),
      B_Wq, B_Wk, B_Wv, B_Wo.reshape(H * DH // 16, 16, D))
    return out.reshape(1, S, 2 * D)
```

```python
import functools
import math

import jax
import jax.numpy as jnp
from jax import lax
import jax.experimental.pallas as pl
import jax.experimental.pallas.tpu as pltpu

bf16, f32, u32, i32 = jnp.bfloat16, jnp.float32, jnp.uint32, jnp.int32

S = 2048
D = 1024
H, DH = 32, 128
M, SEG = 8, 32
NSEG = S // SEG
KS = 4

XR = 24
PRE = S - NSEG * XR
RING = 576
QOFF = 64
HS = 514
NPAIR = H // 2
L2 = 2 * (M + SEG)

C = 128
NC = S // C
NB = D // 128
KPAD = 16

CFG = dict(
    agroup=2, pstore=True, och=8, op_per=[4, 3],
    s2_at=[list(range(0, 32)), list(range(62, 94))],
    s0_at=[list(range(0, 4)) + list(range(16, 20)), list(range(62, 66)) + list(range(78, 82))],
    nopro=False, unroll=4,
)


def _bf(x):
    return pltpu.bitcast(x, bf16)


def _kernel(q_hbm, k_hbm, v_hbm, skt_hbm, h_hbm, dd_hbm, x_hbm, mem0_hbm,
            wq_hbm, wk_hbm, wv_hbm, wo_hbm, out_hbm,
            st0, st1, st2, wo_st, wo_p, x_buf, mem_ref, outb,
            coef, k_buf, v_buf, q_buf, h_buf, kvo,
            uh, y_buf, kf, f_p, g_p, xp, sems,
            *bufs):
    wp = bufs[0:6]
    ring = bufs[6:14]
    o_sc = bufs[14:30]
    q_sc = bufs[30:46]
    p_sc, fill_ref, skt_buf, dd_buf = bufs[46:50]
    stage = (st0, st1, st2)
    w_hbm = (wk_hbm, wv_hbm, wq_hbm)
    scale = DH ** -0.5
    cfg = CFG
    SW, SWO, SX, SSM, SK, SV, SH, SQ, SOUT = 0, 12, 20, 26, 29, 31, 33, 35, 37

    def w_copy(g, c):
        r0 = c * 256
        return pltpu.make_async_copy(
            w_hbm[g // 2].at[pl.ds(r0, 256), pl.ds(16 * (g % 2), 16), :],
            stage[g % 3].at[pl.ds(r0, 256)],
            sems.at[SW + (g % 3) * 4 + c])

    def wo_copy(n):
        return pltpu.make_async_copy(
            wo_hbm.at[:, :, pl.ds(pl.multiple_of(n * 128, 128), 128)],
            wo_st.at[pl.ds(n * 256, 256)], sems.at[SWO + n])

    def xc_copy(c):
        cols = pl.ds(pl.multiple_of(c * 256, 256), 256)
        return pltpu.make_async_copy(x_hbm.at[pl.ds(0, PRE), cols],
                                     x_buf.at[pl.ds(0, PRE), cols], sems.at[SX + c])

    def x_copy(part):
        r0, n = ((PRE, 256), (PRE + 256, S - PRE - 256))[part]
        return pltpu.make_async_copy(
            x_hbm.at[pl.ds(r0, n)], x_buf.at[pl.ds(r0, n)], sems.at[SX + 4 + part])

    def small_copies():
        return [pltpu.make_async_copy(skt_hbm, skt_buf, sems.at[SSM + 0]),
                pltpu.make_async_copy(dd_hbm, dd_buf, sems.at[SSM + 1]),
                pltpu.make_async_copy(mem0_hbm, mem_ref, sems.at[SSM + 2])]

    def col(b):
        return pl.ds(pl.multiple_of(b * 128, 128), 128)

    def kvh_copies(b):
        sl = b % 2
        return [pltpu.make_async_copy(k_hbm.at[:, col(b)],
                                      k_buf.at[sl, pl.ds(KPAD, S)], sems.at[SK + sl]),
                pltpu.make_async_copy(v_hbm.at[:, col(b)], v_buf.at[sl], sems.at[SV + sl]),
                pltpu.make_async_copy(h_hbm.at[col(b)], h_buf.at[sl], sems.at[SH + sl])]

    def q_copy(b):
        sl = b % 2
        return pltpu.make_async_copy(q_hbm.at[:, col(b)], q_buf.at[sl], sems.at[SQ + sl])

    def outa_copy(b):
        return pltpu.make_async_copy(kvo.at[b], out_hbm.at[:, col(b)], sems.at[SOUT + 0])

    def outa_piece(b, r0, n):
        return pltpu.make_async_copy(kvo.at[b, pl.ds(r0, n)],
                                     out_hbm.at[pl.ds(r0, n), col(b)], sems.at[SOUT + 1])

    def outb_piece(r0, n):
        return pltpu.make_async_copy(outb.at[pl.ds(r0, n)],
                                     out_hbm.at[pl.ds(r0, n), pl.ds(D, D)], sems.at[SOUT + 3])

    def outb_copy(cb):
        rows = pl.ds(pl.multiple_of(cb * 8 * SEG, 8 * SEG), 8 * SEG)
        return pltpu.make_async_copy(outb.at[rows], out_hbm.at[rows, pl.ds(D, D)],
                                     sems.at[SOUT + 2])

    def relayout(g, c, lo_i=0, hi_i=128):
        src, dst = stage[g % 3], wp[g]
        d0 = c * 256
        for i in range(lo_i, hi_i):
            a = pltpu.bitcast(src[d0 + 2 * i], u32)
            b = pltpu.bitcast(src[d0 + 2 * i + 1], u32)
            lo = (a & jnp.uint32(0xFFFF)) | (b << 16)
            hi = (a >> 16) | (b & jnp.uint32(0xFFFF0000))
            row = c * 128 + i
            dst[pl.ds(row, 8, stride=2 * HS), :] = lo
            dst[pl.ds(row + HS, 8, stride=2 * HS), :] = hi

    def wo_pack(n, r0=0, r1=256):
        for r in range(r0, r1, 8):
            blk = pltpu.bitcast(wo_st[pl.ds(n * 256 + r, 8)], u32)
            wo_p[n, r * 8:(r + 8) * 8, :] = blk.reshape(64, 128)

    def wt(m, h):
        g, hh = 2 * m + h // 16, h % 16
        return _bf(wp[g][hh * HS:hh * HS + D // 2, :])

    def ring_cols(m, p):
        c0 = 512 * m + 256 * (p % 2)
        return slice(c0, c0 + 256)

    def s0_kv(sl, b, slot, j, i):
        t0 = pl.multiple_of(j * 2 * C, 2 * C)
        kw = k_buf.at[sl, pl.ds(t0, 2 * C + KPAD)]
        vw = v_buf.at[sl, pl.ds(t0, 2 * C)]
        ow = kvo.at[slot, pl.ds(t0, 2 * C)]
        kf[i] = kw[32 * i:32 * i + 32 + KPAD, :].astype(f32)
        acc = None
        for tap in range(KS):
            term = kf[i, KPAD - tap:KPAD - tap + 32, :] * coef[b, tap:tap + 1, :]
            acc = term if acc is None else acc + term
        ow[32 * i:32 * i + 32, :] = (acc * vw[32 * i:32 * i + 32, :].astype(f32)).astype(bf16)

    def s1_h(sl, j):
        for t in range(2):
            a = 2 * j + t
            hh = h_buf[sl, :, pl.ds(pl.multiple_of(a * C, C), C)]
            for half in range(2):
                fm = _bf(f_p[half * 64:(half + 1) * 64, :])
                uh[sl * 2 * NC + NC + a, half * C:(half + 1) * C, :] = lax.dot_general(
                    fm, hh, (((1,), (1,)), ((), ())), preferred_element_type=f32)

    def s1_u(sl, slot, j):
        for t in range(2):
            a = 2 * j + t
            kv = kvo[slot, pl.ds(pl.multiple_of(a * C, C), C), :]
            for half in range(2):
                fm = _bf(f_p[half * 64:(half + 1) * 64, :])
                uh[sl * 2 * NC + a, half * C:(half + 1) * C, :] = jnp.dot(
                    fm, kv, preferred_element_type=f32)

    def s2_parts(sl, j):
        sgn = (1 - 2 * (lax.broadcasted_iota(i32, (8, 128), 0) % 2)).astype(f32)
        u0 = sl * 2 * NC
        h0 = u0 + NC
        r0 = pl.multiple_of(j * 32, 32)
        prev = []

        def one(idx, pace):
            grp, a = divmod(idx, NC)
            re, im = pl.ds(r0 + 16 * grp, 8), pl.ds(r0 + 16 * grp + 8, 8)
            yr = yi = None
            for b in range(a + 1):
                if b == a:
                    uh[4 * NC, 0:8, :] = pace
                ur, ui = uh[u0 + b, re, :], uh[u0 + b, im, :]
                hr, hi = uh[h0 + a - b, re, :], uh[h0 + a - b, im, :]
                yr = ur * hr if yr is None else yr + ur * hr
                yi = ur * hi if yi is None else yi + ur * hi
                yr = yr - ui * hi
                yi = yi + ui * hr
            if a > 0:
                zr, zi = yr - prev[1], yi + prev[0]
            else:
                zr, zi = yr, yi
            prev[:] = [yr * sgn, yi * sgn]
            z = jnp.concatenate([zr, zi], axis=0).astype(bf16)
            r = (a % 2) * 16 + 8 * grp
            y_buf[sl, j, a // 2, r:r + 8, :] = pltpu.bitcast(z, u32)
        return one

    def s3(sl, b, slot, j):
        gm = _bf(g_p[...])
        for t in range(2):
            a = 2 * j + t
            rows = pl.ds(pl.multiple_of(a * C, C), C)
            yp = y_buf[sl, :, j, 16 * t:16 * t + 16, :].reshape(C, 128)
            y = jnp.dot(gm, _bf(yp), preferred_element_type=f32)
            y = y + kvo[slot, rows, :].astype(f32) * coef[b, KS:KS + 1, :]
            kvo[slot, rows, :] = (q_buf[sl, rows, :].astype(f32) * y).astype(bf16)

    for cp in small_copies():
        cp.start()
    for c in range(4):
        xc_copy(c).start()
        w_copy(0, c).start()
        if c > 0:
            w_copy(1, c - 1).start()

    r = lax.broadcasted_iota(i32, (L2, L2), 0)
    c_ = lax.broadcasted_iota(i32, (L2, L2), 1)
    head = lambda i: jnp.where(i < 2 * M, i // M, (i - 2 * M) // SEG)
    ok = (r < 2 * M) | (c_ < 2 * M) | (c_ <= r)
    fill_ref[...] = jnp.where(head(r) == head(c_),
                              jnp.where(ok, 0.0, -1e9 / scale), -jnp.inf).astype(f32)

    rr = lax.broadcasted_iota(i32, (2 * C, C), 0)
    nn = lax.broadcasted_iota(i32, (2 * C, C), 1)
    kk = 8 * (rr // 16) + rr % 8
    mm = ((2 * kk + 1) * nn + C * ((rr // 8) % 2)) % (4 * C)
    fm = jnp.cos(mm.astype(f32) * (math.pi / (2 * C)))
    f_p[...] = pltpu.bitcast(fm.astype(bf16), u32)
    g_p[...] = pltpu.bitcast((fm.T * (1.0 / C)).astype(bf16), u32)
    for sl in range(2):
        k_buf[sl, 0:KPAD, :] = jnp.zeros((KPAD, 128), bf16)
    uh[0:32] = jnp.zeros((32, 2 * C, 128), f32)

    for cp in small_copies():
        cp.wait()
    skt = skt_buf[...].astype(f32)
    ddv = dd_buf[...].astype(f32)
    for b in range(NB):
        coef[b, 0:KS, :] = skt[:, b * 128:(b + 1) * 128]
        coef[b, KS:KS + 1, :] = ddv[b:b + 1, :]

    def pro_body(g, i, tasks):
        r0 = pl.multiple_of(i * 128, 128)
        x = x_buf[pl.ds(r0, 128), :]
        for p in range(8):
            ys = []
            for t in range(2):
                y = jnp.dot(x, wt(g // 2, 16 * (g % 2) + 2 * p + t),
                            preferred_element_type=f32)
                ys.append(y)
                for fn in tasks.get(2 * p + t, ()):
                    fn(y)
            pp = 8 * (g % 2) + p
            ring[pp // 2][pl.ds(pl.multiple_of(QOFF + r0, 64), 128),
                          ring_cols(g // 2, pp)] = jnp.concatenate(ys, axis=1).astype(bf16)

    def add_relayout(tasks, g, c, r):
        for u in range(15):
            def fn(y, u=u):
                stage[g % 3][D] = y[r:r + 16].astype(bf16)
                relayout(g, c, (128 * u) // 15, (128 * (u + 1)) // 15)
            tasks.setdefault(u, []).append(fn)

    def add_wo(tasks, n0):
        for u in range(15):
            def fn(y, u=u):
                wo_st[2048] = y[96:112].astype(bf16)
                for r in range((64 * u) // 15, (64 * (u + 1)) // 15):
                    wo_pack(n0 + r // 32, 8 * (r % 32), 8 * (r % 32) + 8)
            tasks.setdefault(u, []).append(fn)

    def add_s01(tasks, j):
        for k in range(8):
            def fn(y, k=k):
                coef[NB, 0:8, :] = y[48:56]
                s0_kv(0, 0, 0, j, k)
            tasks.setdefault(k, []).append(fn)
        tasks.setdefault(3, []).append(lambda y: s1_h(0, j))
        tasks.setdefault(11, []).append(lambda y: s1_u(0, 0, j))

    def period(g, body):
        if cfg['nopro']:
            return
        with jax.named_scope('pro%d' % g):
            lax.fori_loop(0, 4, lambda i, c: (body(i), c)[1], 0)

    def p0(c):
        @pl.when(c == 1)
        def _():
            w_copy(1, 3).start()
            for i in range(4):
                w_copy(2, i).start()

        @pl.when(c > 0)
        def _():
            w_copy(1, c - 1).wait()
        xc_copy(c).wait()
        w_copy(0, c).wait()
        relayout(0, c)
        xp[...] = pltpu.bitcast(
            x_buf[0:PRE, pl.ds(pl.multiple_of(c * 256, 256), 256)], u32)
        tasks = {}
        add_relayout(tasks, 1, (c + 3) % 4, 0)
        k0 = pl.multiple_of(c * 128, 128)
        for p in range(8):
            ys = []
            for t in range(2):
                hh = 2 * p + t
                w = _bf(wp[0][pl.ds(k0 + hh * HS, 128), :])
                y = (jnp.dot(_bf(xp[...]), w, preferred_element_type=f32)
                     + uh[2 * hh:2 * hh + 2].reshape(PRE, 128))
                uh[2 * hh:2 * hh + 2] = y.reshape(2, 2 * C, 128)
                ys.append(y)
                for fn in tasks.get(hh, ()):
                    fn(y[256 * t:])
            ring[p // 2][QOFF:QOFF + PRE, ring_cols(0, p)] = (
                jnp.concatenate(ys, axis=1).astype(bf16))
    period(0, p0)
    w_copy(1, 3).wait()
    relayout(1, 3)

    def p1(i):
        @pl.when(i == 0)
        def _():
            w_copy(3, 0).start()
            w_copy(3, 1).start()
            for cp in kvh_copies(0):
                cp.start()
            w_copy(4, 0).start()
            w_copy(4, 1).start()
            for c in range(2, 4):
                w_copy(3, c).start()
                w_copy(4, c).start()
        w_copy(2, i).wait()
        tasks = {}
        add_relayout(tasks, 2, i, 0)
        pro_body(1, i, tasks)
    period(1, p1)

    def p2(i):
        @pl.when(i == 0)
        def _():
            for c in range(4):
                w_copy(5, c).start()
                wo_copy(2 * c).start()
                wo_copy(2 * c + 1).start()
            x_copy(0).start()
            for cp in kvh_copies(1):
                cp.start()
            x_copy(1).start()
            for cp in kvh_copies(0):
                cp.wait()
        w_copy(3, i).wait()
        w_copy(4, i).wait()
        tasks = {}
        add_relayout(tasks, 3, i, 0)
        add_relayout(tasks, 4, i, 96)
        add_s01(tasks, i)
        pro_body(2, i, tasks)
    period(2, p2)

    def p3(i):
        w_copy(5, i).wait()
        wo_copy(2 * i).wait()
        wo_copy(2 * i + 1).wait()
        tasks = {}
        add_relayout(tasks, 5, i, 0)
        add_wo(tasks, 2 * i)
        add_s01(tasks, 4 + i)
        pro_body(3, i, tasks)
    period(3, p3)
    x_copy(0).wait()

    def step(cb, j, mem, par):
        s = cb * 8 + j
        x0 = pl.multiple_of(PRE + XR * s, 8)
        wpos = pl.multiple_of(lax.rem(s, RING // XR) * XR, 8)
        rpos = pl.multiple_of(lax.rem(s + QOFF // SEG, RING // SEG) * SEG, 32)
        rbase = pl.multiple_of((s - par) * SEG, 64)
        m0 = 0 if par == 0 else 72
        x8 = 8 + SEG * par

        sl1 = (cb + 1) % 2
        b1 = jnp.minimum(cb + 1, NB - 1)
        slot1 = cb + 1
        b3 = jnp.maximum(cb - 1, 0)
        slot3 = jnp.where(cb == 0, NB, cb - 1)
        s2 = s2_parts(cb % 2, j)
        nu = [0]

        def unit(pace):
            u = nu[0]
            nu[0] += 1
            if u in cfg['s0_at'][par]:
                coef[NB, 0:8, :] = pace
                s0_kv(sl1, b1, slot1, j, cfg['s0_at'][par].index(u))
            if u in cfg['s2_at'][par]:
                s2(cfg['s2_at'][par].index(u), pace)

        def proj_q(p, lq):
            ys = []
            for t in range(2):
                ys.append(jnp.dot(lq, wt(2, 2 * p + t), preferred_element_type=f32))
                unit(ys[-1][:M])
            r0, r1 = (0, 48) if par == 0 else (48, 80)
            q_sc[p][r0:r1, :] = jnp.concatenate(ys, axis=1).astype(bf16)

        def proj_kv(p, m, lhs):
            ys = [jnp.dot(lhs, wt(m, 2 * p + t), preferred_element_type=f32)
                  for t in range(2)]
            ring[p // 2][pl.ds(wpos, XR), ring_cols(m, p)] = jnp.concatenate(
                [y[M:] for y in ys], axis=1).astype(bf16)
            unit(ys[0][:M])
            return jnp.concatenate([y[:M] for y in ys], axis=0).astype(bf16)

        def gather(m, p, mm):
            xx = ring[p // 2][pl.ds(rpos, SEG), ring_cols(m, p)]
            return jnp.concatenate([mm, xx[:, :DH], xx[:, DH:]], axis=0)

        def qk(p, mems):
            b = q_sc[p]
            q2 = jnp.concatenate([b[m0:m0 + M, :DH], b[m0:m0 + M, DH:],
                                  b[x8:x8 + SEG, :DH], b[x8:x8 + SEG, DH:]], axis=0)
            sc = lax.dot_general(q2, gather(0, p, mems[0]), (((1,), (1,)), ((), ())),
                                 preferred_element_type=f32)
            fill = fill_ref[...]
            sc = jnp.where(fill == 0.0, sc, fill)
            mx = jnp.max(sc, axis=1, keepdims=True)
            e = jnp.exp((sc - mx) * scale)
            l = jnp.sum(e, axis=1, keepdims=True)
            rc = pl.reciprocal(l, approx=True)
            rc = rc * (2.0 - l * rc)
            pr = (e * rc).astype(bf16)
            if not cfg['pstore']:
                return pr
            p_sc[p] = pltpu.bitcast(pr, u32)

        def pv(p, pr, mems):
            if cfg['pstore']:
                pr = _bf(p_sc[p])
            o = jnp.dot(pr, gather(1, p, mems[1]), preferred_element_type=f32)
            o_sc[p][m0:m0 + M, :] = jnp.concatenate([o[0:M], o[M:2 * M]], axis=1).astype(bf16)
            o_sc[p][x8:x8 + SEG, :] = jnp.concatenate(
                [o[2 * M:2 * M + SEG], o[2 * M + SEG:]], axis=1).astype(bf16)

        accs = [None] * 8
        odots = [(k, n) for k in range(0, H, cfg['och']) for n in range(8)]
        lcache = {}

        def oproj(cnt):
            r0, r1 = (0, 32) if par == 0 else (32, 80)
            for _ in range(min(cnt, len(odots))):
                k, n = odots.pop(0)
                ke = k + cfg['och']
                if k not in lcache:
                    lcache[k] = jnp.concatenate(
                        [o_sc[p][r0:r1, :] for p in range(k // 2, ke // 2)], axis=1)
                y = jnp.dot(lcache[k], _bf(wo_p[n, k * 64:ke * 64, :]),
                            preferred_element_type=f32)
                accs[n] = y if accs[n] is None else y + accs[n]
                unit(accs[n][:M])

        n1 = s + 7
        s1_u((n1 // 8) % 2, n1 // 8, n1 % 8)
        s1_h(sl1, j)
        s3(sl1, b3, slot3, j)

        if par == 0:
            lq = jnp.concatenate([mem, x_buf[pl.ds(rbase, 40), :]], axis=0)
        else:
            lq = jnp.concatenate([x_buf[pl.ds(rbase + 40, 24), :], mem], axis=0)
        for p in range(NPAIR):
            proj_q(p, lq)

        lhs = jnp.concatenate([mem, x_buf[pl.ds(x0, XR), :]], axis=0)
        mems, prs = {}, {}
        ag = cfg['agroup']
        for t in range(NPAIR + ag + 1):
            if t < NPAIR:
                mems[t] = [proj_kv(t, m, lhs) for m in range(2)]
            else:
                oproj(cfg['op_per'][par])
            if t % ag == 0:
                for p in range(t - 2 * ag, t - ag):
                    if 0 <= p < NPAIR:
                        pv(p, prs.pop(p), mems.pop(p))
                for p in range(t - ag, t):
                    if 0 <= p < NPAIR:
                        prs[p] = qk(p, mems[p])
        oproj(len(odots))
        out = jnp.concatenate(accs, axis=1).astype(bf16)
        if par == 0:
            outb[pl.ds(rbase, 24), :] = out[M:]
            return out[:M]
        outb[pl.ds(rbase + 24, 40), :] = out[:40]
        return out[40:]

    def outer(cb, carry):
        @pl.when(cb + 2 < NB)
        def _():
            for cp in kvh_copies(cb + 2):
                cp.start()

        q_copy(cb).start()

        @pl.when(cb >= 2)
        def _():
            outa_copy(cb - 2).start()

        @pl.when(cb >= 1)
        def _():
            outb_copy(cb - 1).start()
            q_copy(cb - 1).wait()

        @pl.when(cb == 1)
        def _():
            x_copy(1).wait()

        @pl.when(cb + 1 < NB)
        def _():
            for cp in kvh_copies(cb + 1):
                cp.wait()

        un = cfg['unroll']

        def inner(jj, c2):
            @pl.when(jnp.logical_and(cb == NB - 1, jj > 0))
            def _():
                for u in range(un // 2):
                    pr = (jj - 1) * (un // 2) + u
                    outa_piece(NB - 2, pl.multiple_of(pr * 4 * C, 4 * C), 4 * C).start()
                    outb_piece(pl.multiple_of(S - 256 + pr * 64, 64), 64).start()
            mem = mem_ref[...]
            for u in range(un):
                mem = step(cb, jj * un + u, mem, u % 2)
            mem_ref[...] = mem
            return c2
        with jax.named_scope('inner'):
            lax.fori_loop(0, 8 // un, inner, 0)
        return carry
    with jax.named_scope('main'):
        lax.fori_loop(0, NB, outer, 0)

    for pr in range(4 - cfg['unroll'] // 2, 4):
        outb_piece(S - 256 + 64 * pr, 64).start()
        outa_piece(NB - 2, pr * 4 * C, 4 * C).start()
    q_copy(NB - 1).wait()
    with jax.named_scope('epi'):
        for j in range(8):
            s3((NB - 1) % 2, NB - 1, NB - 1, j)
            if j % 2 == 1:
                outa_piece(NB - 1, (j - 1) * 2 * C, 4 * C).start()

    for b in range(NB - 2):
        outa_copy(b).wait()
    for n in range(NB - 1):
        outb_copy(n).wait()
    for j in range(4):
        outb_piece(S - 256 + 64 * j, 64).wait()
        outa_piece(NB - 2, j * 4 * C, 4 * C).wait()
        outa_piece(NB - 1, j * 4 * C, 4 * C).wait()


@functools.partial(jax.jit, static_argnames=("B_seg_len",))
def pallas_concat_heads__ssm_conv_h3__memory_aug_recurrent_mem_tr__prompt_kernel(
    A_q, A_k, A_v, A_shift_k, A_ssm_k, A_ssm_D, B_x, B_mem0, B_Wq, B_Wk, B_Wv, B_Wo,
    B_seg_len=SEG,
):
    assert B_seg_len == SEG
    assert A_q.shape == (1, S, D) and B_x.shape == (1, S, D)
    assert B_Wq.shape == (D, H, DH) and B_mem0.shape == (1, M, D)
    vm = pltpu.VMEM
    dma = pltpu.SemaphoreType.DMA
    scratch = [
        vm((D + 4, 16, DH), bf16), vm((D + 4, 16, DH), bf16),
        vm((D + 4, 16, DH), bf16),
        vm((2048 + 4, 16, 128), bf16),
        vm((8, H * DH // 2, 128), u32),
        vm((S, D), bf16),
        vm((M, D), bf16),
        vm((S, D), bf16),
        vm((NB + 1, 32, 128), f32),
        vm((2, S + 64, 128), bf16),
        vm((2, S, 128), bf16), vm((2, S, 128), bf16),
        vm((2, 128, S), bf16),
        vm((NB + 1, S, 128), bf16),
        vm((4 * NC + 1, 2 * C, 128), f32),
        vm((2, 8, 8, 32, 128), u32),
        vm((8, 32 + KPAD, 128), f32),
        vm((C, C), u32), vm((C // 2, 2 * C), u32),
        vm((PRE // 2, 256), u32),
        dma((41,)),
    ]
    scratch += [vm((16 * HS, 128), u32)] * 6
    scratch += [vm((RING, 8 * DH), bf16)] * 8
    scratch += [vm((L2, 2 * DH), bf16)] * (2 * NPAIR)
    scratch += [vm((NPAIR, L2 // 2, L2), u32)]
    scratch += [vm((L2, L2), f32), vm((KS, D), bf16), vm((NB, 128), bf16)]

    out = pl.pallas_call(
        _kernel,
        out_shape=jax.ShapeDtypeStruct((S, 2 * D), bf16),
        in_specs=[pl.BlockSpec(memory_space=pl.ANY)] * 12,
        out_specs=pl.BlockSpec(memory_space=pl.ANY),
        scratch_shapes=scratch,
        compiler_params=pltpu.CompilerParams(vmem_limit_bytes=120 * 1024 * 1024,
                                             disable_bounds_checks=True,
                                             disable_semaphore_checks=True),
        name="ssm_memtr",
    )(A_q.reshape(S, D), A_k.reshape(S, D), A_v.reshape(S, D), A_shift_k.T, A_ssm_k,
      A_ssm_D.reshape(NB, 128), B_x.reshape(S, D), B_mem0.reshape(M, D),
      B_Wq, B_Wk, B_Wv, B_Wo.reshape(H * DH // 16, 16, D))
    return out.reshape(1, S, 2 * D)
```

```python
import functools
import math

import jax
import jax.numpy as jnp
from jax import lax
import jax.experimental.pallas as pl
import jax.experimental.pallas.tpu as pltpu

bf16, f32, u32, i32 = jnp.bfloat16, jnp.float32, jnp.uint32, jnp.int32

S = 2048
D = 1024
H, DH = 32, 128
M, SEG = 8, 32
NSEG = S // SEG
KS = 4

XR = 24
PRE = S - NSEG * XR
RING = 576
QOFF = 64
HS = 514
NPAIR = H // 2
L2 = 2 * (M + SEG)

C = 128
NC = S // C
NB = D // 128
KPAD = 16

CFG = dict(
    agroup=2, pstore=True, och=8, op_per=[4, 3],
    s2_at=[list(range(0, 32)), list(range(62, 94))],
    s0_at=[list(range(0, 4)) + list(range(16, 20)), list(range(62, 66)) + list(range(78, 82))],
    nopro=False, unroll=4,
)


def _bf(x):
    return pltpu.bitcast(x, bf16)


def _kernel(q_hbm, k_hbm, v_hbm, skt_hbm, h_hbm, dd_hbm, x_hbm, mem0_hbm,
            wq_hbm, wk_hbm, wv_hbm, wo_hbm, out_hbm,
            st0, st1, st2, wo_st, wo_p, x_buf, mem_ref, outb,
            coef, k_buf, v_buf, q_buf, h_buf, kvo,
            uh, y_buf, kf, f_p, g_p, xp, sems,
            *bufs):
    wp = bufs[0:6]
    ring = bufs[6:14]
    o_sc = bufs[14:30]
    q_sc = bufs[30:46]
    p_sc, fill_ref, skt_buf, dd_buf = bufs[46:50]
    stage = (st0, st1, st2)
    w_hbm = (wk_hbm, wv_hbm, wq_hbm)
    scale = DH ** -0.5
    cfg = CFG
    SW, SWO, SX, SSM, SK, SV, SH, SQ, SOUT = 0, 12, 20, 26, 29, 31, 33, 35, 37

    def w_copy(g, c):
        r0 = c * 256
        return pltpu.make_async_copy(
            w_hbm[g // 2].at[pl.ds(r0, 256), pl.ds(16 * (g % 2), 16), :],
            stage[g % 3].at[pl.ds(r0, 256)],
            sems.at[SW + (g % 3) * 4 + c])

    def wo_copy(n):
        return pltpu.make_async_copy(
            wo_hbm.at[:, :, pl.ds(pl.multiple_of(n * 128, 128), 128)],
            wo_st.at[pl.ds(n * 256, 256)], sems.at[SWO + n])

    def xc_copy(c):
        cols = pl.ds(pl.multiple_of(c * 256, 256), 256)
        return pltpu.make_async_copy(x_hbm.at[pl.ds(0, PRE), cols],
                                     x_buf.at[pl.ds(0, PRE), cols], sems.at[SX + c])

    def x_copy(part):
        r0, n = ((PRE, 256), (PRE + 256, S - PRE - 256))[part]
        return pltpu.make_async_copy(
            x_hbm.at[pl.ds(r0, n)], x_buf.at[pl.ds(r0, n)], sems.at[SX + 4 + part])

    def small_copies():
        return [pltpu.make_async_copy(skt_hbm, skt_buf, sems.at[SSM + 0]),
                pltpu.make_async_copy(dd_hbm, dd_buf, sems.at[SSM + 1]),
                pltpu.make_async_copy(mem0_hbm, mem_ref, sems.at[SSM + 2])]

    def col(b):
        return pl.ds(pl.multiple_of(b * 128, 128), 128)

    def kvh_copies(b):
        sl = b % 2
        return [pltpu.make_async_copy(k_hbm.at[:, col(b)],
                                      k_buf.at[sl, pl.ds(KPAD, S)], sems.at[SK + sl]),
                pltpu.make_async_copy(v_hbm.at[:, col(b)], v_buf.at[sl], sems.at[SV + sl]),
                pltpu.make_async_copy(h_hbm.at[col(b)], h_buf.at[sl], sems.at[SH + sl])]

    def q_copy(b):
        sl = b % 2
        return pltpu.make_async_copy(q_hbm.at[:, col(b)], q_buf.at[sl], sems.at[SQ + sl])

    def outa_copy(b):
        return pltpu.make_async_copy(kvo.at[b], out_hbm.at[:, col(b)], sems.at[SOUT + 0])

    def outa_piece(b, r0, n):
        return pltpu.make_async_copy(kvo.at[b, pl.ds(r0, n)],
                                     out_hbm.at[pl.ds(r0, n), col(b)], sems.at[SOUT + 1])

    def outb_piece(r0, n):
        return pltpu.make_async_copy(outb.at[pl.ds(r0, n)],
                                     out_hbm.at[pl.ds(r0, n), pl.ds(D, D)], sems.at[SOUT + 3])

    def outb_copy(cb):
        rows = pl.ds(pl.multiple_of(cb * 8 * SEG, 8 * SEG), 8 * SEG)
        return pltpu.make_async_copy(outb.at[rows], out_hbm.at[rows, pl.ds(D, D)],
                                     sems.at[SOUT + 2])

    def relayout(g, c, lo_i=0, hi_i=128):
        src, dst = stage[g % 3], wp[g]
        d0 = c * 256
        for i in range(lo_i, hi_i):
            a = pltpu.bitcast(src[d0 + 2 * i], u32)
            b = pltpu.bitcast(src[d0 + 2 * i + 1], u32)
            lo = (a & jnp.uint32(0xFFFF)) | (b << 16)
            hi = (a >> 16) | (b & jnp.uint32(0xFFFF0000))
            row = c * 128 + i
            dst[pl.ds(row, 8, stride=2 * HS), :] = lo
            dst[pl.ds(row + HS, 8, stride=2 * HS), :] = hi

    def wo_pack(n, r0=0, r1=256):
        for r in range(r0, r1, 8):
            blk = pltpu.bitcast(wo_st[pl.ds(n * 256 + r, 8)], u32)
            wo_p[n, r * 8:(r + 8) * 8, :] = blk.reshape(64, 128)

    def wt(m, h):
        g, hh = 2 * m + h // 16, h % 16
        return _bf(wp[g][hh * HS:hh * HS + D // 2, :])

    def ring_cols(m, p):
        c0 = 512 * m + 256 * (p % 2)
        return slice(c0, c0 + 256)

    def s0_kv(sl, b, slot, j, i):
        t0 = pl.multiple_of(j * 2 * C, 2 * C)
        kw = k_buf.at[sl, pl.ds(t0, 2 * C + KPAD)]
        vw = v_buf.at[sl, pl.ds(t0, 2 * C)]
        ow = kvo.at[slot, pl.ds(t0, 2 * C)]
        kf[i] = kw[32 * i:32 * i + 32 + KPAD, :].astype(f32)
        acc = None
        for tap in range(KS):
            term = kf[i, KPAD - tap:KPAD - tap + 32, :] * coef[b, tap:tap + 1, :]
            acc = term if acc is None else acc + term
        ow[32 * i:32 * i + 32, :] = (acc * vw[32 * i:32 * i + 32, :].astype(f32)).astype(bf16)

    def s1_h(sl, j):
        for t in range(2):
            a = 2 * j + t
            hh = h_buf[sl, :, pl.ds(pl.multiple_of(a * C, C), C)]
            for half in range(2):
                fm = _bf(f_p[half * 64:(half + 1) * 64, :])
                uh[sl * 2 * NC + NC + a, half * C:(half + 1) * C, :] = lax.dot_general(
                    fm, hh, (((1,), (1,)), ((), ())), preferred_element_type=f32)

    def s1_u(sl, slot, j):
        for t in range(2):
            a = 2 * j + t
            kv = kvo[slot, pl.ds(pl.multiple_of(a * C, C), C), :]
            for half in range(2):
                fm = _bf(f_p[half * 64:(half + 1) * 64, :])
                uh[sl * 2 * NC + a, half * C:(half + 1) * C, :] = jnp.dot(
                    fm, kv, preferred_element_type=f32)

    def s2_parts(sl, j):
        u0 = sl * 2 * NC
        h0 = u0 + NC
        r0 = pl.multiple_of(j * 32, 32)
        prev = []

        def one(idx, pace):
            grp, a = divmod(idx, NC)
            re, im = pl.ds(r0 + 16 * grp, 8), pl.ds(r0 + 16 * grp + 8, 8)
            yr = yi = None
            for b in range(a + 1):
                if b == a:
                    uh[4 * NC, 0:8, :] = pace
                ur, ui = uh[u0 + b, re, :], uh[u0 + b, im, :]
                hr, hi = uh[h0 + a - b, re, :], uh[h0 + a - b, im, :]
                yr = ur * hr if yr is None else yr + ur * hr
                yi = ur * hi if yi is None else yi + ur * hi
                yr = yr - ui * hi
                yi = yi + ui * hr
            pp, qq = yr - yi, yr + yi
            if a > 0:
                zp, zq = pp - prev[1], qq + prev[0]
            else:
                zp, zq = pp, qq
            prev[:] = [pp, qq]
            z = pltpu.bitcast(jnp.concatenate([zp, zq], axis=0).astype(bf16), u32)
            r = (a % 2) * 16 + 4 * grp
            y_buf[sl, j, a // 2, r:r + 4, :] = z[0:4]
            y_buf[sl, j, a // 2, r + 8:r + 12, :] = z[4:8]
        return one

    def s3(sl, b, slot, j):
        rev = 7 - lax.broadcasted_iota(i32, (8, 128), 0)
        for t in range(2):
            a = 2 * j + t
            rows = pl.ds(pl.multiple_of(a * C, C), C)
            eo = []
            for part in range(2):
                r = 16 * t + 8 * part
                yp = y_buf[sl, :, j, r:r + 8, :].reshape(C // 2, 128)
                eo.append(jnp.dot(_bf(g_p[part * 32:(part + 1) * 32, :]), _bf(yp),
                                  preferred_element_type=f32))
            lo, hi = eo[0] + eo[1], eo[0] - eo[1]
            hi = [jnp.take_along_axis(hi[8 * i:8 * i + 8], rev, axis=0) for i in range(7, -1, -1)]
            y = jnp.concatenate([lo] + hi, axis=0)
            y = y + kvo[slot, rows, :].astype(f32) * coef[b, KS:KS + 1, :]
            kvo[slot, rows, :] = (q_buf[sl, rows, :].astype(f32) * y).astype(bf16)

    for cp in small_copies():
        cp.start()
    for c in range(4):
        xc_copy(c).start()
        w_copy(0, c).start()
        if c > 0:
            w_copy(1, c - 1).start()

    r = lax.broadcasted_iota(i32, (L2, L2), 0)
    c_ = lax.broadcasted_iota(i32, (L2, L2), 1)
    head = lambda i: jnp.where(i < 2 * M, i // M, (i - 2 * M) // SEG)
    ok = (r < 2 * M) | (c_ < 2 * M) | (c_ <= r)
    fill_ref[...] = jnp.where(head(r) == head(c_),
                              jnp.where(ok, 0.0, -1e9 / scale), -jnp.inf).astype(f32)

    rr = lax.broadcasted_iota(i32, (2 * C, C), 0)
    nn = lax.broadcasted_iota(i32, (2 * C, C), 1)
    kk = 8 * (rr // 16) + rr % 8
    mm = (2 * kk + 1) * (4 * nn + 1) + 4 * C * ((rr // 8) % 2) * (1 + 2 * (kk % 2))
    fm = jnp.cos((mm % (16 * C)).astype(f32) * (math.pi / (8 * C)))
    f_p[...] = pltpu.bitcast(fm.astype(bf16), u32)
    rr = lax.broadcasted_iota(i32, (C, C), 0)
    kk = lax.broadcasted_iota(i32, (C, C), 1)
    mm = (2 * kk + 1) * (2 * (rr % (C // 2)) + 1) + C * (7 - 6 * ((kk + rr // (C // 2)) % 2))
    gm = jnp.cos((mm % (8 * C)).astype(f32) * (math.pi / (4 * C))) * (2 ** -0.5 / C)
    g_p[...] = pltpu.bitcast(gm.astype(bf16), u32)
    for sl in range(2):
        k_buf[sl, 0:KPAD, :] = jnp.zeros((KPAD, 128), bf16)
    uh[0:32] = jnp.zeros((32, 2 * C, 128), f32)

    for cp in small_copies():
        cp.wait()
    skt = skt_buf[...].astype(f32)
    ddv = dd_buf[...].astype(f32)
    for b in range(NB):
        coef[b, 0:KS, :] = skt[:, b * 128:(b + 1) * 128]
        coef[b, KS:KS + 1, :] = ddv[b:b + 1, :]

    def pro_body(g, i, tasks):
        r0 = pl.multiple_of(i * 128, 128)
        x = x_buf[pl.ds(r0, 128), :]
        for p in range(8):
            ys = []
            for t in range(2):
                y = jnp.dot(x, wt(g // 2, 16 * (g % 2) + 2 * p + t),
                            preferred_element_type=f32)
                ys.append(y)
                for fn in tasks.get(2 * p + t, ()):
                    fn(y)
            pp = 8 * (g % 2) + p
            ring[pp // 2][pl.ds(pl.multiple_of(QOFF + r0, 64), 128),
                          ring_cols(g // 2, pp)] = jnp.concatenate(ys, axis=1).astype(bf16)

    def add_relayout(tasks, g, c, r):
        for u in range(15):
            def fn(y, u=u):
                stage[g % 3][D] = y[r:r + 16].astype(bf16)
                relayout(g, c, (128 * u) // 15, (128 * (u + 1)) // 15)
            tasks.setdefault(u, []).append(fn)

    def add_wo(tasks, n0):
        for u in range(15):
            def fn(y, u=u):
                wo_st[2048] = y[96:112].astype(bf16)
                for r in range((64 * u) // 15, (64 * (u + 1)) // 15):
                    wo_pack(n0 + r // 32, 8 * (r % 32), 8 * (r % 32) + 8)
            tasks.setdefault(u, []).append(fn)

    def add_s01(tasks, j):
        for k in range(8):
            def fn(y, k=k):
                coef[NB, 0:8, :] = y[48:56]
                s0_kv(0, 0, 0, j, k)
            tasks.setdefault(k, []).append(fn)
        tasks.setdefault(3, []).append(lambda y: s1_h(0, j))
        tasks.setdefault(11, []).append(lambda y: s1_u(0, 0, j))

    def period(g, body):
        if cfg['nopro']:
            return
        with jax.named_scope('pro%d' % g):
            lax.fori_loop(0, 4, lambda i, c: (body(i), c)[1], 0)

    def p0(c):
        @pl.when(c == 1)
        def _():
            w_copy(1, 3).start()
            for i in range(4):
                w_copy(2, i).start()

        @pl.when(c > 0)
        def _():
            w_copy(1, c - 1).wait()
        xc_copy(c).wait()
        w_copy(0, c).wait()
        relayout(0, c)
        xp[...] = pltpu.bitcast(
            x_buf[0:PRE, pl.ds(pl.multiple_of(c * 256, 256), 256)], u32)
        tasks = {}
        add_relayout(tasks, 1, (c + 3) % 4, 0)
        k0 = pl.multiple_of(c * 128, 128)
        for p in range(8):
            ys = []
            for t in range(2):
                hh = 2 * p + t
                w = _bf(wp[0][pl.ds(k0 + hh * HS, 128), :])
                y = (jnp.dot(_bf(xp[...]), w, preferred_element_type=f32)
                     + uh[2 * hh:2 * hh + 2].reshape(PRE, 128))
                uh[2 * hh:2 * hh + 2] = y.reshape(2, 2 * C, 128)
                ys.append(y)
                for fn in tasks.get(hh, ()):
                    fn(y[256 * t:])
            ring[p // 2][QOFF:QOFF + PRE, ring_cols(0, p)] = (
                jnp.concatenate(ys, axis=1).astype(bf16))
    period(0, p0)
    w_copy(1, 3).wait()
    relayout(1, 3)

    def p1(i):
        @pl.when(i == 0)
        def _():
            w_copy(3, 0).start()
            w_copy(3, 1).start()
            for cp in kvh_copies(0):
                cp.start()
            w_copy(4, 0).start()
            w_copy(4, 1).start()
            for c in range(2, 4):
                w_copy(3, c).start()
                w_copy(4, c).start()
        w_copy(2, i).wait()
        tasks = {}
        add_relayout(tasks, 2, i, 0)
        pro_body(1, i, tasks)
    period(1, p1)

    def p2(i):
        @pl.when(i == 0)
        def _():
            for c in range(4):
                w_copy(5, c).start()
                wo_copy(2 * c).start()
                wo_copy(2 * c + 1).start()
            x_copy(0).start()
            for cp in kvh_copies(1):
                cp.start()
            x_copy(1).start()
            for cp in kvh_copies(0):
                cp.wait()
        w_copy(3, i).wait()
        w_copy(4, i).wait()
        tasks = {}
        add_relayout(tasks, 3, i, 0)
        add_relayout(tasks, 4, i, 96)
        add_s01(tasks, i)
        pro_body(2, i, tasks)
    period(2, p2)

    def p3(i):
        w_copy(5, i).wait()
        wo_copy(2 * i).wait()
        wo_copy(2 * i + 1).wait()
        tasks = {}
        add_relayout(tasks, 5, i, 0)
        add_wo(tasks, 2 * i)
        add_s01(tasks, 4 + i)
        pro_body(3, i, tasks)
    period(3, p3)
    x_copy(0).wait()

    def step(cb, j, mem, par):
        s = cb * 8 + j
        x0 = pl.multiple_of(PRE + XR * s, 8)
        wpos = pl.multiple_of(lax.rem(s, RING // XR) * XR, 8)
        rpos = pl.multiple_of(lax.rem(s + QOFF // SEG, RING // SEG) * SEG, 32)
        rbase = pl.multiple_of((s - par) * SEG, 64)
        m0 = 0 if par == 0 else 72
        x8 = 8 + SEG * par

        sl1 = (cb + 1) % 2
        b1 = jnp.minimum(cb + 1, NB - 1)
        slot1 = cb + 1
        b3 = jnp.maximum(cb - 1, 0)
        slot3 = jnp.where(cb == 0, NB, cb - 1)
        s2 = s2_parts(cb % 2, j)
        nu = [0]

        def unit(pace):
            u = nu[0]
            nu[0] += 1
            if u in cfg['s0_at'][par]:
                coef[NB, 0:8, :] = pace
                s0_kv(sl1, b1, slot1, j, cfg['s0_at'][par].index(u))
            if u in cfg['s2_at'][par]:
                s2(cfg['s2_at'][par].index(u), pace)

        def proj_q(p, lq):
            ys = []
            for t in range(2):
                ys.append(jnp.dot(lq, wt(2, 2 * p + t), preferred_element_type=f32))
                unit(ys[-1][:M])
            r0, r1 = (0, 48) if par == 0 else (48, 80)
            q_sc[p][r0:r1, :] = jnp.concatenate(ys, axis=1).astype(bf16)

        def proj_kv(p, m, lhs):
            ys = [jnp.dot(lhs, wt(m, 2 * p + t), preferred_element_type=f32)
                  for t in range(2)]
            ring[p // 2][pl.ds(wpos, XR), ring_cols(m, p)] = jnp.concatenate(
                [y[M:] for y in ys], axis=1).astype(bf16)
            unit(ys[0][:M])
            return jnp.concatenate([y[:M] for y in ys], axis=0).astype(bf16)

        def gather(m, p, mm):
            xx = ring[p // 2][pl.ds(rpos, SEG), ring_cols(m, p)]
            return jnp.concatenate([mm, xx[:, :DH], xx[:, DH:]], axis=0)

        def qk(p, mems):
            b = q_sc[p]
            q2 = jnp.concatenate([b[m0:m0 + M, :DH], b[m0:m0 + M, DH:],
                                  b[x8:x8 + SEG, :DH], b[x8:x8 + SEG, DH:]], axis=0)
            sc = lax.dot_general(q2, gather(0, p, mems[0]), (((1,), (1,)), ((), ())),
                                 preferred_element_type=f32)
            fill = fill_ref[...]
            sc = jnp.where(fill == 0.0, sc, fill)
            mx = jnp.max(sc, axis=1, keepdims=True)
            e = jnp.exp((sc - mx) * scale)
            l = jnp.sum(e, axis=1, keepdims=True)
            rc = pl.reciprocal(l, approx=True)
            rc = rc * (2.0 - l * rc)
            pr = (e * rc).astype(bf16)
            if not cfg['pstore']:
                return pr
            p_sc[p] = pltpu.bitcast(pr, u32)

        def pv(p, pr, mems):
            if cfg['pstore']:
                pr = _bf(p_sc[p])
            o = jnp.dot(pr, gather(1, p, mems[1]), preferred_element_type=f32)
            o_sc[p][m0:m0 + M, :] = jnp.concatenate([o[0:M], o[M:2 * M]], axis=1).astype(bf16)
            o_sc[p][x8:x8 + SEG, :] = jnp.concatenate(
                [o[2 * M:2 * M + SEG], o[2 * M + SEG:]], axis=1).astype(bf16)

        accs = [None] * 8
        odots = [(k, n) for k in range(0, H, cfg['och']) for n in range(8)]
        lcache = {}

        def oproj(cnt):
            r0, r1 = (0, 32) if par == 0 else (32, 80)
            for _ in range(min(cnt, len(odots))):
                k, n = odots.pop(0)
                ke = k + cfg['och']
                if k not in lcache:
                    lcache[k] = jnp.concatenate(
                        [o_sc[p][r0:r1, :] for p in range(k // 2, ke // 2)], axis=1)
                y = jnp.dot(lcache[k], _bf(wo_p[n, k * 64:ke * 64, :]),
                            preferred_element_type=f32)
                accs[n] = y if accs[n] is None else y + accs[n]
                unit(accs[n][:M])

        n1 = s + 7
        s1_u((n1 // 8) % 2, n1 // 8, n1 % 8)
        s1_h(sl1, j)
        s3(sl1, b3, slot3, j)

        if par == 0:
            lq = jnp.concatenate([mem, x_buf[pl.ds(rbase, 40), :]], axis=0)
        else:
            lq = jnp.concatenate([x_buf[pl.ds(rbase + 40, 24), :], mem], axis=0)
        for p in range(NPAIR):
            proj_q(p, lq)

        lhs = jnp.concatenate([mem, x_buf[pl.ds(x0, XR), :]], axis=0)
        mems, prs = {}, {}
        ag = cfg['agroup']
        for t in range(NPAIR + ag + 1):
            if t < NPAIR:
                mems[t] = [proj_kv(t, m, lhs) for m in range(2)]
            else:
                oproj(cfg['op_per'][par])
            if t % ag == 0:
                for p in range(t - 2 * ag, t - ag):
                    if 0 <= p < NPAIR:
                        pv(p, prs.pop(p), mems.pop(p))
                for p in range(t - ag, t):
                    if 0 <= p < NPAIR:
                        prs[p] = qk(p, mems[p])
        oproj(len(odots))
        out = jnp.concatenate(accs, axis=1).astype(bf16)
        if par == 0:
            outb[pl.ds(rbase, 24), :] = out[M:]
            return out[:M]
        outb[pl.ds(rbase + 24, 40), :] = out[:40]
        return out[40:]

    def outer(cb, carry):
        @pl.when(cb + 2 < NB)
        def _():
            for cp in kvh_copies(cb + 2):
                cp.start()

        q_copy(cb).start()

        @pl.when(cb >= 2)
        def _():
            outa_copy(cb - 2).start()

        @pl.when(cb >= 1)
        def _():
            outb_copy(cb - 1).start()
            q_copy(cb - 1).wait()

        @pl.when(cb == 1)
        def _():
            x_copy(1).wait()

        @pl.when(cb + 1 < NB)
        def _():
            for cp in kvh_copies(cb + 1):
                cp.wait()

        un = cfg['unroll']

        def inner(jj, c2):
            @pl.when(jnp.logical_and(cb == NB - 1, jj > 0))
            def _():
                for u in range(un // 2):
                    pr = (jj - 1) * (un // 2) + u
                    outa_piece(NB - 2, pl.multiple_of(pr * 4 * C, 4 * C), 4 * C).start()
                    outb_piece(pl.multiple_of(S - 256 + pr * 64, 64), 64).start()
            mem = mem_ref[...]
            for u in range(un):
                mem = step(cb, jj * un + u, mem, u % 2)
            mem_ref[...] = mem
            return c2
        with jax.named_scope('inner'):
            lax.fori_loop(0, 8 // un, inner, 0)
        return carry
    with jax.named_scope('main'):
        lax.fori_loop(0, NB, outer, 0)

    for pr in range(4 - cfg['unroll'] // 2, 4):
        outb_piece(S - 256 + 64 * pr, 64).start()
        outa_piece(NB - 2, pr * 4 * C, 4 * C).start()
    q_copy(NB - 1).wait()
    with jax.named_scope('epi'):
        for j in range(8):
            s3((NB - 1) % 2, NB - 1, NB - 1, j)
            if j % 2 == 1:
                outa_piece(NB - 1, (j - 1) * 2 * C, 4 * C).start()

    for b in range(NB - 2):
        outa_copy(b).wait()
    for n in range(NB - 1):
        outb_copy(n).wait()
    for j in range(4):
        outb_piece(S - 256 + 64 * j, 64).wait()
        outa_piece(NB - 2, j * 4 * C, 4 * C).wait()
        outa_piece(NB - 1, j * 4 * C, 4 * C).wait()


@functools.partial(jax.jit, static_argnames=("B_seg_len",))
def pallas_concat_heads__ssm_conv_h3__memory_aug_recurrent_mem_tr__prompt_kernel(
    A_q, A_k, A_v, A_shift_k, A_ssm_k, A_ssm_D, B_x, B_mem0, B_Wq, B_Wk, B_Wv, B_Wo,
    B_seg_len=SEG,
):
    assert B_seg_len == SEG
    assert A_q.shape == (1, S, D) and B_x.shape == (1, S, D)
    assert B_Wq.shape == (D, H, DH) and B_mem0.shape == (1, M, D)
    vm = pltpu.VMEM
    dma = pltpu.SemaphoreType.DMA
    scratch = [
        vm((D + 4, 16, DH), bf16), vm((D + 4, 16, DH), bf16),
        vm((D + 4, 16, DH), bf16),
        vm((2048 + 4, 16, 128), bf16),
        vm((8, H * DH // 2, 128), u32),
        vm((S, D), bf16),
        vm((M, D), bf16),
        vm((S, D), bf16),
        vm((NB + 1, 32, 128), f32),
        vm((2, S + 64, 128), bf16),
        vm((2, S, 128), bf16), vm((2, S, 128), bf16),
        vm((2, 128, S), bf16),
        vm((NB + 1, S, 128), bf16),
        vm((4 * NC + 1, 2 * C, 128), f32),
        vm((2, 8, 8, 32, 128), u32),
        vm((8, 32 + KPAD, 128), f32),
        vm((C, C), u32), vm((C // 2, C), u32),
        vm((PRE // 2, 256), u32),
        dma((41,)),
    ]
    scratch += [vm((16 * HS, 128), u32)] * 6
    scratch += [vm((RING, 8 * DH), bf16)] * 8
    scratch += [vm((L2, 2 * DH), bf16)] * (2 * NPAIR)
    scratch += [vm((NPAIR, L2 // 2, L2), u32)]
    scratch += [vm((L2, L2), f32), vm((KS, D), bf16), vm((NB, 128), bf16)]

    out = pl.pallas_call(
        _kernel,
        out_shape=jax.ShapeDtypeStruct((S, 2 * D), bf16),
        in_specs=[pl.BlockSpec(memory_space=pl.ANY)] * 12,
        out_specs=pl.BlockSpec(memory_space=pl.ANY),
        scratch_shapes=scratch,
        compiler_params=pltpu.CompilerParams(vmem_limit_bytes=120 * 1024 * 1024,
                                             disable_bounds_checks=True,
                                             disable_semaphore_checks=True),
        name="ssm_memtr",
    )(A_q.reshape(S, D), A_k.reshape(S, D), A_v.reshape(S, D), A_shift_k.T, A_ssm_k,
      A_ssm_D.reshape(NB, 128), B_x.reshape(S, D), B_mem0.reshape(M, D),
      B_Wq, B_Wk, B_Wv, B_Wo.reshape(H * DH // 16, 16, D))
    return out.reshape(1, S, 2 * D)
```

```python
import functools
import math

import jax
import jax.numpy as jnp
from jax import lax
import jax.experimental.pallas as pl
import jax.experimental.pallas.tpu as pltpu

bf16, f32, u32, i32 = jnp.bfloat16, jnp.float32, jnp.uint32, jnp.int32

S = 2048
D = 1024
H, DH = 32, 128
M, SEG = 8, 32
NSEG = S // SEG
KS = 4

XR = 24
PRE = S - NSEG * XR
RING = 576
QOFF = 64
HS = 514
NPAIR = H // 2
L2 = 2 * (M + SEG)

C = 128
NC = S // C
NB = D // 128
KPAD = 16

CFG = dict(
    agroup=2, pstore=True, och=8, op_per=[4, 3],
    s2_at=[list(range(0, 32)), list(range(62, 94))],
    s0_at=[list(range(0, 4)) + list(range(16, 20)), list(range(62, 66)) + list(range(78, 82))],
    nopro=False,
)


def _bf(x):
    return pltpu.bitcast(x, bf16)


def _kernel(q_hbm, k_hbm, v_hbm, skt_hbm, h_hbm, dd_hbm, x_hbm, mem0_hbm,
            wq_hbm, wk_hbm, wv_hbm, wo_hbm, out_hbm,
            st0, st1, st2, wo_st, wo_p, x_buf, mem_ref, outb,
            coef, k_buf, v_buf, q_buf, h_buf, kvo,
            uh, y_buf, kf, f_p, g_p, xp, sems, zero,
            *bufs):
    wp = bufs[0:6]
    ring = bufs[6:14]
    o_sc = bufs[14:30]
    q_sc = bufs[30:46]
    p_sc, fill_ref, skt_buf, dd_buf = bufs[46:50]
    stage = (st0, st1, st2)
    w_hbm = (wk_hbm, wv_hbm, wq_hbm)
    scale = DH ** -0.5
    cfg = CFG
    SW, SWO, SX, SSM, SKVH, SQ, SOUT = 0, 12, 20, 26, 29, 33, 37

    def w_copy(g, c):
        r0 = c * 256
        return pltpu.make_async_copy(
            w_hbm[g // 2].at[pl.ds(r0, 256), pl.ds(16 * (g % 2), 16), :],
            stage[g % 3].at[pl.ds(r0, 256)],
            sems.at[SW + (g % 3) * 4 + c])

    def wo_copy(n):
        return pltpu.make_async_copy(
            wo_hbm.at[:, :, pl.ds(pl.multiple_of(n * 128, 128), 128)],
            wo_st.at[pl.ds(n * 256, 256)], sems.at[SWO + n])

    def xc_copy(c):
        cols = pl.ds(pl.multiple_of(c * 256, 256), 256)
        return pltpu.make_async_copy(x_hbm.at[pl.ds(0, PRE), cols],
                                     x_buf.at[pl.ds(0, PRE), cols], sems.at[SX + c])

    def x_copy(part):
        r0, n = ((PRE, 128), (PRE + 128, S - PRE - 128))[part]
        return pltpu.make_async_copy(
            x_hbm.at[pl.ds(r0, n)], x_buf.at[pl.ds(r0, n)], sems.at[SX + 4 + part])

    def small_copies():
        return [pltpu.make_async_copy(skt_hbm, skt_buf, sems.at[SSM + 0]),
                pltpu.make_async_copy(dd_hbm, dd_buf, sems.at[SSM + 1]),
                pltpu.make_async_copy(mem0_hbm, mem_ref, sems.at[SSM + 2])]

    def col(b):
        return pl.ds(pl.multiple_of(b * 128, 128), 128)

    HALF = S // 2

    def half_rows(half, off=0):
        return pl.ds(pl.multiple_of(half * HALF, HALF) + off, HALF)

    def kvh_copies(b, half):
        sl, t = b & 1, half_rows(half)
        sem = sems.at[SKVH + 2 * sl + half]
        return [pltpu.make_async_copy(k_hbm.at[t, col(b)],
                                      k_buf.at[sl, half_rows(half, KPAD)], sem),
                pltpu.make_async_copy(v_hbm.at[t, col(b)], v_buf.at[sl, t], sem),
                pltpu.make_async_copy(h_hbm.at[col(b), t], h_buf.at[sl, :, t], sem)]

    def q_copy(b, half):
        sl, t = b & 1, half_rows(half)
        return pltpu.make_async_copy(q_hbm.at[t, col(b)], q_buf.at[sl, t],
                                     sems.at[SQ + 2 * sl + half])

    def outa_copy(b, half):
        t = half_rows(half)
        return pltpu.make_async_copy(kvo.at[b, t], out_hbm.at[t, col(b)], sems.at[SOUT])

    def outa_piece(b, r0, n):
        return pltpu.make_async_copy(kvo.at[b, pl.ds(r0, n)],
                                     out_hbm.at[pl.ds(r0, n), col(b)], sems.at[SOUT + 1])

    def outb_copy(it):
        rows = pl.ds(pl.multiple_of(it * 4 * SEG, 4 * SEG), 4 * SEG)
        return pltpu.make_async_copy(outb.at[rows], out_hbm.at[rows, pl.ds(D, D)],
                                     sems.at[SOUT + 2])

    def relayout(g, c, lo_i=0, hi_i=128):
        src, dst = stage[g % 3], wp[g]
        d0 = c * 256
        for i in range(lo_i, hi_i):
            a = pltpu.bitcast(src[d0 + 2 * i], u32)
            b = pltpu.bitcast(src[d0 + 2 * i + 1], u32)
            lo = (a & jnp.uint32(0xFFFF)) | (b << 16)
            hi = (a >> 16) | (b & jnp.uint32(0xFFFF0000))
            row = c * 128 + i
            dst[pl.ds(row, 8, stride=2 * HS), :] = lo
            dst[pl.ds(row + HS, 8, stride=2 * HS), :] = hi

    def wo_pack(n, r0=0, r1=256):
        for r in range(r0, r1, 8):
            blk = pltpu.bitcast(wo_st[pl.ds(n * 256 + r, 8)], u32)
            wo_p[n, r * 8:(r + 8) * 8, :] = blk.reshape(64, 128)

    def wt(m, h):
        g, hh = 2 * m + h // 16, h % 16
        return _bf(wp[g][hh * HS:hh * HS + D // 2, :])

    def ring_cols(m, p):
        c0 = 512 * m + 256 * (p % 2)
        return slice(c0, c0 + 256)

    def s0_kv(sl, b, slot, j, i):
        t0 = pl.multiple_of(j * 2 * C, 2 * C)
        kw = k_buf.at[sl, pl.ds(t0, 2 * C + KPAD)]
        vw = v_buf.at[sl, pl.ds(t0, 2 * C)]
        ow = kvo.at[slot, pl.ds(t0, 2 * C)]
        kf[i] = kw[32 * i:32 * i + 32 + KPAD, :].astype(f32)
        acc = None
        for tap in range(KS):
            term = kf[i, KPAD - tap:KPAD - tap + 32, :] * coef[b, tap:tap + 1, :]
            acc = term if acc is None else acc + term
        ow[32 * i:32 * i + 32, :] = (acc * vw[32 * i:32 * i + 32, :].astype(f32)).astype(bf16)

    def s1_h(sl, j):
        for t in range(2):
            a = 2 * j + t
            hh = h_buf[sl, :, pl.ds(pl.multiple_of(a * C, C), C)]
            for half in range(2):
                fm = _bf(f_p[half * 64:(half + 1) * 64, :])
                uh[sl * 2 * NC + NC + a, half * C:(half + 1) * C, :] = lax.dot_general(
                    fm, hh, (((1,), (1,)), ((), ())), preferred_element_type=f32)

    def s1_u(sl, slot, j):
        for t in range(2):
            a = 2 * j + t
            kv = kvo[slot, pl.ds(pl.multiple_of(a * C, C), C), :]
            for half in range(2):
                fm = _bf(f_p[half * 64:(half + 1) * 64, :])
                uh[sl * 2 * NC + a, half * C:(half + 1) * C, :] = jnp.dot(
                    fm, kv, preferred_element_type=f32)

    def s2_parts(sl, j):
        u0 = sl * 2 * NC
        h0 = u0 + NC
        r0 = pl.multiple_of(j * 32, 32)
        prev = []

        def one(idx, pace):
            grp, a = divmod(idx, NC)
            re, im = pl.ds(r0 + 16 * grp, 8), pl.ds(r0 + 16 * grp + 8, 8)
            yr = yi = None
            for b in range(a + 1):
                if b == a:
                    uh[4 * NC + zero[0], 0:8, :] = pace
                ur, ui = uh[u0 + b, re, :], uh[u0 + b, im, :]
                hr, hi = uh[h0 + a - b, re, :], uh[h0 + a - b, im, :]
                yr = ur * hr if yr is None else yr + ur * hr
                yi = ur * hi if yi is None else yi + ur * hi
                yr = yr - ui * hi
                yi = yi + ui * hr
            pp, qq = yr - yi, yr + yi
            if a > 0:
                zp, zq = pp - prev[1], qq + prev[0]
            else:
                zp, zq = pp, qq
            prev[:] = [pp, qq]
            z = pltpu.bitcast(jnp.concatenate([zp, zq], axis=0).astype(bf16), u32)
            r = (a % 2) * 16 + 4 * grp
            y_buf[sl, j, a // 2, r:r + 4, :] = z[0:4]
            y_buf[sl, j, a // 2, r + 8:r + 12, :] = z[4:8]
        return one

    def s3(sl, b, slot, j):
        rev = 7 - lax.broadcasted_iota(i32, (8, 128), 0)
        for t in range(2):
            a = 2 * j + t
            rows = pl.ds(pl.multiple_of(a * C, C), C)
            eo = []
            for part in range(2):
                r = 16 * t + 8 * part
                yp = y_buf[sl, :, j, r:r + 8, :].reshape(C // 2, 128)
                eo.append(jnp.dot(_bf(g_p[part * 32:(part + 1) * 32, :]), _bf(yp),
                                  preferred_element_type=f32))
            lo, hi = eo[0] + eo[1], eo[0] - eo[1]
            hi = [jnp.take_along_axis(hi[8 * i:8 * i + 8], rev, axis=0) for i in range(7, -1, -1)]
            y = jnp.concatenate([lo] + hi, axis=0)
            y = y + kvo[slot, rows, :].astype(f32) * coef[b, KS:KS + 1, :]
            kvo[slot, rows, :] = (q_buf[sl, rows, :].astype(f32) * y).astype(bf16)

    zero[0] = 0
    for c in range(4):
        w_copy(0, c).start()
        xc_copy(c).start()
        if c == 0:
            for cp in small_copies():
                cp.start()
        else:
            w_copy(1, c - 1).start()

    r = lax.broadcasted_iota(i32, (L2, L2), 0)
    c_ = lax.broadcasted_iota(i32, (L2, L2), 1)
    head = lambda i: jnp.where(i < 2 * M, i // M, (i - 2 * M) // SEG)
    ok = (r < 2 * M) | (c_ < 2 * M) | (c_ <= r)
    fill_ref[...] = jnp.where(head(r) == head(c_),
                              jnp.where(ok, 0.0, -1e9 / scale), -jnp.inf).astype(f32)

    rr = lax.broadcasted_iota(i32, (2 * C, C), 0)
    nn = lax.broadcasted_iota(i32, (2 * C, C), 1)
    kk = 8 * (rr // 16) + rr % 8
    mm = (2 * kk + 1) * (4 * nn + 1) + 4 * C * ((rr // 8) % 2) * (1 + 2 * (kk % 2))
    fm = jnp.cos((mm % (16 * C)).astype(f32) * (math.pi / (8 * C)))
    f_p[...] = pltpu.bitcast(fm.astype(bf16), u32)
    rr = lax.broadcasted_iota(i32, (C, C), 0)
    kk = lax.broadcasted_iota(i32, (C, C), 1)
    mm = (2 * kk + 1) * (2 * (rr % (C // 2)) + 1) + C * (7 - 6 * ((kk + rr // (C // 2)) % 2))
    gm = jnp.cos((mm % (8 * C)).astype(f32) * (math.pi / (4 * C))) * (2 ** -0.5 / C)
    g_p[...] = pltpu.bitcast(gm.astype(bf16), u32)
    for sl in range(2):
        k_buf[sl, 0:KPAD, :] = jnp.zeros((KPAD, 128), bf16)
    uh[0:32] = jnp.zeros((32, 2 * C, 128), f32)

    def pro_body(g, i, tasks):
        r0 = pl.multiple_of(i * 128, 128)
        x = x_buf[pl.ds(r0, 128), :]
        for p in range(8):
            ys = []
            for t in range(2):
                y = jnp.dot(x, wt(g // 2, 16 * (g % 2) + 2 * p + t),
                            preferred_element_type=f32)
                ys.append(y)
                for fn in tasks.get(2 * p + t, ()):
                    fn(y)
            pp = 8 * (g % 2) + p
            ring[pp // 2][pl.ds(pl.multiple_of(QOFF + r0, 64), 128),
                          ring_cols(g // 2, pp)] = jnp.concatenate(ys, axis=1).astype(bf16)

    def add_relayout(tasks, g, c, r):
        for u in range(15):
            def fn(y, u=u):
                stage[g % 3][D + zero[0]] = y[r:r + 16].astype(bf16)
                relayout(g, c, (128 * u) // 15, (128 * (u + 1)) // 15)
            tasks.setdefault(u, []).append(fn)

    def add_wo(tasks, n0):
        for u in range(15):
            def fn(y, u=u):
                wo_st[2048 + zero[0]] = y[96:112].astype(bf16)
                for r in range((64 * u) // 15, (64 * (u + 1)) // 15):
                    wo_pack(n0 + r // 32, 8 * (r % 32), 8 * (r % 32) + 8)
            tasks.setdefault(u, []).append(fn)

    def add_s01(tasks, j):
        for k in range(8):
            def fn(y, k=k):
                coef[NB + zero[0], 0:8, :] = y[48:56]
                s0_kv(0, 0, 0, j, k)
            tasks.setdefault(k, []).append(fn)
        tasks.setdefault(3, []).append(lambda y: s1_h(0, j))
        tasks.setdefault(11, []).append(lambda y: s1_u(0, 0, j))

    def period(g, body):
        if cfg['nopro']:
            return
        with jax.named_scope('pro%d' % g):
            lax.fori_loop(0, 4, lambda i, c: (body(i), c)[1], 0)

    def p0(c):
        @pl.when(c == 1)
        def _():
            w_copy(1, 3).start()
            for i in range(4):
                w_copy(2, i).start()

        @pl.when(c > 0)
        def _():
            w_copy(1, c - 1).wait()
        w_copy(0, c).wait()
        relayout(0, c)
        xc_copy(c).wait()
        xp[...] = pltpu.bitcast(
            x_buf[0:PRE, pl.ds(pl.multiple_of(c * 256, 256), 256)], u32)
        tasks = {}
        add_relayout(tasks, 1, (c + 3) % 4, 0)
        k0 = pl.multiple_of(c * 128, 128)
        for p in range(8):
            ys = []
            for t in range(2):
                hh = 2 * p + t
                w = _bf(wp[0][pl.ds(k0 + hh * HS, 128), :])
                y = (jnp.dot(_bf(xp[...]), w, preferred_element_type=f32)
                     + uh[2 * hh:2 * hh + 2].reshape(PRE, 128))
                uh[2 * hh:2 * hh + 2] = y.reshape(2, 2 * C, 128)
                ys.append(y)
                for fn in tasks.get(hh, ()):
                    fn(y[256 * t:])
            ring[p // 2][QOFF:QOFF + PRE, ring_cols(0, p)] = (
                jnp.concatenate(ys, axis=1).astype(bf16))
    period(0, p0)
    for cp in small_copies():
        cp.wait()
    skt = skt_buf[...].astype(f32)
    ddv = dd_buf[...].astype(f32)
    for b in range(NB):
        coef[b, 0:KS, :] = skt[:, b * 128:(b + 1) * 128]
        coef[b, KS:KS + 1, :] = ddv[b:b + 1, :]
    w_copy(1, 3).wait()
    relayout(1, 3)

    def p1(i):
        @pl.when(i == 0)
        def _():
            w_copy(3, 0).start()
            w_copy(3, 1).start()
            for cp in kvh_copies(0, 0) + kvh_copies(0, 1):
                cp.start()
            w_copy(4, 0).start()
            w_copy(4, 1).start()
            for c in range(2, 4):
                w_copy(3, c).start()
                w_copy(4, c).start()
        w_copy(2, i).wait()
        tasks = {}
        add_relayout(tasks, 2, i, 0)
        pro_body(1, i, tasks)
    period(1, p1)

    def p2(i):
        @pl.when(i == 0)
        def _():
            for c in range(4):
                w_copy(5, c).start()
                if c < 3:
                    wo_copy(2 * c).start()
                    wo_copy(2 * c + 1).start()
            for cp in kvh_copies(0, 0) + kvh_copies(0, 1):
                cp.wait()
        w_copy(3, i).wait()
        w_copy(4, i).wait()
        tasks = {}
        add_relayout(tasks, 3, i, 0)
        add_relayout(tasks, 4, i, 96)
        add_s01(tasks, i)
        pro_body(2, i, tasks)
    period(2, p2)

    def p3(i):
        @pl.when(i == 1)
        def _():
            wo_copy(6).start()
            wo_copy(7).start()
            x_copy(0).start()
            for cp in kvh_copies(1, 0) + kvh_copies(1, 1):
                cp.start()
            x_copy(1).start()

        @pl.when(i > 0)
        def _():
            wo_copy(2 * i - 2).wait()
            wo_copy(2 * i - 1).wait()
        w_copy(5, i).wait()
        tasks = {}
        add_relayout(tasks, 5, i, 0)
        add_wo(tasks, 2 * ((i + 3) % 4))
        add_s01(tasks, 4 + i)
        pro_body(3, i, tasks)
    period(3, p3)
    for n in (6, 7):
        wo_copy(n).wait()
        wo_pack(n)
    x_copy(0).wait()

    def step(cb, j, mem, par):
        s = cb * 8 + j
        x0 = pl.multiple_of(PRE + XR * s, 8)
        wpos = pl.multiple_of(lax.rem(s, RING // XR) * XR, 8)
        rpos = pl.multiple_of(lax.rem(s + QOFF // SEG, RING // SEG) * SEG, 32)
        rbase = pl.multiple_of((s - par) * SEG, 64)
        m0 = 0 if par == 0 else 72
        x8 = 8 + SEG * par

        sl1 = (cb + 1) & 1
        b1 = jnp.minimum(cb + 1, NB - 1)
        slot1 = cb + 1
        b3 = jnp.maximum(cb - 1, 0)
        slot3 = jnp.where(cb == 0, NB, cb - 1)
        s2 = s2_parts(cb & 1, j)
        nu = [0]

        def unit(pace):
            u = nu[0]
            nu[0] += 1
            if u in cfg['s0_at'][par]:
                coef[NB + zero[0], 0:8, :] = pace
                s0_kv(sl1, b1, slot1, j, cfg['s0_at'][par].index(u))
            if u in cfg['s2_at'][par]:
                s2(cfg['s2_at'][par].index(u), pace)

        def proj_q(p, lq):
            ys = []
            for t in range(2):
                ys.append(jnp.dot(lq, wt(2, 2 * p + t), preferred_element_type=f32))
                unit(ys[-1][:M])
            r0, r1 = (0, 48) if par == 0 else (48, 80)
            q_sc[p][r0:r1, :] = jnp.concatenate(ys, axis=1).astype(bf16)

        def proj_kv(p, m, lhs):
            ys = [jnp.dot(lhs, wt(m, 2 * p + t), preferred_element_type=f32)
                  for t in range(2)]
            ring[p // 2][pl.ds(wpos, XR), ring_cols(m, p)] = jnp.concatenate(
                [y[M:] for y in ys], axis=1).astype(bf16)
            unit(ys[0][:M])
            return jnp.concatenate([y[:M] for y in ys], axis=0).astype(bf16)

        def gather(m, p, mm):
            xx = ring[p // 2][pl.ds(rpos, SEG), ring_cols(m, p)]
            return jnp.concatenate([mm, xx[:, :DH], xx[:, DH:]], axis=0)

        def qk(p, mems):
            b = q_sc[p]
            q2 = jnp.concatenate([b[m0:m0 + M, :DH], b[m0:m0 + M, DH:],
                                  b[x8:x8 + SEG, :DH], b[x8:x8 + SEG, DH:]], axis=0)
            sc = lax.dot_general(q2, gather(0, p, mems[0]), (((1,), (1,)), ((), ())),
                                 preferred_element_type=f32)
            fill = fill_ref[...]
            sc = jnp.where(fill == 0.0, sc, fill)
            mx = jnp.max(sc, axis=1, keepdims=True)
            e = jnp.exp((sc - mx) * scale)
            l = jnp.sum(e, axis=1, keepdims=True)
            rc = pl.reciprocal(l, approx=True)
            rc = rc * (2.0 - l * rc)
            pr = (e * rc).astype(bf16)
            if not cfg['pstore']:
                return pr
            p_sc[p] = pltpu.bitcast(pr, u32)

        def pv(p, pr, mems):
            if cfg['pstore']:
                pr = _bf(p_sc[p])
            o = jnp.dot(pr, gather(1, p, mems[1]), preferred_element_type=f32)
            o_sc[p][m0:m0 + M, :] = jnp.concatenate([o[0:M], o[M:2 * M]], axis=1).astype(bf16)
            o_sc[p][x8:x8 + SEG, :] = jnp.concatenate(
                [o[2 * M:2 * M + SEG], o[2 * M + SEG:]], axis=1).astype(bf16)

        accs = [None] * 8
        odots = [(k, n) for k in range(0, H, cfg['och']) for n in range(8)]
        lcache = {}

        def oproj(cnt):
            r0, r1 = (0, 32) if par == 0 else (32, 80)
            for _ in range(min(cnt, len(odots))):
                k, n = odots.pop(0)
                ke = k + cfg['och']
                if k not in lcache:
                    lcache[k] = jnp.concatenate(
                        [o_sc[p][r0:r1, :] for p in range(k // 2, ke // 2)], axis=1)
                y = jnp.dot(lcache[k], _bf(wo_p[n, k * 64:ke * 64, :]),
                            preferred_element_type=f32)
                accs[n] = y if accs[n] is None else y + accs[n]
                unit(accs[n][:M])

        n1 = s + 7
        s1_u((n1 >> 3) & 1, n1 >> 3, n1 & 7)
        s1_h(sl1, j)
        s3(sl1, b3, slot3, j)

        if par == 0:
            lq = jnp.concatenate([mem, x_buf[pl.ds(rbase, 40), :]], axis=0)
        else:
            lq = jnp.concatenate([x_buf[pl.ds(rbase + 40, 24), :], mem], axis=0)
        for p in range(NPAIR):
            proj_q(p, lq)

        lhs = jnp.concatenate([mem, x_buf[pl.ds(x0, XR), :]], axis=0)
        mems, prs = {}, {}
        ag = cfg['agroup']
        for t in range(NPAIR + ag + 1):
            if t < NPAIR:
                mems[t] = [proj_kv(t, m, lhs) for m in range(2)]
            else:
                oproj(cfg['op_per'][par])
            if t % ag == 0:
                for p in range(t - 2 * ag, t - ag):
                    if 0 <= p < NPAIR:
                        pv(p, prs.pop(p), mems.pop(p))
                for p in range(t - ag, t):
                    if 0 <= p < NPAIR:
                        prs[p] = qk(p, mems[p])
        oproj(len(odots))
        out = jnp.concatenate(accs, axis=1).astype(bf16)
        if par == 0:
            outb[pl.ds(rbase, 24), :] = out[M:]
            return out[:M]
        outb[pl.ds(rbase + 24, 40), :] = out[:40]
        return out[40:]

    def four_steps(it, carry):
        cb, jj = it >> 1, it & 1

        @pl.when(cb + 1 < NB)
        def _():
            for cp in kvh_copies(cb + 1, jj):
                cp.wait()

        @pl.when(cb >= 1)
        def _():
            q_copy(cb - 1, jj).wait()

        @pl.when(it == 1)
        def _():
            x_copy(1).wait()

        @pl.when(it >= 1)
        def _():
            outb_copy(it - 1).start()

        @pl.when(it >= 3)
        def _():
            outa_copy((it - 3) >> 1, (it - 3) & 1).start()

        mem = mem_ref[...]
        for u in range(4):
            mem = step(cb, jj * 4 + u, mem, u % 2)
        mem_ref[...] = mem

        @pl.when(cb + 2 < NB)
        def _():
            for cp in kvh_copies(cb + 2, jj):
                cp.start()

        q_copy(cb, jj).start()
        return carry
    with jax.named_scope('main'):
        lax.fori_loop(0, 2 * NB, four_steps, 0)

    outb_copy(2 * NB - 1).start()
    outa_copy(NB - 2, 1).start()
    q_copy(NB - 1, 0).wait()
    q_copy(NB - 1, 1).wait()
    with jax.named_scope('epi'):
        for j in range(8):
            s3((NB - 1) % 2, NB - 1, NB - 1, j)
            if j % 2 == 1:
                outa_piece(NB - 1, (j - 1) * 2 * C, 4 * C).start()

    for it in range(2 * NB - 2):
        outa_copy(it // 2, it % 2).wait()
    for it in range(2 * NB):
        outb_copy(it).wait()
    for j in range(4):
        outa_piece(NB - 1, j * 4 * C, 4 * C).wait()


@functools.partial(jax.jit, static_argnames=("B_seg_len",))
def pallas_concat_heads__ssm_conv_h3__memory_aug_recurrent_mem_tr__prompt_kernel(
    A_q, A_k, A_v, A_shift_k, A_ssm_k, A_ssm_D, B_x, B_mem0, B_Wq, B_Wk, B_Wv, B_Wo,
    B_seg_len=SEG,
):
    assert B_seg_len == SEG
    assert A_q.shape == (1, S, D) and B_x.shape == (1, S, D)
    assert B_Wq.shape == (D, H, DH) and B_mem0.shape == (1, M, D)
    vm = pltpu.VMEM
    dma = pltpu.SemaphoreType.DMA
    scratch = [
        vm((D + 4, 16, DH), bf16), vm((D + 4, 16, DH), bf16),
        vm((D + 4, 16, DH), bf16),
        vm((2048 + 4, 16, 128), bf16),
        vm((8, H * DH // 2, 128), u32),
        vm((S, D), bf16),
        vm((M, D), bf16),
        vm((S, D), bf16),
        vm((NB + 1, 32, 128), f32),
        vm((2, S + 64, 128), bf16),
        vm((2, S, 128), bf16), vm((2, S, 128), bf16),
        vm((2, 128, S), bf16),
        vm((NB + 1, S, 128), bf16),
        vm((4 * NC + 1, 2 * C, 128), f32),
        vm((2, 8, 8, 32, 128), u32),
        vm((8, 32 + KPAD, 128), f32),
        vm((C, C), u32), vm((C // 2, C), u32),
        vm((PRE // 2, 256), u32),
        dma((40,)),
        pltpu.SMEM((1,), i32),
    ]
    scratch += [vm((16 * HS, 128), u32)] * 6
    scratch += [vm((RING, 8 * DH), bf16)] * 8
    scratch += [vm((L2, 2 * DH), bf16)] * (2 * NPAIR)
    scratch += [vm((NPAIR, L2 // 2, L2), u32)]
    scratch += [vm((L2, L2), f32), vm((KS, D), bf16), vm((NB, 128), bf16)]

    out = pl.pallas_call(
        _kernel,
        out_shape=jax.ShapeDtypeStruct((S, 2 * D), bf16),
        in_specs=[pl.BlockSpec(memory_space=pl.ANY)] * 12,
        out_specs=pl.BlockSpec(memory_space=pl.ANY),
        scratch_shapes=scratch,
        compiler_params=pltpu.CompilerParams(vmem_limit_bytes=120 * 1024 * 1024,
                                             disable_bounds_checks=True,
                                             disable_semaphore_checks=True),
        name="ssm_memtr",
    )(A_q.reshape(S, D), A_k.reshape(S, D), A_v.reshape(S, D), A_shift_k.T, A_ssm_k,
      A_ssm_D.reshape(NB, 128), B_x.reshape(S, D), B_mem0.reshape(M, D),
      B_Wq, B_Wk, B_Wv, B_Wo.reshape(H * DH // 16, 16, D))
    return out.reshape(1, S, 2 * D)
```

```python
import functools
import math

import jax
import jax.numpy as jnp
from jax import lax
import jax.experimental.pallas as pl
import jax.experimental.pallas.tpu as pltpu

bf16, f32, u32, i32 = jnp.bfloat16, jnp.float32, jnp.uint32, jnp.int32

S = 2048
D = 1024
H, DH = 32, 128
M, SEG = 8, 32
NSEG = S // SEG
KS = 4

XR = 24
PRE = S - NSEG * XR
RING = 576
QOFF = 64
HS = 514
NPAIR = H // 2
L2 = 2 * (M + SEG)

C = 128
NC = S // C
NB = D // 128
KPAD = 16

CFG = dict(
    att={4: ([], [0, 1, 2, 3]), 18: ([12, 13, 14, 15], []),
         **{t: ([t - 6, t - 5], [t - 2, t - 1]) for t in range(6, 18, 2)}},
    pstore=True, och=8, op_per=[4, 4],
    s2_at=[list(range(0, 32)), list(range(62, 94))],
    s0_at=[list(range(16, 24)), list(range(78, 86))],
    nopro=False, border='uyh', exp2=True, mstore=True,
)


def _bf(x):
    return pltpu.bitcast(x, bf16)


def _kernel(q_hbm, k_hbm, v_hbm, skt_hbm, h_hbm, dd_hbm, x_hbm, mem0_hbm,
            wq_hbm, wk_hbm, wv_hbm, wo_hbm, out_hbm,
            st0, st1, st2, wo_st, wo_p, x_buf, mem_ref, outb,
            coef, k_buf, v_buf, q_buf, h_buf, kvo,
            uh, y_buf, kf, f_p, g_p, xp, sems, zero,
            *bufs):
    wp = bufs[0:6]
    ring = bufs[6:14]
    o_sc = bufs[14:30]
    q_sc = bufs[30:46]
    p_sc, m_sc, fill_ref, skt_buf, dd_buf = bufs[46:51]
    stage = (st0, st1, st2)
    w_hbm = (wk_hbm, wv_hbm, wq_hbm)
    scale = DH ** -0.5
    cfg = CFG
    SW, SWO, SX, SSM, SKVH, SQ, SOUT = 0, 12, 20, 26, 29, 33, 37

    def w_copy(g, c):
        r0 = c * 256
        return pltpu.make_async_copy(
            w_hbm[g // 2].at[pl.ds(r0, 256), pl.ds(16 * (g % 2), 16), :],
            stage[g % 3].at[pl.ds(r0, 256)],
            sems.at[SW + (g % 3) * 4 + c])

    def wo_copy(n):
        return pltpu.make_async_copy(
            wo_hbm.at[:, :, pl.ds(pl.multiple_of(n * 128, 128), 128)],
            wo_st.at[pl.ds(n * 256, 256)], sems.at[SWO + n])

    def xc_copy(c):
        cols = pl.ds(pl.multiple_of(c * 256, 256), 256)
        return pltpu.make_async_copy(x_hbm.at[pl.ds(0, PRE), cols],
                                     x_buf.at[pl.ds(0, PRE), cols], sems.at[SX + c])

    def x_copy(part):
        r0, n = ((PRE, 128), (PRE + 128, S - PRE - 128))[part]
        return pltpu.make_async_copy(
            x_hbm.at[pl.ds(r0, n)], x_buf.at[pl.ds(r0, n)], sems.at[SX + 4 + part])

    def small_copies():
        return [pltpu.make_async_copy(skt_hbm, skt_buf, sems.at[SSM + 0]),
                pltpu.make_async_copy(dd_hbm, dd_buf, sems.at[SSM + 1]),
                pltpu.make_async_copy(mem0_hbm, mem_ref, sems.at[SSM + 2])]

    def col(b):
        return pl.ds(pl.multiple_of(b * 128, 128), 128)

    HALF = S // 2

    def half_rows(half, off=0):
        return pl.ds(pl.multiple_of(half * HALF, HALF) + off, HALF)

    def kvh_copies(b, half):
        sl, t = b & 1, half_rows(half)
        sem = sems.at[SKVH + 2 * sl + half]
        return [pltpu.make_async_copy(k_hbm.at[t, col(b)],
                                      k_buf.at[sl, half_rows(half, KPAD)], sem),
                pltpu.make_async_copy(v_hbm.at[t, col(b)], v_buf.at[sl, t], sem),
                pltpu.make_async_copy(h_hbm.at[col(b), t], h_buf.at[sl, :, t], sem)]

    def q_copy(b, half):
        sl, t = b & 1, half_rows(half)
        return pltpu.make_async_copy(q_hbm.at[t, col(b)], q_buf.at[sl, t],
                                     sems.at[SQ + 2 * sl + half])

    def outa_copy(b, half):
        t = half_rows(half)
        return pltpu.make_async_copy(kvo.at[b, t], out_hbm.at[t, col(b)], sems.at[SOUT])

    def outa_piece(b, r0, n):
        return pltpu.make_async_copy(kvo.at[b, pl.ds(r0, n)],
                                     out_hbm.at[pl.ds(r0, n), col(b)], sems.at[SOUT + 1])

    def outb_copy(it):
        rows = pl.ds(pl.multiple_of(it * 4 * SEG, 4 * SEG), 4 * SEG)
        return pltpu.make_async_copy(outb.at[rows], out_hbm.at[rows, pl.ds(D, D)],
                                     sems.at[SOUT + 2])

    def relayout(g, c, lo_i=0, hi_i=128):
        src, dst = stage[g % 3], wp[g]
        d0 = c * 256
        for i in range(lo_i, hi_i):
            a = pltpu.bitcast(src[d0 + 2 * i], u32)
            b = pltpu.bitcast(src[d0 + 2 * i + 1], u32)
            lo = (a & jnp.uint32(0xFFFF)) | (b << 16)
            hi = (a >> 16) | (b & jnp.uint32(0xFFFF0000))
            row = c * 128 + i
            dst[pl.ds(row, 8, stride=2 * HS), :] = lo
            dst[pl.ds(row + HS, 8, stride=2 * HS), :] = hi

    def wo_pack(n, r0=0, r1=256):
        for r in range(r0, r1, 8):
            blk = pltpu.bitcast(wo_st[pl.ds(n * 256 + r, 8)], u32)
            wo_p[n, r * 8:(r + 8) * 8, :] = blk.reshape(64, 128)

    def wt(m, h):
        g, hh = 2 * m + h // 16, h % 16
        return _bf(wp[g][hh * HS:hh * HS + D // 2, :])

    def ring_cols(m, p):
        c0 = 512 * m + 256 * (p % 2)
        return slice(c0, c0 + 256)

    def s0_kv(sl, b, slot, j, i):
        t0 = pl.multiple_of(j * 2 * C, 2 * C)
        kw = k_buf.at[sl, pl.ds(t0, 2 * C + KPAD)]
        vw = v_buf.at[sl, pl.ds(t0, 2 * C)]
        ow = kvo.at[slot, pl.ds(t0, 2 * C)]
        kf[i] = kw[32 * i:32 * i + 32 + KPAD, :].astype(f32)
        acc = None
        for tap in range(KS):
            term = kf[i, KPAD - tap:KPAD - tap + 32, :] * coef[b, tap:tap + 1, :]
            acc = term if acc is None else acc + term
        ow[32 * i:32 * i + 32, :] = (acc * vw[32 * i:32 * i + 32, :].astype(f32)).astype(bf16)

    def s1_h(sl, j):
        for t in range(2):
            a = 2 * j + t
            hh = h_buf[sl, :, pl.ds(pl.multiple_of(a * C, C), C)]
            for half in range(2):
                fm = _bf(f_p[half * 64:(half + 1) * 64, :])
                uh[sl * 2 * NC + NC + a, half * C:(half + 1) * C, :] = lax.dot_general(
                    fm, hh, (((1,), (1,)), ((), ())), preferred_element_type=f32)

    def s1_u(sl, slot, j):
        for t in range(2):
            a = 2 * j + t
            kv = kvo[slot, pl.ds(pl.multiple_of(a * C, C), C), :]
            for half in range(2):
                fm = _bf(f_p[half * 64:(half + 1) * 64, :])
                uh[sl * 2 * NC + a, half * C:(half + 1) * C, :] = jnp.dot(
                    fm, kv, preferred_element_type=f32)

    def s2_parts(sl, j):
        u0 = sl * 2 * NC
        h0 = u0 + NC
        r0 = pl.multiple_of(j * 32, 32)
        prev = []

        def one(idx, pace):
            grp, a = divmod(idx, NC)
            re, im = pl.ds(r0 + 16 * grp, 8), pl.ds(r0 + 16 * grp + 8, 8)
            yr = yi = None
            for b in range(a + 1):
                if b == a:
                    uh[4 * NC + zero[0], 0:8, :] = pace
                ur, ui = uh[u0 + b, re, :], uh[u0 + b, im, :]
                hr, hi = uh[h0 + a - b, re, :], uh[h0 + a - b, im, :]
                yr = ur * hr if yr is None else yr + ur * hr
                yi = ur * hi if yi is None else yi + ur * hi
                yr = yr - ui * hi
                yi = yi + ui * hr
            pp, qq = yr - yi, yr + yi
            if a > 0:
                zp, zq = pp - prev[1], qq + prev[0]
            else:
                zp, zq = pp, qq
            prev[:] = [pp, qq]
            z = pltpu.bitcast(jnp.concatenate([zp, zq], axis=0).astype(bf16), u32)
            r = (a % 2) * 16 + 4 * grp
            y_buf[sl, j, a // 2, r:r + 4, :] = z[0:4]
            y_buf[sl, j, a // 2, r + 8:r + 12, :] = z[4:8]
        return one

    def s3(sl, b, slot, j):
        rev = 7 - lax.broadcasted_iota(i32, (8, 128), 0)
        for t in range(2):
            a = 2 * j + t
            rows = pl.ds(pl.multiple_of(a * C, C), C)
            eo = []
            for part in range(2):
                r = 16 * t + 8 * part
                yp = y_buf[sl, :, j, r:r + 8, :].reshape(C // 2, 128)
                eo.append(jnp.dot(_bf(g_p[part * 32:(part + 1) * 32, :]), _bf(yp),
                                  preferred_element_type=f32))
            lo, hi = eo[0] + eo[1], eo[0] - eo[1]
            hi = [jnp.take_along_axis(hi[8 * i:8 * i + 8], rev, axis=0) for i in range(7, -1, -1)]
            y = jnp.concatenate([lo] + hi, axis=0)
            y = y + kvo[slot, rows, :].astype(f32) * coef[b, KS:KS + 1, :]
            kvo[slot, rows, :] = (q_buf[sl, rows, :].astype(f32) * y).astype(bf16)

    zero[0] = 0
    for c in range(4):
        w_copy(0, c).start()
        xc_copy(c).start()
        if c == 0:
            for cp in small_copies():
                cp.start()
        else:
            w_copy(1, c - 1).start()

    r = lax.broadcasted_iota(i32, (L2, L2), 0)
    c_ = lax.broadcasted_iota(i32, (L2, L2), 1)
    head = lambda i: jnp.where(i < 2 * M, i // M, (i - 2 * M) // SEG)
    ok = (r < 2 * M) | (c_ < 2 * M) | (c_ <= r)
    fill_ref[...] = jnp.where(head(r) == head(c_),
                              jnp.where(ok, 0.0, -1e9 / scale), -jnp.inf).astype(f32)

    rr = lax.broadcasted_iota(i32, (2 * C, C), 0)
    nn = lax.broadcasted_iota(i32, (2 * C, C), 1)
    kk = 8 * (rr // 16) + rr % 8
    mm = (2 * kk + 1) * (4 * nn + 1) + 4 * C * ((rr // 8) % 2) * (1 + 2 * (kk % 2))
    fm = jnp.cos((mm % (16 * C)).astype(f32) * (math.pi / (8 * C)))
    f_p[...] = pltpu.bitcast(fm.astype(bf16), u32)
    rr = lax.broadcasted_iota(i32, (C, C), 0)
    kk = lax.broadcasted_iota(i32, (C, C), 1)
    mm = (2 * kk + 1) * (2 * (rr % (C // 2)) + 1) + C * (7 - 6 * ((kk + rr // (C // 2)) % 2))
    gm = jnp.cos((mm % (8 * C)).astype(f32) * (math.pi / (4 * C))) * (2 ** -0.5 / C)
    g_p[...] = pltpu.bitcast(gm.astype(bf16), u32)
    for sl in range(2):
        k_buf[sl, 0:KPAD, :] = jnp.zeros((KPAD, 128), bf16)
    uh[0:32] = jnp.zeros((32, 2 * C, 128), f32)

    def pro_body(g, i, tasks):
        r0 = pl.multiple_of(i * 128, 128)
        x = x_buf[pl.ds(r0, 128), :]
        for p in range(8):
            ys = []
            for t in range(2):
                y = jnp.dot(x, wt(g // 2, 16 * (g % 2) + 2 * p + t),
                            preferred_element_type=f32)
                ys.append(y)
                for fn in tasks.get(2 * p + t, ()):
                    fn(y)
            pp = 8 * (g % 2) + p
            ring[pp // 2][pl.ds(pl.multiple_of(QOFF + r0, 64), 128),
                          ring_cols(g // 2, pp)] = jnp.concatenate(ys, axis=1).astype(bf16)

    def add_relayout(tasks, g, c, r):
        for u in range(15):
            def fn(y, u=u):
                stage[g % 3][D + zero[0]] = y[r:r + 16].astype(bf16)
                relayout(g, c, (128 * u) // 15, (128 * (u + 1)) // 15)
            tasks.setdefault(u, []).append(fn)

    def add_wo(tasks, n0):
        for u in range(15):
            def fn(y, u=u):
                wo_st[2048 + zero[0]] = y[96:112].astype(bf16)
                for r in range((64 * u) // 15, (64 * (u + 1)) // 15):
                    wo_pack(n0 + r // 32, 8 * (r % 32), 8 * (r % 32) + 8)
            tasks.setdefault(u, []).append(fn)

    def add_s01(tasks, j):
        for k in range(8):
            def fn(y, k=k):
                coef[NB + zero[0], 0:8, :] = y[48:56]
                s0_kv(0, 0, 0, j, k)
            tasks.setdefault(k, []).append(fn)
        tasks.setdefault(3, []).append(lambda y: s1_h(0, j))
        tasks.setdefault(11, []).append(lambda y: s1_u(0, 0, j))

    def period(g, body):
        if cfg['nopro']:
            return
        with jax.named_scope('pro%d' % g):
            lax.fori_loop(0, 4, lambda i, c: (body(i), c)[1], 0)

    def p0(c):
        @pl.when(c == 1)
        def _():
            w_copy(1, 3).start()
            for i in range(4):
                w_copy(2, i).start()

        @pl.when(c > 0)
        def _():
            w_copy(1, c - 1).wait()
        w_copy(0, c).wait()
        relayout(0, c)
        xc_copy(c).wait()
        xp[...] = pltpu.bitcast(
            x_buf[0:PRE, pl.ds(pl.multiple_of(c * 256, 256), 256)], u32)
        tasks = {}
        add_relayout(tasks, 1, (c + 3) % 4, 0)
        k0 = pl.multiple_of(c * 128, 128)
        for p in range(8):
            ys = []
            for t in range(2):
                hh = 2 * p + t
                w = _bf(wp[0][pl.ds(k0 + hh * HS, 128), :])
                y = (jnp.dot(_bf(xp[...]), w, preferred_element_type=f32)
                     + uh[2 * hh:2 * hh + 2].reshape(PRE, 128))
                uh[2 * hh:2 * hh + 2] = y.reshape(2, 2 * C, 128)
                ys.append(y)
                for fn in tasks.get(hh, ()):
                    fn(y[256 * t:])
            ring[p // 2][QOFF:QOFF + PRE, ring_cols(0, p)] = (
                jnp.concatenate(ys, axis=1).astype(bf16))
    period(0, p0)
    for cp in small_copies():
        cp.wait()
    skt = skt_buf[...].astype(f32)
    ddv = dd_buf[...].astype(f32)
    for b in range(NB):
        coef[b, 0:KS, :] = skt[:, b * 128:(b + 1) * 128]
        coef[b, KS:KS + 1, :] = ddv[b:b + 1, :]
    w_copy(1, 3).wait()
    relayout(1, 3)

    def p1(i):
        @pl.when(i == 0)
        def _():
            w_copy(3, 0).start()
            w_copy(3, 1).start()
            for cp in kvh_copies(0, 0) + kvh_copies(0, 1):
                cp.start()
            w_copy(4, 0).start()
            w_copy(4, 1).start()
            for c in range(2, 4):
                w_copy(3, c).start()
                w_copy(4, c).start()
        w_copy(2, i).wait()
        tasks = {}
        add_relayout(tasks, 2, i, 0)
        pro_body(1, i, tasks)
    period(1, p1)

    def p2(i):
        @pl.when(i == 0)
        def _():
            for c in range(4):
                w_copy(5, c).start()
                if c < 3:
                    wo_copy(2 * c).start()
                    wo_copy(2 * c + 1).start()
            for cp in kvh_copies(0, 0) + kvh_copies(0, 1):
                cp.wait()
        w_copy(3, i).wait()
        w_copy(4, i).wait()
        tasks = {}
        add_relayout(tasks, 3, i, 0)
        add_relayout(tasks, 4, i, 96)
        add_s01(tasks, i)
        pro_body(2, i, tasks)
    period(2, p2)

    def p3(i):
        @pl.when(i == 1)
        def _():
            wo_copy(6).start()
            wo_copy(7).start()
            x_copy(0).start()
            for cp in kvh_copies(1, 0) + kvh_copies(1, 1):
                cp.start()
            x_copy(1).start()

        @pl.when(i > 0)
        def _():
            wo_copy(2 * i - 2).wait()
            wo_copy(2 * i - 1).wait()
        w_copy(5, i).wait()
        tasks = {}
        add_relayout(tasks, 5, i, 0)
        add_wo(tasks, 2 * ((i + 3) % 4))
        add_s01(tasks, 4 + i)
        pro_body(3, i, tasks)
    period(3, p3)
    for n in (6, 7):
        wo_copy(n).wait()
        wo_pack(n)
    x_copy(0).wait()

    def step(cb, j, mem, par):
        s = cb * 8 + j
        x0 = pl.multiple_of(PRE + XR * s, 8)
        wpos = pl.multiple_of(lax.rem(s, RING // XR) * XR, 8)
        rpos = pl.multiple_of(lax.rem(s + QOFF // SEG, RING // SEG) * SEG, 32)
        rbase = pl.multiple_of((s - par) * SEG, 64)
        m0 = 0 if par == 0 else 72
        x8 = 8 + SEG * par

        sl1 = (cb + 1) & 1
        b1 = jnp.minimum(cb + 1, NB - 1)
        slot1 = cb + 1
        b3 = jnp.maximum(cb - 1, 0)
        slot3 = jnp.where(cb == 0, NB, cb - 1)
        s2 = s2_parts(cb & 1, j)
        nu = [0]

        def unit(pace):
            u = nu[0]
            nu[0] += 1
            if u in cfg['s0_at'][par]:
                coef[NB + zero[0], 0:8, :] = pace
                s0_kv(sl1, b1, slot1, j, cfg['s0_at'][par].index(u))
            if u in cfg['s2_at'][par]:
                s2(cfg['s2_at'][par].index(u), pace)

        def proj_q(p, lq):
            ys = []
            for t in range(2):
                ys.append(jnp.dot(lq, wt(2, 2 * p + t), preferred_element_type=f32))
                unit(ys[-1][:M])
            r0, r1 = (0, 48) if par == 0 else (48, 80)
            q_sc[p][r0:r1, :] = jnp.concatenate(ys, axis=1).astype(bf16)

        def proj_kv(p, m, lhs):
            ys = [jnp.dot(lhs, wt(m, 2 * p + t), preferred_element_type=f32)
                  for t in range(2)]
            ring[p // 2][pl.ds(wpos, XR), ring_cols(m, p)] = jnp.concatenate(
                [y[M:] for y in ys], axis=1).astype(bf16)
            unit(ys[0][:M])
            if cfg['mstore']:
                m_sc[2 * p + m] = jnp.concatenate([y[:M] for y in ys], axis=1).astype(bf16)
                return None
            return jnp.concatenate([y[:M] for y in ys], axis=0).astype(bf16)

        def gather(m, p, mm):
            xx = ring[p // 2][pl.ds(rpos, SEG), ring_cols(m, p)]
            if cfg['mstore']:
                mm = jnp.concatenate([m_sc[2 * p + m, :, :DH], m_sc[2 * p + m, :, DH:]], axis=0)
            return jnp.concatenate([mm, xx[:, :DH], xx[:, DH:]], axis=0)

        def qk(p, mems):
            b = q_sc[p]
            q2 = jnp.concatenate([b[m0:m0 + M, :DH], b[m0:m0 + M, DH:],
                                  b[x8:x8 + SEG, :DH], b[x8:x8 + SEG, DH:]], axis=0)
            sc = lax.dot_general(q2, gather(0, p, mems[0]), (((1,), (1,)), ((), ())),
                                 preferred_element_type=f32)
            fill = fill_ref[...]
            sc = jnp.where(fill == 0.0, sc, fill)
            mx = jnp.max(sc, axis=1, keepdims=True)
            if cfg['exp2']:
                e = jnp.exp2((sc - mx) * (scale * math.log2(math.e)))
            else:
                e = jnp.exp((sc - mx) * scale)
            l = jnp.sum(e, axis=1, keepdims=True)
            rc = pl.reciprocal(l, approx=True)
            rc = rc * (2.0 - l * rc)
            pr = (e * rc).astype(bf16)
            if not cfg['pstore']:
                return pr
            p_sc[p] = pltpu.bitcast(pr, u32)

        def pv(p, pr, mems):
            if cfg['pstore']:
                pr = _bf(p_sc[p])
            o = jnp.dot(pr, gather(1, p, mems[1]), preferred_element_type=f32)
            o_sc[p][m0:m0 + M, :] = jnp.concatenate([o[0:M], o[M:2 * M]], axis=1).astype(bf16)
            o_sc[p][x8:x8 + SEG, :] = jnp.concatenate(
                [o[2 * M:2 * M + SEG], o[2 * M + SEG:]], axis=1).astype(bf16)

        accs = [None] * 8
        odots = [(k, n) for k in range(0, H, cfg['och']) for n in range(8)]
        lcache = {}

        def oproj(cnt):
            r0, r1 = (0, 32) if par == 0 else (32, 80)
            for _ in range(min(cnt, len(odots))):
                k, n = odots.pop(0)
                ke = k + cfg['och']
                if k not in lcache:
                    lcache[k] = jnp.concatenate(
                        [o_sc[p][r0:r1, :] for p in range(k // 2, ke // 2)], axis=1)
                y = jnp.dot(lcache[k], _bf(wo_p[n, k * 64:ke * 64, :]),
                            preferred_element_type=f32)
                accs[n] = y if accs[n] is None else y + accs[n]
                unit(accs[n][:M])

        n1 = s + 7
        pre = dict(u=lambda: s1_u((n1 >> 3) & 1, n1 >> 3, n1 & 7),
                   h=lambda: s1_h(sl1, j),
                   y=lambda: s3(sl1, b3, slot3, j))
        for key in cfg['border']:
            pre[key]()

        if par == 0:
            lq = jnp.concatenate([mem, x_buf[pl.ds(rbase, 40), :]], axis=0)
        else:
            lq = jnp.concatenate([x_buf[pl.ds(rbase + 40, 24), :], mem], axis=0)
        for p in range(NPAIR):
            proj_q(p, lq)

        lhs = jnp.concatenate([mem, x_buf[pl.ds(x0, XR), :]], axis=0)
        mems, prs = {}, {}
        att = cfg['att']
        for t in range(max(att) + 1):
            if t < NPAIR:
                mems[t] = [proj_kv(t, m, lhs) for m in range(2)]
            else:
                oproj(cfg['op_per'][par])
            for p in att.get(t, ((), ()))[0]:
                pv(p, prs.pop(p), mems.pop(p))
            for p in att.get(t, ((), ()))[1]:
                prs[p] = qk(p, mems[p])
        oproj(len(odots))
        out = jnp.concatenate(accs, axis=1).astype(bf16)
        if par == 0:
            outb[pl.ds(rbase, 24), :] = out[M:]
            return out[:M]
        outb[pl.ds(rbase + 24, 40), :] = out[:40]
        return out[40:]

    def four_steps(it, carry):
        cb, jj = it >> 1, it & 1

        @pl.when(cb + 1 < NB)
        def _():
            for cp in kvh_copies(cb + 1, jj):
                cp.wait()

        @pl.when(cb >= 1)
        def _():
            q_copy(cb - 1, jj).wait()

        @pl.when(it == 1)
        def _():
            x_copy(1).wait()

        @pl.when(it >= 1)
        def _():
            outb_copy(it - 1).start()

        @pl.when(it >= 3)
        def _():
            outa_copy((it - 3) >> 1, (it - 3) & 1).start()

        mem = mem_ref[...]
        for u in range(4):
            mem = step(cb, jj * 4 + u, mem, u % 2)
        mem_ref[...] = mem

        @pl.when(cb + 2 < NB)
        def _():
            for cp in kvh_copies(cb + 2, jj):
                cp.start()

        q_copy(cb, jj).start()
        return carry
    with jax.named_scope('main'):
        lax.fori_loop(0, 2 * NB, four_steps, 0)

    outb_copy(2 * NB - 1).start()
    outa_copy(NB - 2, 1).start()
    q_copy(NB - 1, 0).wait()
    q_copy(NB - 1, 1).wait()
    with jax.named_scope('epi'):
        for j in range(8):
            s3((NB - 1) % 2, NB - 1, NB - 1, j)
            if j % 2 == 1:
                outa_piece(NB - 1, (j - 1) * 2 * C, 4 * C).start()

    for it in range(2 * NB - 2):
        outa_copy(it // 2, it % 2).wait()
    for it in range(2 * NB):
        outb_copy(it).wait()
    for j in range(4):
        outa_piece(NB - 1, j * 4 * C, 4 * C).wait()


@functools.partial(jax.jit, static_argnames=("B_seg_len",))
def pallas_concat_heads__ssm_conv_h3__memory_aug_recurrent_mem_tr__prompt_kernel(
    A_q, A_k, A_v, A_shift_k, A_ssm_k, A_ssm_D, B_x, B_mem0, B_Wq, B_Wk, B_Wv, B_Wo,
    B_seg_len=SEG,
):
    assert B_seg_len == SEG
    assert A_q.shape == (1, S, D) and B_x.shape == (1, S, D)
    assert B_Wq.shape == (D, H, DH) and B_mem0.shape == (1, M, D)
    vm = pltpu.VMEM
    dma = pltpu.SemaphoreType.DMA
    scratch = [
        vm((D + 4, 16, DH), bf16), vm((D + 4, 16, DH), bf16),
        vm((D + 4, 16, DH), bf16),
        vm((2048 + 4, 16, 128), bf16),
        vm((8, H * DH // 2, 128), u32),
        vm((S, D), bf16),
        vm((M, D), bf16),
        vm((S, D), bf16),
        vm((NB + 1, 32, 128), f32),
        vm((2, S + 64, 128), bf16),
        vm((2, S, 128), bf16), vm((2, S, 128), bf16),
        vm((2, 128, S), bf16),
        vm((NB + 1, S, 128), bf16),
        vm((4 * NC + 1, 2 * C, 128), f32),
        vm((2, 8, 8, 32, 128), u32),
        vm((8, 32 + KPAD, 128), f32),
        vm((C, C), u32), vm((C // 2, C), u32),
        vm((PRE // 2, 256), u32),
        dma((40,)),
        pltpu.SMEM((1,), i32),
    ]
    scratch += [vm((16 * HS, 128), u32)] * 6
    scratch += [vm((RING, 8 * DH), bf16)] * 8
    scratch += [vm((L2, 2 * DH), bf16)] * (2 * NPAIR)
    scratch += [vm((NPAIR, L2 // 2, L2), u32)]
    scratch += [vm((2 * NPAIR, M, 2 * DH), bf16)]
    scratch += [vm((L2, L2), f32), vm((KS, D), bf16), vm((NB, 128), bf16)]

    out = pl.pallas_call(
        _kernel,
        out_shape=jax.ShapeDtypeStruct((S, 2 * D), bf16),
        in_specs=[pl.BlockSpec(memory_space=pl.ANY)] * 12,
        out_specs=pl.BlockSpec(memory_space=pl.ANY),
        scratch_shapes=scratch,
        compiler_params=pltpu.CompilerParams(vmem_limit_bytes=120 * 1024 * 1024,
                                             disable_bounds_checks=True,
                                             disable_semaphore_checks=True),
        name="ssm_memtr",
    )(A_q.reshape(S, D), A_k.reshape(S, D), A_v.reshape(S, D), A_shift_k.T, A_ssm_k,
      A_ssm_D.reshape(NB, 128), B_x.reshape(S, D), B_mem0.reshape(M, D),
      B_Wq, B_Wk, B_Wv, B_Wo.reshape(H * DH // 16, 16, D))
    return out.reshape(1, S, 2 * D)
```

```python
import functools
import math

import jax
import jax.numpy as jnp
from jax import lax
import jax.experimental.pallas as pl
import jax.experimental.pallas.tpu as pltpu

bf16, f32, u32, i32 = jnp.bfloat16, jnp.float32, jnp.uint32, jnp.int32

S = 2048
D = 1024
H, DH = 32, 128
M, SEG = 8, 32
NSEG = S // SEG
KS = 4

XR = 24
PRE = S - NSEG * XR
RING = 576
QOFF = 64
HS = 514
NPAIR = H // 2
L2 = 2 * (M + SEG)

C = 128
NC = S // C
NB = D // 128
KPAD = 16

CFG = dict(
    att={4: ([], [0, 1, 2, 3]), 18: ([12, 13, 14, 15], []),
         **{t: ([t - 6, t - 5], [t - 2, t - 1]) for t in range(6, 18, 2)}},
    pstore=True, och=8, op_per=[4, 4],
    s2_at=[list(range(0, 32)), list(range(62, 94))],
    s0_at=[list(range(16, 24)), list(range(78, 86))],
    nopro=False, border='uyh', exp2=True, mstore=True,
)


def _bf(x):
    return pltpu.bitcast(x, bf16)


def _kernel(q_hbm, k_hbm, v_hbm, skt_hbm, h_hbm, dd_hbm, x_hbm, mem0_hbm,
            wq_hbm, wk_hbm, wv_hbm, wo_hbm, out_hbm,
            st0, st1, st2, wo_st, wo_p, x_buf, mem_ref, outb,
            coef, k_buf, v_buf, q_buf, h_buf, kvo,
            uh, y_buf, kf, f_p, g_p, xp, sems, zero,
            *bufs):
    wp = bufs[0:6]
    ring = bufs[6:14]
    o_sc = bufs[14:30]
    q_sc = bufs[30:46]
    p_sc, m_sc, fill_ref, skt_buf, dd_buf = bufs[46:51]
    stage = (st0, st1, st2)
    w_hbm = (wk_hbm, wv_hbm, wq_hbm)
    scale = DH ** -0.5
    cfg = CFG
    SW, SWO, SX, SSM, SKVH, SQ, SOUT = 0, 12, 20, 26, 29, 33, 37

    def w_copy(g, c):
        r0 = c * 256
        return pltpu.make_async_copy(
            w_hbm[g // 2].at[pl.ds(r0, 256), pl.ds(16 * (g % 2), 16), :],
            stage[g % 3].at[pl.ds(r0, 256)],
            sems.at[SW + (g % 3) * 4 + c])

    def wo_copy(n):
        return pltpu.make_async_copy(
            wo_hbm.at[:, :, pl.ds(pl.multiple_of(n * 128, 128), 128)],
            wo_st.at[pl.ds(n * 256, 256)], sems.at[SWO + n])

    def xc_copy(c):
        cols = pl.ds(pl.multiple_of(c * 256, 256), 256)
        return pltpu.make_async_copy(x_hbm.at[pl.ds(0, PRE), cols],
                                     x_buf.at[pl.ds(0, PRE), cols], sems.at[SX + c])

    def x_copy(part):
        r0, n = ((PRE, 128), (PRE + 128, S - PRE - 128))[part]
        return pltpu.make_async_copy(
            x_hbm.at[pl.ds(r0, n)], x_buf.at[pl.ds(r0, n)], sems.at[SX + 4 + part])

    def small_copies():
        return [pltpu.make_async_copy(skt_hbm, skt_buf, sems.at[SSM + 0]),
                pltpu.make_async_copy(dd_hbm, dd_buf, sems.at[SSM + 1]),
                pltpu.make_async_copy(mem0_hbm, mem_ref, sems.at[SSM + 2])]

    def col(b):
        return pl.ds(pl.multiple_of(b * 128, 128), 128)

    HALF = S // 2

    def half_rows(half, off=0):
        return pl.ds(pl.multiple_of(half * HALF, HALF) + off, HALF)

    def kvh_copies(b, half):
        sl, t = b & 1, half_rows(half)
        sem = sems.at[SKVH + 2 * sl + half]
        return [pltpu.make_async_copy(k_hbm.at[t, col(b)],
                                      k_buf.at[sl, half_rows(half, KPAD)], sem),
                pltpu.make_async_copy(v_hbm.at[t, col(b)], v_buf.at[sl, t], sem),
                pltpu.make_async_copy(h_hbm.at[col(b), t], h_buf.at[sl, :, t], sem)]

    def q_copy(b, half):
        sl, t = b & 1, half_rows(half)
        return pltpu.make_async_copy(q_hbm.at[t, col(b)], q_buf.at[sl, t],
                                     sems.at[SQ + 2 * sl + half])

    def outa_copy(b, half):
        t = half_rows(half)
        return pltpu.make_async_copy(kvo.at[b, t], out_hbm.at[t, col(b)], sems.at[SOUT])

    def outa_piece(b, r0, n):
        return pltpu.make_async_copy(kvo.at[b, pl.ds(r0, n)],
                                     out_hbm.at[pl.ds(r0, n), col(b)], sems.at[SOUT + 1])

    def outb_copy(it):
        rows = pl.ds(pl.multiple_of(it * 4 * SEG, 4 * SEG), 4 * SEG)
        return pltpu.make_async_copy(outb.at[rows], out_hbm.at[rows, pl.ds(D, D)],
                                     sems.at[SOUT + 2])

    def relayout(g, c, lo_i=0, hi_i=128):
        src, dst = stage[g % 3], wp[g]
        d0 = c * 256
        for i in range(lo_i, hi_i):
            a = pltpu.bitcast(src[d0 + 2 * i], u32)
            b = pltpu.bitcast(src[d0 + 2 * i + 1], u32)
            lo = (a & jnp.uint32(0xFFFF)) | (b << 16)
            hi = (a >> 16) | (b & jnp.uint32(0xFFFF0000))
            row = c * 128 + i
            dst[pl.ds(row, 8, stride=2 * HS), :] = lo
            dst[pl.ds(row + HS, 8, stride=2 * HS), :] = hi

    def wo_pack(n, r0=0, r1=256):
        for r in range(r0, r1, 8):
            blk = pltpu.bitcast(wo_st[pl.ds(n * 256 + r, 8)], u32)
            wo_p[n, r * 8:(r + 8) * 8, :] = blk.reshape(64, 128)

    def wt(m, h):
        g, hh = 2 * m + h // 16, h % 16
        return _bf(wp[g][hh * HS:hh * HS + D // 2, :])

    def ring_cols(m, p):
        c0 = 512 * m + 256 * (p % 2)
        return slice(c0, c0 + 256)

    def s0_kv(sl, b, slot, j, i):
        t0 = pl.multiple_of(j * 2 * C, 2 * C)
        kw = k_buf.at[sl, pl.ds(t0, 2 * C + KPAD)]
        vw = v_buf.at[sl, pl.ds(t0, 2 * C)]
        ow = kvo.at[slot, pl.ds(t0, 2 * C)]
        kf[i] = kw[32 * i:32 * i + 32 + KPAD, :].astype(f32)
        acc = None
        for tap in range(KS):
            term = kf[i, KPAD - tap:KPAD - tap + 32, :] * coef[b, tap:tap + 1, :]
            acc = term if acc is None else acc + term
        ow[32 * i:32 * i + 32, :] = (acc * vw[32 * i:32 * i + 32, :].astype(f32)).astype(bf16)

    def s1_h(sl, j):
        for t in range(2):
            a = 2 * j + t
            hh = h_buf[sl, :, pl.ds(pl.multiple_of(a * C, C), C)]
            for half in range(2):
                fm = _bf(f_p[half * 64:(half + 1) * 64, :])
                uh[sl * 2 * NC + NC + a, half * C:(half + 1) * C, :] = lax.dot_general(
                    fm, hh, (((1,), (1,)), ((), ())), preferred_element_type=f32)

    def s1_u(sl, slot, j):
        for t in range(2):
            a = 2 * j + t
            kv = kvo[slot, pl.ds(pl.multiple_of(a * C, C), C), :]
            for half in range(2):
                fm = _bf(f_p[half * 64:(half + 1) * 64, :])
                uh[sl * 2 * NC + a, half * C:(half + 1) * C, :] = jnp.dot(
                    fm, kv, preferred_element_type=f32)

    def s2_parts(sl, j):
        u0 = sl * 2 * NC
        h0 = u0 + NC
        r0 = pl.multiple_of(j * 32, 32)
        prev = []

        def one(idx, pace):
            grp, a = divmod(idx, NC)
            re, im = pl.ds(r0 + 16 * grp, 8), pl.ds(r0 + 16 * grp + 8, 8)
            yr = yi = None
            for b in range(a + 1):
                if b == a:
                    uh[4 * NC + zero[0], 0:8, :] = pace
                ur, ui = uh[u0 + b, re, :], uh[u0 + b, im, :]
                hr, hi = uh[h0 + a - b, re, :], uh[h0 + a - b, im, :]
                yr = ur * hr if yr is None else yr + ur * hr
                yi = ur * hi if yi is None else yi + ur * hi
                yr = yr - ui * hi
                yi = yi + ui * hr
            pp, qq = yr - yi, yr + yi
            if a > 0:
                zp, zq = pp - prev[1], qq + prev[0]
            else:
                zp, zq = pp, qq
            prev[:] = [pp, qq]
            z = pltpu.bitcast(jnp.concatenate([zp, zq], axis=0).astype(bf16), u32)
            r = (a % 2) * 16 + 4 * grp
            y_buf[sl, j, a // 2, r:r + 4, :] = z[0:4]
            y_buf[sl, j, a // 2, r + 8:r + 12, :] = z[4:8]
        return one

    def s3(sl, b, slot, j):
        rev = 7 - lax.broadcasted_iota(i32, (8, 128), 0)
        for t in range(2):
            a = 2 * j + t
            rows = pl.ds(pl.multiple_of(a * C, C), C)
            eo = []
            for part in range(2):
                r = 16 * t + 8 * part
                yp = y_buf[sl, :, j, r:r + 8, :].reshape(C // 2, 128)
                eo.append(jnp.dot(_bf(g_p[part * 32:(part + 1) * 32, :]), _bf(yp),
                                  preferred_element_type=f32))
            lo, hi = eo[0] + eo[1], eo[0] - eo[1]
            hi = [jnp.take_along_axis(hi[8 * i:8 * i + 8], rev, axis=0) for i in range(7, -1, -1)]
            y = jnp.concatenate([lo] + hi, axis=0)
            y = y + kvo[slot, rows, :].astype(f32) * coef[b, KS:KS + 1, :]
            kvo[slot, rows, :] = (q_buf[sl, rows, :].astype(f32) * y).astype(bf16)

    zero[0] = 0
    for c in range(4):
        w_copy(0, c).start()
        xc_copy(c).start()
        if c == 0:
            for cp in small_copies():
                cp.start()
        else:
            w_copy(1, c - 1).start()

    r = lax.broadcasted_iota(i32, (L2, L2), 0)
    c_ = lax.broadcasted_iota(i32, (L2, L2), 1)
    head = lambda i: jnp.where(i < 2 * M, i // M, (i - 2 * M) // SEG)
    ok = (r < 2 * M) | (c_ < 2 * M) | (c_ <= r)
    fill_ref[...] = jnp.where(head(r) == head(c_),
                              jnp.where(ok, 0.0, -1e9 / scale), -jnp.inf).astype(f32)

    rr = lax.broadcasted_iota(i32, (2 * C, C), 0)
    nn = lax.broadcasted_iota(i32, (2 * C, C), 1)
    kk = 8 * (rr // 16) + rr % 8
    mm = (2 * kk + 1) * (4 * nn + 1) + 4 * C * ((rr // 8) % 2) * (1 + 2 * (kk % 2))
    fm = jnp.cos((mm % (16 * C)).astype(f32) * (math.pi / (8 * C)))
    f_p[...] = pltpu.bitcast(fm.astype(bf16), u32)
    rr = lax.broadcasted_iota(i32, (C, C), 0)
    kk = lax.broadcasted_iota(i32, (C, C), 1)
    mm = (2 * kk + 1) * (2 * (rr % (C // 2)) + 1) + C * (7 - 6 * ((kk + rr // (C // 2)) % 2))
    gm = jnp.cos((mm % (8 * C)).astype(f32) * (math.pi / (4 * C))) * (2 ** -0.5 / C)
    g_p[...] = pltpu.bitcast(gm.astype(bf16), u32)
    for sl in range(2):
        k_buf[sl, 0:KPAD, :] = jnp.zeros((KPAD, 128), bf16)
    uh[0:32] = jnp.zeros((32, 2 * C, 128), f32)

    def pro_body(g, i, tasks):
        r0 = pl.multiple_of(i * 128, 128)
        x = x_buf[pl.ds(r0, 128), :]
        for p in range(8):
            ys = []
            for t in range(2):
                y = jnp.dot(x, wt(g // 2, 16 * (g % 2) + 2 * p + t),
                            preferred_element_type=f32)
                ys.append(y)
                for fn in tasks.get(2 * p + t, ()):
                    fn(y)
            pp = 8 * (g % 2) + p
            ring[pp // 2][pl.ds(pl.multiple_of(QOFF + r0, 64), 128),
                          ring_cols(g // 2, pp)] = jnp.concatenate(ys, axis=1).astype(bf16)

    def add_relayout(tasks, g, c, r):
        for u in range(15):
            def fn(y, u=u):
                stage[g % 3][D + zero[0]] = y[r:r + 16].astype(bf16)
                relayout(g, c, (128 * u) // 15, (128 * (u + 1)) // 15)
            tasks.setdefault(u, []).append(fn)

    def add_wo(tasks, n0):
        for u in range(15):
            def fn(y, u=u):
                wo_st[2048 + zero[0]] = y[96:112].astype(bf16)
                for r in range((64 * u) // 15, (64 * (u + 1)) // 15):
                    wo_pack(n0 + r // 32, 8 * (r % 32), 8 * (r % 32) + 8)
            tasks.setdefault(u, []).append(fn)

    def add_s01(tasks, j):
        for k in range(8):
            def fn(y, k=k):
                coef[NB + zero[0], 0:8, :] = y[48:56]
                s0_kv(0, 0, 0, j, k)
            tasks.setdefault(k, []).append(fn)
        tasks.setdefault(3, []).append(lambda y: s1_h(0, j))
        tasks.setdefault(11, []).append(lambda y: s1_u(0, 0, j))

    def period(g, body):
        if cfg['nopro']:
            return
        with jax.named_scope('pro%d' % g):
            lax.fori_loop(0, 4, lambda i, c: (body(i), c)[1], 0)

    def p0(c):
        @pl.when(c > 0)
        def _():
            w_copy(1, c - 1).wait()
        w_copy(0, c).wait()
        relayout(0, c)
        xc_copy(c).wait()
        xp[...] = pltpu.bitcast(
            x_buf[0:PRE, pl.ds(pl.multiple_of(c * 256, 256), 256)], u32)
        tasks = {}
        add_relayout(tasks, 1, (c + 3) % 4, 0)
        k0 = pl.multiple_of(c * 128, 128)
        for p in range(8):
            ys = []
            for t in range(2):
                hh = 2 * p + t
                w = _bf(wp[0][pl.ds(k0 + hh * HS, 128), :])
                y = (jnp.dot(_bf(xp[...]), w, preferred_element_type=f32)
                     + uh[2 * hh:2 * hh + 2].reshape(PRE, 128))
                uh[2 * hh:2 * hh + 2] = y.reshape(2, 2 * C, 128)
                ys.append(y)
                for fn in tasks.get(hh, ()):
                    fn(y[256 * t:])
            ring[p // 2][QOFF:QOFF + PRE, ring_cols(0, p)] = (
                jnp.concatenate(ys, axis=1).astype(bf16))

        @pl.when(c == 0)
        def _():
            w_copy(1, 3).start()
            for i in range(4):
                w_copy(2, i).start()
    period(0, p0)
    w_copy(1, 3).wait()
    relayout(1, 3)
    for cp in small_copies():
        cp.wait()
    w_copy(3, 0).start()
    w_copy(3, 1).start()
    for cp in kvh_copies(0, 0) + kvh_copies(0, 1):
        cp.start()
    w_copy(4, 0).start()
    w_copy(4, 1).start()
    for c in range(2, 4):
        w_copy(3, c).start()
        w_copy(4, c).start()
    skt = skt_buf[...].astype(f32)
    ddv = dd_buf[...].astype(f32)
    for b in range(NB):
        coef[b, 0:KS, :] = skt[:, b * 128:(b + 1) * 128]
        coef[b, KS:KS + 1, :] = ddv[b:b + 1, :]

    def p1(i):
        w_copy(2, i).wait()
        tasks = {}
        add_relayout(tasks, 2, i, 0)
        pro_body(1, i, tasks)
    period(1, p1)
    for c in range(4):
        w_copy(5, c).start()
        if c < 3:
            wo_copy(2 * c).start()
            wo_copy(2 * c + 1).start()
    for cp in kvh_copies(0, 0) + kvh_copies(0, 1):
        cp.wait()

    def p2(i):
        w_copy(3, i).wait()
        w_copy(4, i).wait()
        tasks = {}
        add_relayout(tasks, 3, i, 0)
        add_relayout(tasks, 4, i, 96)
        add_s01(tasks, i)
        pro_body(2, i, tasks)
    period(2, p2)

    def p3(i):
        @pl.when(i > 0)
        def _():
            wo_copy(2 * i - 2).wait()
            wo_copy(2 * i - 1).wait()
        w_copy(5, i).wait()
        tasks = {}
        add_relayout(tasks, 5, i, 0)
        add_wo(tasks, 2 * ((i + 3) % 4))
        add_s01(tasks, 4 + i)
        pro_body(3, i, tasks)

        @pl.when(i == 0)
        def _():
            wo_copy(6).start()
            wo_copy(7).start()
            x_copy(0).start()
            for cp in kvh_copies(1, 0) + kvh_copies(1, 1):
                cp.start()
            x_copy(1).start()
    period(3, p3)
    for n in (6, 7):
        wo_copy(n).wait()
        wo_pack(n)
    x_copy(0).wait()

    def step(cb, j, mem, par):
        s = cb * 8 + j
        x0 = pl.multiple_of(PRE + XR * s, 8)
        wpos = pl.multiple_of(lax.rem(s, RING // XR) * XR, 8)
        rpos = pl.multiple_of(lax.rem(s + QOFF // SEG, RING // SEG) * SEG, 32)
        rbase = pl.multiple_of((s - par) * SEG, 64)
        m0 = 0 if par == 0 else 72
        x8 = 8 + SEG * par

        sl1 = (cb + 1) & 1
        b1 = jnp.minimum(cb + 1, NB - 1)
        slot1 = cb + 1
        b3 = jnp.maximum(cb - 1, 0)
        slot3 = jnp.where(cb == 0, NB, cb - 1)
        s2 = s2_parts(cb & 1, j)
        nu = [0]

        def unit(pace):
            u = nu[0]
            nu[0] += 1
            if u in cfg['s0_at'][par]:
                coef[NB + zero[0], 0:8, :] = pace
                s0_kv(sl1, b1, slot1, j, cfg['s0_at'][par].index(u))
            if u in cfg['s2_at'][par]:
                s2(cfg['s2_at'][par].index(u), pace)

        def proj_q(p, lq):
            ys = []
            for t in range(2):
                ys.append(jnp.dot(lq, wt(2, 2 * p + t), preferred_element_type=f32))
                unit(ys[-1][:M])
            r0, r1 = (0, 48) if par == 0 else (48, 80)
            q_sc[p][r0:r1, :] = jnp.concatenate(ys, axis=1).astype(bf16)

        def proj_kv(p, m, lhs):
            ys = [jnp.dot(lhs, wt(m, 2 * p + t), preferred_element_type=f32)
                  for t in range(2)]
            ring[p // 2][pl.ds(wpos, XR), ring_cols(m, p)] = jnp.concatenate(
                [y[M:] for y in ys], axis=1).astype(bf16)
            unit(ys[0][:M])
            if cfg['mstore']:
                m_sc[2 * p + m] = jnp.concatenate([y[:M] for y in ys], axis=1).astype(bf16)
                return None
            return jnp.concatenate([y[:M] for y in ys], axis=0).astype(bf16)

        def gather(m, p, mm):
            xx = ring[p // 2][pl.ds(rpos, SEG), ring_cols(m, p)]
            if cfg['mstore']:
                mm = jnp.concatenate([m_sc[2 * p + m, :, :DH], m_sc[2 * p + m, :, DH:]], axis=0)
            return jnp.concatenate([mm, xx[:, :DH], xx[:, DH:]], axis=0)

        def qk(p, mems):
            b = q_sc[p]
            q2 = jnp.concatenate([b[m0:m0 + M, :DH], b[m0:m0 + M, DH:],
                                  b[x8:x8 + SEG, :DH], b[x8:x8 + SEG, DH:]], axis=0)
            sc = lax.dot_general(q2, gather(0, p, mems[0]), (((1,), (1,)), ((), ())),
                                 preferred_element_type=f32)
            fill = fill_ref[...]
            sc = jnp.where(fill == 0.0, sc, fill)
            mx = jnp.max(sc, axis=1, keepdims=True)
            if cfg['exp2']:
                e = jnp.exp2((sc - mx) * (scale * math.log2(math.e)))
            else:
                e = jnp.exp((sc - mx) * scale)
            l = jnp.sum(e, axis=1, keepdims=True)
            rc = pl.reciprocal(l, approx=True)
            rc = rc * (2.0 - l * rc)
            pr = (e * rc).astype(bf16)
            if not cfg['pstore']:
                return pr
            p_sc[p] = pltpu.bitcast(pr, u32)

        def pv(p, pr, mems):
            if cfg['pstore']:
                pr = _bf(p_sc[p])
            o = jnp.dot(pr, gather(1, p, mems[1]), preferred_element_type=f32)
            o_sc[p][m0:m0 + M, :] = jnp.concatenate([o[0:M], o[M:2 * M]], axis=1).astype(bf16)
            o_sc[p][x8:x8 + SEG, :] = jnp.concatenate(
                [o[2 * M:2 * M + SEG], o[2 * M + SEG:]], axis=1).astype(bf16)

        accs = [None] * 8
        odots = [(k, n) for k in range(0, H, cfg['och']) for n in range(8)]
        lcache = {}

        def oproj(cnt):
            r0, r1 = (0, 32) if par == 0 else (32, 80)
            for _ in range(min(cnt, len(odots))):
                k, n = odots.pop(0)
                ke = k + cfg['och']
                if k not in lcache:
                    lcache[k] = jnp.concatenate(
                        [o_sc[p][r0:r1, :] for p in range(k // 2, ke // 2)], axis=1)
                y = jnp.dot(lcache[k], _bf(wo_p[n, k * 64:ke * 64, :]),
                            preferred_element_type=f32)
                accs[n] = y if accs[n] is None else y + accs[n]
                unit(accs[n][:M])

        n1 = s + 7
        pre = dict(u=lambda: s1_u((n1 >> 3) & 1, n1 >> 3, n1 & 7),
                   h=lambda: s1_h(sl1, j),
                   y=lambda: s3(sl1, b3, slot3, j))
        for key in cfg['border']:
            pre[key]()

        if par == 0:
            lq = jnp.concatenate([mem, x_buf[pl.ds(rbase, 40), :]], axis=0)
        else:
            lq = jnp.concatenate([x_buf[pl.ds(rbase + 40, 24), :], mem], axis=0)
        for p in range(NPAIR):
            proj_q(p, lq)

        lhs = jnp.concatenate([mem, x_buf[pl.ds(x0, XR), :]], axis=0)
        mems, prs = {}, {}
        att = cfg['att']
        for t in range(max(att) + 1):
            if t < NPAIR:
                mems[t] = [proj_kv(t, m, lhs) for m in range(2)]
            else:
                oproj(cfg['op_per'][par])
            for p in att.get(t, ((), ()))[0]:
                pv(p, prs.pop(p), mems.pop(p))
            for p in att.get(t, ((), ()))[1]:
                prs[p] = qk(p, mems[p])
        oproj(len(odots))
        out = jnp.concatenate(accs, axis=1).astype(bf16)
        if par == 0:
            outb[pl.ds(rbase, 24), :] = out[M:]
            return out[:M]
        outb[pl.ds(rbase + 24, 40), :] = out[:40]
        return out[40:]

    def four_steps(it, carry):
        cb, jj = it >> 1, it & 1

        @pl.when(cb + 1 < NB)
        def _():
            for cp in kvh_copies(cb + 1, jj):
                cp.wait()

        @pl.when(cb >= 1)
        def _():
            q_copy(cb - 1, jj).wait()

        @pl.when(it == 1)
        def _():
            x_copy(1).wait()

        @pl.when(it >= 1)
        def _():
            outb_copy(it - 1).start()

        @pl.when(it >= 3)
        def _():
            outa_copy((it - 3) >> 1, (it - 3) & 1).start()

        mem = mem_ref[...]
        for u in range(4):
            mem = step(cb, jj * 4 + u, mem, u % 2)
        mem_ref[...] = mem

        @pl.when(cb + 2 < NB)
        def _():
            for cp in kvh_copies(cb + 2, jj):
                cp.start()

        q_copy(cb, jj).start()
        return carry
    with jax.named_scope('main'):
        lax.fori_loop(0, 2 * NB, four_steps, 0)

    outb_copy(2 * NB - 1).start()
    outa_copy(NB - 2, 1).start()
    q_copy(NB - 1, 0).wait()
    q_copy(NB - 1, 1).wait()
    with jax.named_scope('epi'):
        for j in range(8):
            s3((NB - 1) % 2, NB - 1, NB - 1, j)
            if j % 2 == 1:
                outa_piece(NB - 1, (j - 1) * 2 * C, 4 * C).start()

    for it in range(2 * NB - 2):
        outa_copy(it // 2, it % 2).wait()
    for it in range(2 * NB):
        outb_copy(it).wait()
    for j in range(4):
        outa_piece(NB - 1, j * 4 * C, 4 * C).wait()


@functools.partial(jax.jit, static_argnames=("B_seg_len",))
def pallas_concat_heads__ssm_conv_h3__memory_aug_recurrent_mem_tr__prompt_kernel(
    A_q, A_k, A_v, A_shift_k, A_ssm_k, A_ssm_D, B_x, B_mem0, B_Wq, B_Wk, B_Wv, B_Wo,
    B_seg_len=SEG,
):
    assert B_seg_len == SEG
    assert A_q.shape == (1, S, D) and B_x.shape == (1, S, D)
    assert B_Wq.shape == (D, H, DH) and B_mem0.shape == (1, M, D)
    vm = pltpu.VMEM
    dma = pltpu.SemaphoreType.DMA
    scratch = [
        vm((D + 4, 16, DH), bf16), vm((D + 4, 16, DH), bf16),
        vm((D + 4, 16, DH), bf16),
        vm((2048 + 4, 16, 128), bf16),
        vm((8, H * DH // 2, 128), u32),
        vm((S, D), bf16),
        vm((M, D), bf16),
        vm((S, D), bf16),
        vm((NB + 1, 32, 128), f32),
        vm((2, S + 64, 128), bf16),
        vm((2, S, 128), bf16), vm((2, S, 128), bf16),
        vm((2, 128, S), bf16),
        vm((NB + 1, S, 128), bf16),
        vm((4 * NC + 1, 2 * C, 128), f32),
        vm((2, 8, 8, 32, 128), u32),
        vm((8, 32 + KPAD, 128), f32),
        vm((C, C), u32), vm((C // 2, C), u32),
        vm((PRE // 2, 256), u32),
        dma((40,)),
        pltpu.SMEM((1,), i32),
    ]
    scratch += [vm((16 * HS, 128), u32)] * 6
    scratch += [vm((RING, 8 * DH), bf16)] * 8
    scratch += [vm((L2, 2 * DH), bf16)] * (2 * NPAIR)
    scratch += [vm((NPAIR, L2 // 2, L2), u32)]
    scratch += [vm((2 * NPAIR, M, 2 * DH), bf16)]
    scratch += [vm((L2, L2), f32), vm((KS, D), bf16), vm((NB, 128), bf16)]

    out = pl.pallas_call(
        _kernel,
        out_shape=jax.ShapeDtypeStruct((S, 2 * D), bf16),
        in_specs=[pl.BlockSpec(memory_space=pl.ANY)] * 12,
        out_specs=pl.BlockSpec(memory_space=pl.ANY),
        scratch_shapes=scratch,
        compiler_params=pltpu.CompilerParams(vmem_limit_bytes=120 * 1024 * 1024,
                                             disable_bounds_checks=True,
                                             disable_semaphore_checks=True),
        name="ssm_memtr",
    )(A_q.reshape(S, D), A_k.reshape(S, D), A_v.reshape(S, D), A_shift_k.T, A_ssm_k,
      A_ssm_D.reshape(NB, 128), B_x.reshape(S, D), B_mem0.reshape(M, D),
      B_Wq, B_Wk, B_Wv, B_Wo.reshape(H * DH // 16, 16, D))
    return out.reshape(1, S, 2 * D)
```

```python
import functools
import math

import jax
import jax.numpy as jnp
from jax import lax
import jax.experimental.pallas as pl
import jax.experimental.pallas.tpu as pltpu

bf16, f32, u32, i32 = jnp.bfloat16, jnp.float32, jnp.uint32, jnp.int32

S = 2048
D = 1024
H, DH = 32, 128
M, SEG = 8, 32
NSEG = S // SEG
KS = 4

XR = 24
PRE = S - NSEG * XR
RING = 576
QOFF = 64
HS = 514
NPAIR = H // 2
L2 = 2 * (M + SEG)

C = 128
NC = S // C
NB = D // 128
KPAD = 16

CFG = dict(
    att={4: ([], [0, 1, 2, 3]), 18: ([12, 13, 14, 15], []),
         **{t: ([t - 6, t - 5], [t - 2, t - 1]) for t in range(6, 18, 2)}},
    pstore=True, och=8, op_per=[4, 4],
    s2_at=[list(range(0, 32)), list(range(62, 94))],
    s0_at=[list(range(17, 25)), list(range(78, 86))],
    nopro=False, border='uyh', exp2=False, mstore=True,
)


def _bf(x):
    return pltpu.bitcast(x, bf16)


def _kernel(q_hbm, k_hbm, v_hbm, skt_hbm, h_hbm, dd_hbm, x_hbm, mem0_hbm,
            wq_hbm, wk_hbm, wv_hbm, wo_hbm, out_hbm,
            st0, st1, st2, wo_st, wo_p, x_buf, mem_ref, outb,
            coef, k_buf, v_buf, q_buf, h_buf, kvo,
            uh, y_buf, kf, f_p, g_p, xp, sems, zero,
            *bufs):
    wp = bufs[0:6]
    ring = bufs[6:14]
    o_sc = bufs[14:30]
    q_sc = bufs[30:46]
    p_sc, m_sc, fill_ref, skt_buf, dd_buf = bufs[46:51]
    stage = (st0, st1, st2)
    w_hbm = (wk_hbm, wv_hbm, wq_hbm)
    scale = DH ** -0.5
    cfg = CFG
    SW, SWO, SX, SSM, SKVH, SQ, SOUT = 0, 12, 20, 26, 29, 33, 37

    def w_copy(g, c):
        r0 = c * 256
        return pltpu.make_async_copy(
            w_hbm[g // 2].at[pl.ds(r0, 256), pl.ds(16 * (g % 2), 16), :],
            stage[g % 3].at[pl.ds(r0, 256)],
            sems.at[SW + (g % 3) * 4 + c])

    def wo_copy(n):
        return pltpu.make_async_copy(
            wo_hbm.at[:, :, pl.ds(pl.multiple_of(n * 128, 128), 128)],
            wo_st.at[pl.ds(n * 256, 256)], sems.at[SWO + n])

    def xc_copy(c):
        cols = pl.ds(pl.multiple_of(c * 256, 256), 256)
        return pltpu.make_async_copy(x_hbm.at[pl.ds(0, PRE), cols],
                                     x_buf.at[pl.ds(0, PRE), cols], sems.at[SX + c])

    def x_copy(part):
        r0, n = ((PRE, 128), (PRE + 128, S - PRE - 128))[part]
        return pltpu.make_async_copy(
            x_hbm.at[pl.ds(r0, n)], x_buf.at[pl.ds(r0, n)], sems.at[SX + 4 + part])

    def small_copies():
        return [pltpu.make_async_copy(skt_hbm, skt_buf, sems.at[SSM + 0]),
                pltpu.make_async_copy(dd_hbm, dd_buf, sems.at[SSM + 1]),
                pltpu.make_async_copy(mem0_hbm, mem_ref, sems.at[SSM + 2])]

    def col(b):
        return pl.ds(pl.multiple_of(b * 128, 128), 128)

    HALF = S // 2

    def half_rows(half, off=0):
        return pl.ds(pl.multiple_of(half * HALF, HALF) + off, HALF)

    def kvh_copies(b, half):
        sl, t = b & 1, half_rows(half)
        sem = sems.at[SKVH + 2 * sl + half]
        return [pltpu.make_async_copy(k_hbm.at[t, col(b)],
                                      k_buf.at[sl, half_rows(half, KPAD)], sem),
                pltpu.make_async_copy(v_hbm.at[t, col(b)], v_buf.at[sl, t], sem),
                pltpu.make_async_copy(h_hbm.at[col(b), t], h_buf.at[sl, :, t], sem)]

    def q_copy(b, half):
        sl, t = b & 1, half_rows(half)
        return pltpu.make_async_copy(q_hbm.at[t, col(b)], q_buf.at[sl, t],
                                     sems.at[SQ + 2 * sl + half])

    def outa_copy(b, half):
        t = half_rows(half)
        return pltpu.make_async_copy(kvo.at[b, t], out_hbm.at[t, col(b)], sems.at[SOUT])

    def outa_piece(b, r0, n):
        return pltpu.make_async_copy(kvo.at[b, pl.ds(r0, n)],
                                     out_hbm.at[pl.ds(r0, n), col(b)], sems.at[SOUT + 1])

    def outb_copy(pr):
        rows = pl.ds(pl.multiple_of(pr * 2 * SEG, 2 * SEG), 2 * SEG)
        return pltpu.make_async_copy(outb.at[rows], out_hbm.at[rows, pl.ds(D, D)],
                                     sems.at[SOUT + 2])

    def relayout(g, c, lo_i=0, hi_i=128):
        src, dst = stage[g % 3], wp[g]
        d0 = c * 256
        for i in range(lo_i, hi_i):
            a = pltpu.bitcast(src[d0 + 2 * i], u32)
            b = pltpu.bitcast(src[d0 + 2 * i + 1], u32)
            lo = (a & jnp.uint32(0xFFFF)) | (b << 16)
            hi = (a >> 16) | (b & jnp.uint32(0xFFFF0000))
            row = c * 128 + i
            dst[pl.ds(row, 8, stride=2 * HS), :] = lo
            dst[pl.ds(row + HS, 8, stride=2 * HS), :] = hi

    def wo_pack(n, r0=0, r1=256):
        for r in range(r0, r1, 8):
            blk = pltpu.bitcast(wo_st[pl.ds(n * 256 + r, 8)], u32)
            wo_p[n, r * 8:(r + 8) * 8, :] = blk.reshape(64, 128)

    def wt(m, h):
        g, hh = 2 * m + h // 16, h % 16
        return _bf(wp[g][hh * HS:hh * HS + D // 2, :])

    def ring_cols(m, p):
        c0 = 512 * m + 256 * (p % 2)
        return slice(c0, c0 + 256)

    def s0_kv(sl, b, slot, j, i):
        t0 = pl.multiple_of(j * 2 * C, 2 * C)
        kw = k_buf.at[sl, pl.ds(t0, 2 * C + KPAD)]
        vw = v_buf.at[sl, pl.ds(t0, 2 * C)]
        ow = kvo.at[slot, pl.ds(t0, 2 * C)]
        kf[i] = kw[32 * i:32 * i + 32 + KPAD, :].astype(f32)
        acc = None
        for tap in range(KS):
            term = kf[i, KPAD - tap:KPAD - tap + 32, :] * coef[b, tap:tap + 1, :]
            acc = term if acc is None else acc + term
        ow[32 * i:32 * i + 32, :] = (acc * vw[32 * i:32 * i + 32, :].astype(f32)).astype(bf16)

    def s1_h(sl, j):
        for t in range(2):
            a = 2 * j + t
            hh = h_buf[sl, :, pl.ds(pl.multiple_of(a * C, C), C)]
            for half in range(2):
                fm = _bf(f_p[half * 64:(half + 1) * 64, :])
                uh[sl * 2 * NC + NC + a, half * C:(half + 1) * C, :] = lax.dot_general(
                    fm, hh, (((1,), (1,)), ((), ())), preferred_element_type=f32)

    def s1_u(sl, slot, j):
        for t in range(2):
            a = 2 * j + t
            kv = kvo[slot, pl.ds(pl.multiple_of(a * C, C), C), :]
            for half in range(2):
                fm = _bf(f_p[half * 64:(half + 1) * 64, :])
                uh[sl * 2 * NC + a, half * C:(half + 1) * C, :] = jnp.dot(
                    fm, kv, preferred_element_type=f32)

    def s2_parts(sl, j):
        u0 = sl * 2 * NC
        h0 = u0 + NC
        r0 = pl.multiple_of(j * 32, 32)
        prev = []

        def one(idx, pace):
            grp, a = divmod(idx, NC)
            re, im = pl.ds(r0 + 16 * grp, 8), pl.ds(r0 + 16 * grp + 8, 8)
            yr = yi = None
            for b in range(a + 1):
                if b == a:
                    uh[4 * NC + zero[0], 0:8, :] = pace
                ur, ui = uh[u0 + b, re, :], uh[u0 + b, im, :]
                hr, hi = uh[h0 + a - b, re, :], uh[h0 + a - b, im, :]
                yr = ur * hr if yr is None else yr + ur * hr
                yi = ur * hi if yi is None else yi + ur * hi
                yr = yr - ui * hi
                yi = yi + ui * hr
            pp, qq = yr - yi, yr + yi
            if a > 0:
                zp, zq = pp - prev[1], qq + prev[0]
            else:
                zp, zq = pp, qq
            prev[:] = [pp, qq]
            z = pltpu.bitcast(jnp.concatenate([zp, zq], axis=0).astype(bf16), u32)
            r = (a % 2) * 16 + 4 * grp
            y_buf[sl, j, a // 2, r:r + 4, :] = z[0:4]
            y_buf[sl, j, a // 2, r + 8:r + 12, :] = z[4:8]
        return one

    def s3(sl, b, slot, j):
        rev = 7 - lax.broadcasted_iota(i32, (8, 128), 0)
        for t in range(2):
            a = 2 * j + t
            rows = pl.ds(pl.multiple_of(a * C, C), C)
            eo = []
            for part in range(2):
                r = 16 * t + 8 * part
                yp = y_buf[sl, :, j, r:r + 8, :].reshape(C // 2, 128)
                eo.append(jnp.dot(_bf(g_p[part * 32:(part + 1) * 32, :]), _bf(yp),
                                  preferred_element_type=f32))
            lo, hi = eo[0] + eo[1], eo[0] - eo[1]
            hi = [jnp.take_along_axis(hi[8 * i:8 * i + 8], rev, axis=0) for i in range(7, -1, -1)]
            y = jnp.concatenate([lo] + hi, axis=0)
            y = y + kvo[slot, rows, :].astype(f32) * coef[b, KS:KS + 1, :]
            kvo[slot, rows, :] = (q_buf[sl, rows, :].astype(f32) * y).astype(bf16)

    zero[0] = 0
    for c in range(4):
        w_copy(0, c).start()
        xc_copy(c).start()
        if c == 0:
            for cp in small_copies():
                cp.start()
        else:
            w_copy(1, c - 1).start()

    r = lax.broadcasted_iota(i32, (L2, L2), 0)
    c_ = lax.broadcasted_iota(i32, (L2, L2), 1)
    head = lambda i: jnp.where(i < 2 * M, i // M, (i - 2 * M) // SEG)
    ok = (r < 2 * M) | (c_ < 2 * M) | (c_ <= r)
    fill_ref[...] = jnp.where(head(r) == head(c_),
                              jnp.where(ok, 0.0, -1e9 / scale), -jnp.inf).astype(f32)

    rr = lax.broadcasted_iota(i32, (2 * C, C), 0)
    nn = lax.broadcasted_iota(i32, (2 * C, C), 1)
    kk = 8 * (rr // 16) + rr % 8
    mm = (2 * kk + 1) * (4 * nn + 1) + 4 * C * ((rr // 8) % 2) * (1 + 2 * (kk % 2))
    fm = jnp.cos((mm % (16 * C)).astype(f32) * (math.pi / (8 * C)))
    f_p[...] = pltpu.bitcast(fm.astype(bf16), u32)
    rr = lax.broadcasted_iota(i32, (C, C), 0)
    kk = lax.broadcasted_iota(i32, (C, C), 1)
    mm = (2 * kk + 1) * (2 * (rr % (C // 2)) + 1) + C * (7 - 6 * ((kk + rr // (C // 2)) % 2))
    gm = jnp.cos((mm % (8 * C)).astype(f32) * (math.pi / (4 * C))) * (2 ** -0.5 / C)
    g_p[...] = pltpu.bitcast(gm.astype(bf16), u32)
    for sl in range(2):
        k_buf[sl, 0:KPAD, :] = jnp.zeros((KPAD, 128), bf16)
    uh[0:32] = jnp.zeros((32, 2 * C, 128), f32)

    def pro_body(g, i, tasks):
        r0 = pl.multiple_of(i * 128, 128)
        x = x_buf[pl.ds(r0, 128), :]
        for p in range(8):
            ys = []
            for t in range(2):
                y = jnp.dot(x, wt(g // 2, 16 * (g % 2) + 2 * p + t),
                            preferred_element_type=f32)
                ys.append(y)
                for fn in tasks.get(2 * p + t, ()):
                    fn(y)
            pp = 8 * (g % 2) + p
            ring[pp // 2][pl.ds(pl.multiple_of(QOFF + r0, 64), 128),
                          ring_cols(g // 2, pp)] = jnp.concatenate(ys, axis=1).astype(bf16)

    def add_relayout(tasks, g, c, r):
        for u in range(15):
            def fn(y, u=u):
                stage[g % 3][D + zero[0]] = y[r:r + 16].astype(bf16)
                relayout(g, c, (128 * u) // 15, (128 * (u + 1)) // 15)
            tasks.setdefault(u, []).append(fn)

    def add_wo(tasks, n0):
        for u in range(15):
            def fn(y, u=u):
                wo_st[2048 + zero[0]] = y[96:112].astype(bf16)
                for r in range((64 * u) // 15, (64 * (u + 1)) // 15):
                    wo_pack(n0 + r // 32, 8 * (r % 32), 8 * (r % 32) + 8)
            tasks.setdefault(u, []).append(fn)

    def add_s01(tasks, j):
        for k in range(8):
            def fn(y, k=k):
                coef[NB + zero[0], 0:8, :] = y[48:56]
                s0_kv(0, 0, 0, j, k)
            tasks.setdefault(k, []).append(fn)
        tasks.setdefault(3, []).append(lambda y: s1_h(0, j))
        tasks.setdefault(11, []).append(lambda y: s1_u(0, 0, j))

    def period(g, body):
        if cfg['nopro']:
            return
        with jax.named_scope('pro%d' % g):
            lax.fori_loop(0, 4, lambda i, c: (body(i), c)[1], 0)

    def p0(c):
        @pl.when(c > 0)
        def _():
            w_copy(1, c - 1).wait()
        w_copy(0, c).wait()
        relayout(0, c)
        xc_copy(c).wait()
        xp[...] = pltpu.bitcast(
            x_buf[0:PRE, pl.ds(pl.multiple_of(c * 256, 256), 256)], u32)
        tasks = {}
        add_relayout(tasks, 1, (c + 3) % 4, 0)
        k0 = pl.multiple_of(c * 128, 128)
        for p in range(8):
            ys = []
            for t in range(2):
                hh = 2 * p + t
                w = _bf(wp[0][pl.ds(k0 + hh * HS, 128), :])
                y = (jnp.dot(_bf(xp[...]), w, preferred_element_type=f32)
                     + uh[2 * hh:2 * hh + 2].reshape(PRE, 128))
                uh[2 * hh:2 * hh + 2] = y.reshape(2, 2 * C, 128)
                ys.append(y)
                for fn in tasks.get(hh, ()):
                    fn(y[256 * t:])
            ring[p // 2][QOFF:QOFF + PRE, ring_cols(0, p)] = (
                jnp.concatenate(ys, axis=1).astype(bf16))

        @pl.when(c == 0)
        def _():
            w_copy(1, 3).start()
            for i in range(4):
                w_copy(2, i).start()
    period(0, p0)
    w_copy(1, 3).wait()
    relayout(1, 3)
    for cp in small_copies():
        cp.wait()
    w_copy(3, 0).start()
    w_copy(3, 1).start()
    for cp in kvh_copies(0, 0) + kvh_copies(0, 1):
        cp.start()
    w_copy(4, 0).start()
    w_copy(4, 1).start()
    for c in range(2, 4):
        w_copy(3, c).start()
        w_copy(4, c).start()
    skt = skt_buf[...].astype(f32)
    ddv = dd_buf[...].astype(f32)
    for b in range(NB):
        coef[b, 0:KS, :] = skt[:, b * 128:(b + 1) * 128]
        coef[b, KS:KS + 1, :] = ddv[b:b + 1, :]

    def p1(i):
        w_copy(2, i).wait()
        tasks = {}
        add_relayout(tasks, 2, i, 0)
        pro_body(1, i, tasks)
    period(1, p1)
    for c in range(4):
        w_copy(5, c).start()
        if c < 3:
            wo_copy(2 * c).start()
            wo_copy(2 * c + 1).start()
    for cp in kvh_copies(0, 0) + kvh_copies(0, 1):
        cp.wait()

    def p2(i):
        w_copy(3, i).wait()
        w_copy(4, i).wait()
        tasks = {}
        add_relayout(tasks, 3, i, 0)
        add_relayout(tasks, 4, i, 96)
        add_s01(tasks, i)
        pro_body(2, i, tasks)
    period(2, p2)

    def p3(i):
        @pl.when(i > 0)
        def _():
            wo_copy(2 * i - 2).wait()
            wo_copy(2 * i - 1).wait()
        w_copy(5, i).wait()
        tasks = {}
        add_relayout(tasks, 5, i, 0)
        add_wo(tasks, 2 * ((i + 3) % 4))
        add_s01(tasks, 4 + i)
        pro_body(3, i, tasks)

        @pl.when(i == 0)
        def _():
            wo_copy(6).start()
            wo_copy(7).start()
            x_copy(0).start()
            for cp in kvh_copies(1, 0) + kvh_copies(1, 1):
                cp.start()
            x_copy(1).start()
    period(3, p3)
    for n in (6, 7):
        wo_copy(n).wait()
        wo_pack(n)
    x_copy(0).wait()

    def step(cb, j, mem, par, after_pre):
        s = cb * 8 + j
        x0 = pl.multiple_of(PRE + XR * s, 8)
        wpos = pl.multiple_of(lax.rem(s, RING // XR) * XR, 8)
        rpos = pl.multiple_of(lax.rem(s + QOFF // SEG, RING // SEG) * SEG, 32)
        rbase = pl.multiple_of((s - par) * SEG, 64)
        m0 = 0 if par == 0 else 72
        x8 = 8 + SEG * par

        sl1 = (cb + 1) & 1
        b1 = jnp.minimum(cb + 1, NB - 1)
        slot1 = cb + 1
        b3 = jnp.maximum(cb - 1, 0)
        slot3 = jnp.where(cb == 0, NB, cb - 1)
        s2 = s2_parts(cb & 1, j)
        nu = [0]

        def unit(pace):
            u = nu[0]
            nu[0] += 1
            if u in cfg['s0_at'][par]:
                coef[NB + zero[0], 0:8, :] = pace
                s0_kv(sl1, b1, slot1, j, cfg['s0_at'][par].index(u))
            if u in cfg['s2_at'][par]:
                s2(cfg['s2_at'][par].index(u), pace)

        def proj_q(p, lq):
            ys = []
            for t in range(2):
                ys.append(jnp.dot(lq, wt(2, 2 * p + t), preferred_element_type=f32))
                unit(ys[-1][:M])
            r0, r1 = (0, 48) if par == 0 else (48, 80)
            q_sc[p][r0:r1, :] = jnp.concatenate(ys, axis=1).astype(bf16)

        def proj_kv(p, m, lhs):
            ys = [jnp.dot(lhs, wt(m, 2 * p + t), preferred_element_type=f32)
                  for t in range(2)]
            ring[p // 2][pl.ds(wpos, XR), ring_cols(m, p)] = jnp.concatenate(
                [y[M:] for y in ys], axis=1).astype(bf16)
            unit(ys[0][:M])
            if cfg['mstore']:
                m_sc[2 * p + m] = jnp.concatenate([y[:M] for y in ys], axis=1).astype(bf16)
                return None
            return jnp.concatenate([y[:M] for y in ys], axis=0).astype(bf16)

        def gather(m, p, mm):
            xx = ring[p // 2][pl.ds(rpos, SEG), ring_cols(m, p)]
            if cfg['mstore']:
                mm = jnp.concatenate([m_sc[2 * p + m, :, :DH], m_sc[2 * p + m, :, DH:]], axis=0)
            return jnp.concatenate([mm, xx[:, :DH], xx[:, DH:]], axis=0)

        def qk(p, mems):
            b = q_sc[p]
            q2 = jnp.concatenate([b[m0:m0 + M, :DH], b[m0:m0 + M, DH:],
                                  b[x8:x8 + SEG, :DH], b[x8:x8 + SEG, DH:]], axis=0)
            sc = lax.dot_general(q2, gather(0, p, mems[0]), (((1,), (1,)), ((), ())),
                                 preferred_element_type=f32)
            fill = fill_ref[...]
            sc = jnp.where(fill == 0.0, sc, fill)
            mx = jnp.max(sc, axis=1, keepdims=True)
            if cfg['exp2']:
                e = jnp.exp2((sc - mx) * (scale * math.log2(math.e)))
            else:
                e = jnp.exp((sc - mx) * scale)
            l = jnp.sum(e, axis=1, keepdims=True)
            rc = pl.reciprocal(l, approx=True)
            rc = rc * (2.0 - l * rc)
            pr = (e * rc).astype(bf16)
            if not cfg['pstore']:
                return pr
            p_sc[p] = pltpu.bitcast(pr, u32)

        def pv(p, pr, mems):
            if cfg['pstore']:
                pr = _bf(p_sc[p])
            o = jnp.dot(pr, gather(1, p, mems[1]), preferred_element_type=f32)
            o_sc[p][m0:m0 + M, :] = jnp.concatenate([o[0:M], o[M:2 * M]], axis=1).astype(bf16)
            o_sc[p][x8:x8 + SEG, :] = jnp.concatenate(
                [o[2 * M:2 * M + SEG], o[2 * M + SEG:]], axis=1).astype(bf16)

        accs = [None] * 8
        odots = [(k, n) for k in range(0, H, cfg['och']) for n in range(8)]
        lcache = {}

        def oproj(cnt):
            r0, r1 = (0, 32) if par == 0 else (32, 80)
            for _ in range(min(cnt, len(odots))):
                k, n = odots.pop(0)
                ke = k + cfg['och']
                if k not in lcache:
                    lcache[k] = jnp.concatenate(
                        [o_sc[p][r0:r1, :] for p in range(k // 2, ke // 2)], axis=1)
                y = jnp.dot(lcache[k], _bf(wo_p[n, k * 64:ke * 64, :]),
                            preferred_element_type=f32)
                accs[n] = y if accs[n] is None else y + accs[n]
                unit(accs[n][:M])

        n1 = s + 7
        pre = dict(u=lambda: s1_u((n1 >> 3) & 1, n1 >> 3, n1 & 7),
                   h=lambda: s1_h(sl1, j),
                   y=lambda: s3(sl1, b3, slot3, j))
        for key in cfg['border']:
            pre[key]()
        if after_pre is not None:
            after_pre()

        if par == 0:
            lq = jnp.concatenate([mem, x_buf[pl.ds(rbase, 40), :]], axis=0)
        else:
            lq = jnp.concatenate([x_buf[pl.ds(rbase + 40, 24), :], mem], axis=0)
        for p in range(NPAIR):
            proj_q(p, lq)

        lhs = jnp.concatenate([mem, x_buf[pl.ds(x0, XR), :]], axis=0)
        mems, prs = {}, {}
        att = cfg['att']
        for t in range(max(att) + 1):
            if t < NPAIR:
                mems[t] = [proj_kv(t, m, lhs) for m in range(2)]
            else:
                oproj(cfg['op_per'][par])
            for p in att.get(t, ((), ()))[0]:
                pv(p, prs.pop(p), mems.pop(p))
            for p in att.get(t, ((), ()))[1]:
                prs[p] = qk(p, mems[p])
        oproj(len(odots))
        out = jnp.concatenate(accs, axis=1).astype(bf16)
        if par == 0:
            outb[pl.ds(rbase, 24), :] = out[M:]
            return out[:M]
        outb[pl.ds(rbase + 24, 40), :] = out[:40]
        return out[40:]

    def four_steps(it, carry):
        cb, jj = it >> 1, it & 1

        @pl.when(cb + 1 < NB)
        def _():
            for cp in kvh_copies(cb + 1, jj):
                cp.wait()

        @pl.when(cb >= 1)
        def _():
            q_copy(cb - 1, jj).wait()

        @pl.when(it == 1)
        def _():
            x_copy(1).wait()

        @pl.when(it >= 1)
        def _():
            outa_copy(jnp.maximum(((it - 1) >> 1) - 1, 0), (it - 1) & 1).wait()
            outb_copy(2 * it - 1).start()

        mem = mem_ref[...]
        for u in range(4):
            after = (lambda: outa_copy(jnp.maximum(cb - 1, 0), jj).start()) if u == 3 else None
            mem = step(cb, jj * 4 + u, mem, u % 2, after)
            if u == 1:
                outb_copy(2 * it).start()
        mem_ref[...] = mem

        @pl.when(it + 1 < 2 * NB)
        def _():
            q_copy((it + 1) >> 1, (it + 1) & 1).start()

        @pl.when(cb + 2 < NB)
        def _():
            for cp in kvh_copies(cb + 2, jj):
                cp.start()
        return carry
    q_copy(0, 0).start()
    with jax.named_scope('main'):
        lax.fori_loop(0, 2 * NB, four_steps, 0)

    outb_copy(NSEG // 2 - 1).start()
    q_copy(NB - 1, 0).wait()
    q_copy(NB - 1, 1).wait()
    with jax.named_scope('epi'):
        for j in range(8):
            s3((NB - 1) % 2, NB - 1, NB - 1, j)
            if j % 2 == 1:
                outa_piece(NB - 1, (j - 1) * 2 * C, 4 * C).start()

    outa_copy(NB - 2, 1).wait()
    for pr in range(NSEG // 2):
        outb_copy(pr).wait()
    for j in range(4):
        outa_piece(NB - 1, j * 4 * C, 4 * C).wait()


@functools.partial(jax.jit, static_argnames=("B_seg_len",))
def pallas_concat_heads__ssm_conv_h3__memory_aug_recurrent_mem_tr__prompt_kernel(
    A_q, A_k, A_v, A_shift_k, A_ssm_k, A_ssm_D, B_x, B_mem0, B_Wq, B_Wk, B_Wv, B_Wo,
    B_seg_len=SEG,
):
    assert B_seg_len == SEG
    assert A_q.shape == (1, S, D) and B_x.shape == (1, S, D)
    assert B_Wq.shape == (D, H, DH) and B_mem0.shape == (1, M, D)
    vm = pltpu.VMEM
    dma = pltpu.SemaphoreType.DMA
    scratch = [
        vm((D + 4, 16, DH), bf16), vm((D + 4, 16, DH), bf16),
        vm((D + 4, 16, DH), bf16),
        vm((2048 + 4, 16, 128), bf16),
        vm((8, H * DH // 2, 128), u32),
        vm((S, D), bf16),
        vm((M, D), bf16),
        vm((S, D), bf16),
        vm((NB + 1, 32, 128), f32),
        vm((2, S + 64, 128), bf16),
        vm((2, S, 128), bf16), vm((2, S, 128), bf16),
        vm((2, 128, S), bf16),
        vm((NB + 1, S, 128), bf16),
        vm((4 * NC + 1, 2 * C, 128), f32),
        vm((2, 8, 8, 32, 128), u32),
        vm((8, 32 + KPAD, 128), f32),
        vm((C, C), u32), vm((C // 2, C), u32),
        vm((PRE // 2, 256), u32),
        dma((40,)),
        pltpu.SMEM((1,), i32),
    ]
    scratch += [vm((16 * HS, 128), u32)] * 6
    scratch += [vm((RING, 8 * DH), bf16)] * 8
    scratch += [vm((L2, 2 * DH), bf16)] * (2 * NPAIR)
    scratch += [vm((NPAIR, L2 // 2, L2), u32)]
    scratch += [vm((2 * NPAIR, M, 2 * DH), bf16)]
    scratch += [vm((L2, L2), f32), vm((KS, D), bf16), vm((NB, 128), bf16)]

    out = pl.pallas_call(
        _kernel,
        out_shape=jax.ShapeDtypeStruct((S, 2 * D), bf16),
        in_specs=[pl.BlockSpec(memory_space=pl.ANY)] * 12,
        out_specs=pl.BlockSpec(memory_space=pl.ANY),
        scratch_shapes=scratch,
        compiler_params=pltpu.CompilerParams(vmem_limit_bytes=120 * 1024 * 1024,
                                             disable_bounds_checks=True,
                                             disable_semaphore_checks=True),
        name="ssm_memtr",
    )(A_q.reshape(S, D), A_k.reshape(S, D), A_v.reshape(S, D), A_shift_k.T, A_ssm_k,
      A_ssm_D.reshape(NB, 128), B_x.reshape(S, D), B_mem0.reshape(M, D),
      B_Wq, B_Wk, B_Wv, B_Wo.reshape(H * DH // 16, 16, D))
    return out.reshape(1, S, 2 * D)
```

```python
import math

import jax
import jax.numpy as jnp
from jax import lax
import jax.experimental.pallas as pl
import jax.experimental.pallas.tpu as pltpu

bf16, f32, u32, i32 = jnp.bfloat16, jnp.float32, jnp.uint32, jnp.int32

S = 2048
D = 1024
H, DH = 32, 128
M, SEG = 8, 32
NSEG = S // SEG
KS = 4

XR = 24
PRE = S - NSEG * XR
RING = 576
QOFF = 64
HS = 514
NPAIR = H // 2
L2 = 2 * (M + SEG)
OCH = 8

C = 128
NC = S // C
NB = D // 128
KPAD = 16

CFG = dict(
    att=[(0, 0), (0, 0), (0, 0), (1, 1)], op_per=[4, 3, 4, 4],
    s2_at=[0, 62, 0, 62], s0_at=[17, 78, 17, 78],
    border=['uyh'] * 4, nopro=False,
)


def _bf(x):
    return pltpu.bitcast(x, bf16)


def _kernel(q_hbm, k_hbm, v_hbm, skt_hbm, h_hbm, dd_hbm, x_hbm, mem0_hbm,
            wq_hbm, wk_hbm, wv_hbm, wo_hbm, out_hbm,
            st0, st1, st2, wo_st, wo_p, x_buf, mem_ref, outb,
            coef, k_buf, v_buf, q_buf, h_buf, kvo,
            uh, y_buf, kf, f_p, g_p, xp, sems, zero,
            *bufs):
    wp = bufs[0:6]
    ring = bufs[6:14]
    o_sc = bufs[14:30]
    q_sc = bufs[30:46]
    p_sc, m_sc, fill_ref, skt_buf, dd_buf = bufs[46:51]
    stage = (st0, st1, st2)
    w_hbm = (wk_hbm, wv_hbm, wq_hbm)
    scale = DH ** -0.5
    cfg = CFG
    SW, SWO, SX, SSM, SKVH, SQ, SOUT = 0, 12, 20, 26, 29, 33, 37

    def w_copy(g, c):
        r0 = c * 256
        return pltpu.make_async_copy(
            w_hbm[g // 2].at[pl.ds(r0, 256), pl.ds(16 * (g % 2), 16), :],
            stage[g % 3].at[pl.ds(r0, 256)],
            sems.at[SW + (g % 3) * 4 + c])

    def wo_copy(n):
        return pltpu.make_async_copy(
            wo_hbm.at[:, :, pl.ds(pl.multiple_of(n * 128, 128), 128)],
            wo_st.at[pl.ds(n * 256, 256)], sems.at[SWO + n])

    def xc_copy(c):
        cols = pl.ds(pl.multiple_of(c * 256, 256), 256)
        return pltpu.make_async_copy(x_hbm.at[pl.ds(0, PRE), cols],
                                     x_buf.at[pl.ds(0, PRE), cols], sems.at[SX + c])

    def x_copy(part):
        r0, n = ((PRE, 128), (PRE + 128, S - PRE - 128))[part]
        return pltpu.make_async_copy(
            x_hbm.at[pl.ds(r0, n)], x_buf.at[pl.ds(r0, n)], sems.at[SX + 4 + part])

    def small_copies():
        return [pltpu.make_async_copy(skt_hbm, skt_buf, sems.at[SSM + 0]),
                pltpu.make_async_copy(dd_hbm, dd_buf, sems.at[SSM + 1]),
                pltpu.make_async_copy(mem0_hbm, mem_ref, sems.at[SSM + 2])]

    def col(b):
        return pl.ds(pl.multiple_of(b * 128, 128), 128)

    HALF = S // 2

    def half_rows(half, off=0):
        return pl.ds(pl.multiple_of(half * HALF, HALF) + off, HALF)

    def kvh_copies(b, half):
        sl, t = b & 1, half_rows(half)
        sem = sems.at[SKVH + 2 * sl + half]
        return [pltpu.make_async_copy(k_hbm.at[t, col(b)],
                                      k_buf.at[sl, half_rows(half, KPAD)], sem),
                pltpu.make_async_copy(v_hbm.at[t, col(b)], v_buf.at[sl, t], sem),
                pltpu.make_async_copy(h_hbm.at[col(b), t], h_buf.at[sl, :, t], sem)]

    def q_copy(b, half):
        sl, t = b & 1, half_rows(half)
        return pltpu.make_async_copy(q_hbm.at[t, col(b)], q_buf.at[sl, t],
                                     sems.at[SQ + 2 * sl + half])

    def outa_copy(b, half):
        t = half_rows(half)
        return pltpu.make_async_copy(kvo.at[b, t], out_hbm.at[t, col(b)], sems.at[SOUT])

    def outa_piece(b, r0, n):
        return pltpu.make_async_copy(kvo.at[b, pl.ds(r0, n)],
                                     out_hbm.at[pl.ds(r0, n), col(b)], sems.at[SOUT + 1])

    def outb_copy(pr):
        rows = pl.ds(pl.multiple_of(pr * 2 * SEG, 2 * SEG), 2 * SEG)
        return pltpu.make_async_copy(outb.at[rows], out_hbm.at[rows, pl.ds(D, D)],
                                     sems.at[SOUT + 2])

    def relayout(g, c, lo_i=0, hi_i=128):
        src, dst = stage[g % 3], wp[g]
        d0 = c * 256
        for i in range(lo_i, hi_i):
            a = pltpu.bitcast(src[d0 + 2 * i], u32)
            b = pltpu.bitcast(src[d0 + 2 * i + 1], u32)
            lo = (a & jnp.uint32(0xFFFF)) | (b << 16)
            hi = (a >> 16) | (b & jnp.uint32(0xFFFF0000))
            row = c * 128 + i
            dst[pl.ds(row, 8, stride=2 * HS), :] = lo
            dst[pl.ds(row + HS, 8, stride=2 * HS), :] = hi

    def wo_pack(n, r0=0, r1=256):
        for r in range(r0, r1, 8):
            blk = pltpu.bitcast(wo_st[pl.ds(n * 256 + r, 8)], u32)
            wo_p[n, r * 8:(r + 8) * 8, :] = blk.reshape(64, 128)

    def wt(m, h):
        g, hh = 2 * m + h // 16, h % 16
        return _bf(wp[g][hh * HS:hh * HS + D // 2, :])

    def ring_cols(m, p):
        c0 = 512 * m + 256 * (p % 2)
        return slice(c0, c0 + 256)

    def s0_kv(sl, b, slot, j, i):
        t0 = pl.multiple_of(j * 2 * C, 2 * C)
        kw = k_buf.at[sl, pl.ds(t0, 2 * C + KPAD)]
        vw = v_buf.at[sl, pl.ds(t0, 2 * C)]
        ow = kvo.at[slot, pl.ds(t0, 2 * C)]
        kf[i] = kw[32 * i:32 * i + 32 + KPAD, :].astype(f32)
        acc = None
        for tap in range(KS):
            term = kf[i, KPAD - tap:KPAD - tap + 32, :] * coef[b, tap:tap + 1, :]
            acc = term if acc is None else acc + term
        ow[32 * i:32 * i + 32, :] = (acc * vw[32 * i:32 * i + 32, :].astype(f32)).astype(bf16)

    def s1_h(sl, j):
        for t in range(2):
            a = 2 * j + t
            hh = h_buf[sl, :, pl.ds(pl.multiple_of(a * C, C), C)]
            for half in range(2):
                fm = _bf(f_p[half * 64:(half + 1) * 64, :])
                uh[sl * 2 * NC + NC + a, half * C:(half + 1) * C, :] = lax.dot_general(
                    fm, hh, (((1,), (1,)), ((), ())), preferred_element_type=f32)

    def s1_u(sl, slot, j):
        for t in range(2):
            a = 2 * j + t
            kv = kvo[slot, pl.ds(pl.multiple_of(a * C, C), C), :]
            for half in range(2):
                fm = _bf(f_p[half * 64:(half + 1) * 64, :])
                uh[sl * 2 * NC + a, half * C:(half + 1) * C, :] = jnp.dot(
                    fm, kv, preferred_element_type=f32)

    def s2_parts(sl, j):
        u0 = sl * 2 * NC
        h0 = u0 + NC
        r0 = pl.multiple_of(j * 32, 32)
        prev = []

        def one(idx, pace):
            grp, a = divmod(idx, NC)
            re, im = pl.ds(r0 + 16 * grp, 8), pl.ds(r0 + 16 * grp + 8, 8)
            yr = yi = None
            for b in range(a + 1):
                if b == a:
                    uh[4 * NC + zero[0], 0:8, :] = pace
                ur, ui = uh[u0 + b, re, :], uh[u0 + b, im, :]
                hr, hi = uh[h0 + a - b, re, :], uh[h0 + a - b, im, :]
                yr = ur * hr if yr is None else yr + ur * hr
                yi = ur * hi if yi is None else yi + ur * hi
                yr = yr - ui * hi
                yi = yi + ui * hr
            pp, qq = yr - yi, yr + yi
            if a > 0:
                zp, zq = pp - prev[1], qq + prev[0]
            else:
                zp, zq = pp, qq
            prev[:] = [pp, qq]
            z = pltpu.bitcast(jnp.concatenate([zp, zq], axis=0).astype(bf16), u32)
            r = (a % 2) * 16 + 4 * grp
            y_buf[sl, j, a // 2, r:r + 4, :] = z[0:4]
            y_buf[sl, j, a // 2, r + 8:r + 12, :] = z[4:8]
        return one

    def s3(sl, b, slot, j):
        rev = 7 - lax.broadcasted_iota(i32, (8, 128), 0)
        for t in range(2):
            a = 2 * j + t
            rows = pl.ds(pl.multiple_of(a * C, C), C)
            eo = []
            for part in range(2):
                r = 16 * t + 8 * part
                yp = y_buf[sl, :, j, r:r + 8, :].reshape(C // 2, 128)
                eo.append(jnp.dot(_bf(g_p[part * 32:(part + 1) * 32, :]), _bf(yp),
                                  preferred_element_type=f32))
            lo, hi = eo[0] + eo[1], eo[0] - eo[1]
            hi = [jnp.take_along_axis(hi[8 * i:8 * i + 8], rev, axis=0) for i in range(7, -1, -1)]
            y = jnp.concatenate([lo] + hi, axis=0)
            y = y + kvo[slot, rows, :].astype(f32) * coef[b, KS:KS + 1, :]
            kvo[slot, rows, :] = (q_buf[sl, rows, :].astype(f32) * y).astype(bf16)

    zero[0] = 0
    for c in range(4):
        w_copy(0, c).start()
        xc_copy(c).start()
        if c == 0:
            for cp in small_copies():
                cp.start()
        else:
            w_copy(1, c - 1).start()

    r = lax.broadcasted_iota(i32, (L2, L2), 0)
    c_ = lax.broadcasted_iota(i32, (L2, L2), 1)
    head = lambda i: jnp.where(i < 2 * M, i // M, (i - 2 * M) // SEG)
    ok = (r < 2 * M) | (c_ < 2 * M) | (c_ <= r)
    fill_ref[...] = jnp.where(head(r) == head(c_),
                              jnp.where(ok, 0.0, -1e9 / scale), -jnp.inf).astype(f32)

    rr = lax.broadcasted_iota(i32, (2 * C, C), 0)
    nn = lax.broadcasted_iota(i32, (2 * C, C), 1)
    kk = 8 * (rr // 16) + rr % 8
    mm = (2 * kk + 1) * (4 * nn + 1) + 4 * C * ((rr // 8) % 2) * (1 + 2 * (kk % 2))
    fm = jnp.cos((mm % (16 * C)).astype(f32) * (math.pi / (8 * C)))
    f_p[...] = pltpu.bitcast(fm.astype(bf16), u32)
    rr = lax.broadcasted_iota(i32, (C, C), 0)
    kk = lax.broadcasted_iota(i32, (C, C), 1)
    mm = (2 * kk + 1) * (2 * (rr % (C // 2)) + 1) + C * (7 - 6 * ((kk + rr // (C // 2)) % 2))
    gm = jnp.cos((mm % (8 * C)).astype(f32) * (math.pi / (4 * C))) * (2 ** -0.5 / C)
    g_p[...] = pltpu.bitcast(gm.astype(bf16), u32)
    for sl in range(2):
        k_buf[sl, 0:KPAD, :] = jnp.zeros((KPAD, 128), bf16)
    uh[0:32] = jnp.zeros((32, 2 * C, 128), f32)

    def pro_body(g, i, tasks):
        r0 = pl.multiple_of(i * 128, 128)
        x = x_buf[pl.ds(r0, 128), :]
        for p in range(8):
            ys = []
            for t in range(2):
                y = jnp.dot(x, wt(g // 2, 16 * (g % 2) + 2 * p + t),
                            preferred_element_type=f32)
                ys.append(y)
                for fn in tasks.get(2 * p + t, ()):
                    fn(y)
            pp = 8 * (g % 2) + p
            ring[pp // 2][pl.ds(pl.multiple_of(QOFF + r0, 64), 128),
                          ring_cols(g // 2, pp)] = jnp.concatenate(ys, axis=1).astype(bf16)

    def add_relayout(tasks, g, c, r):
        for u in range(15):
            def fn(y, u=u):
                stage[g % 3][D + zero[0]] = y[r:r + 16].astype(bf16)
                relayout(g, c, (128 * u) // 15, (128 * (u + 1)) // 15)
            tasks.setdefault(u, []).append(fn)

    def add_wo(tasks, n0):
        for u in range(15):
            def fn(y, u=u):
                wo_st[2048 + zero[0]] = y[96:112].astype(bf16)
                for r in range((64 * u) // 15, (64 * (u + 1)) // 15):
                    wo_pack(n0 + r // 32, 8 * (r % 32), 8 * (r % 32) + 8)
            tasks.setdefault(u, []).append(fn)

    def add_s01(tasks, j):
        for k in range(8):
            def fn(y, k=k):
                coef[NB + zero[0], 0:8, :] = y[48:56]
                s0_kv(0, 0, 0, j, k)
            tasks.setdefault(k, []).append(fn)
        tasks.setdefault(3, []).append(lambda y: s1_h(0, j))
        tasks.setdefault(11, []).append(lambda y: s1_u(0, 0, j))

    def period(g, body):
        if cfg['nopro']:
            return
        with jax.named_scope('pro%d' % g):
            lax.fori_loop(0, 4, lambda i, c: (body(i), c)[1], 0)

    def p0(c):
        @pl.when(c > 0)
        def _():
            w_copy(1, c - 1).wait()
        w_copy(0, c).wait()
        relayout(0, c)
        xc_copy(c).wait()
        xp[...] = pltpu.bitcast(
            x_buf[0:PRE, pl.ds(pl.multiple_of(c * 256, 256), 256)], u32)
        tasks = {}
        add_relayout(tasks, 1, (c + 3) % 4, 0)
        k0 = pl.multiple_of(c * 128, 128)
        for p in range(8):
            ys = []
            for t in range(2):
                hh = 2 * p + t
                w = _bf(wp[0][pl.ds(k0 + hh * HS, 128), :])
                y = (jnp.dot(_bf(xp[...]), w, preferred_element_type=f32)
                     + uh[2 * hh:2 * hh + 2].reshape(PRE, 128))
                uh[2 * hh:2 * hh + 2] = y.reshape(2, 2 * C, 128)
                ys.append(y)
                for fn in tasks.get(hh, ()):
                    fn(y[256 * t:])
            ring[p // 2][QOFF:QOFF + PRE, ring_cols(0, p)] = (
                jnp.concatenate(ys, axis=1).astype(bf16))

        @pl.when(c == 0)
        def _():
            w_copy(1, 3).start()
            for i in range(4):
                w_copy(2, i).start()
    period(0, p0)
    w_copy(1, 3).wait()
    relayout(1, 3)
    for cp in small_copies():
        cp.wait()
    w_copy(3, 0).start()
    w_copy(3, 1).start()
    for cp in kvh_copies(0, 0) + kvh_copies(0, 1):
        cp.start()
    w_copy(4, 0).start()
    w_copy(4, 1).start()
    for c in range(2, 4):
        w_copy(3, c).start()
        w_copy(4, c).start()
    skt = skt_buf[...].astype(f32)
    ddv = dd_buf[...].astype(f32)
    for b in range(NB):
        coef[b, 0:KS, :] = skt[:, b * 128:(b + 1) * 128]
        coef[b, KS:KS + 1, :] = ddv[b:b + 1, :]

    def p1(i):
        w_copy(2, i).wait()
        tasks = {}
        add_relayout(tasks, 2, i, 0)
        pro_body(1, i, tasks)
    period(1, p1)
    for c in range(4):
        w_copy(5, c).start()
        if c < 3:
            wo_copy(2 * c).start()
            wo_copy(2 * c + 1).start()
    for cp in kvh_copies(0, 0) + kvh_copies(0, 1):
        cp.wait()

    def p2(i):
        w_copy(3, i).wait()
        w_copy(4, i).wait()
        tasks = {}
        add_relayout(tasks, 3, i, 0)
        add_relayout(tasks, 4, i, 96)
        add_s01(tasks, i)
        pro_body(2, i, tasks)
    period(2, p2)

    def p3(i):
        @pl.when(i > 0)
        def _():
            wo_copy(2 * i - 2).wait()
            wo_copy(2 * i - 1).wait()
        w_copy(5, i).wait()
        tasks = {}
        add_relayout(tasks, 5, i, 0)
        add_wo(tasks, 2 * ((i + 3) % 4))
        add_s01(tasks, 4 + i)
        pro_body(3, i, tasks)

        @pl.when(i == 0)
        def _():
            wo_copy(6).start()
            wo_copy(7).start()
            x_copy(0).start()
            for cp in kvh_copies(1, 0) + kvh_copies(1, 1):
                cp.start()
            x_copy(1).start()
    period(3, p3)
    for n in (6, 7):
        wo_copy(n).wait()
        wo_pack(n)
    x_copy(0).wait()

    def step(cb, j, mem, u4, after_pre):
        par = u4 % 2
        s = cb * 8 + j
        x0 = pl.multiple_of(PRE + XR * s, 8)
        wpos = pl.multiple_of(lax.rem(s, RING // XR) * XR, 8)
        rpos = pl.multiple_of(lax.rem(s + QOFF // SEG, RING // SEG) * SEG, 32)
        rbase = pl.multiple_of((s - par) * SEG, 64)
        m0 = 0 if par == 0 else 72
        x8 = 8 + SEG * par

        sl1 = (cb + 1) & 1
        b1 = jnp.minimum(cb + 1, NB - 1)
        slot1 = cb + 1
        b3 = jnp.maximum(cb - 1, 0)
        slot3 = jnp.where(cb == 0, NB, cb - 1)
        s2 = s2_parts(cb & 1, j)
        nu = [0]

        def unit(pace):
            u = nu[0]
            nu[0] += 1
            if 0 <= u - cfg['s0_at'][u4] < 8:
                coef[NB + zero[0], 0:8, :] = pace
                s0_kv(sl1, b1, slot1, j, u - cfg['s0_at'][u4])
            if 0 <= u - cfg['s2_at'][u4] < 2 * NC:
                s2(u - cfg['s2_at'][u4], pace)

        def proj_q(p, lq):
            ys = []
            for t in range(2):
                ys.append(jnp.dot(lq, wt(2, 2 * p + t), preferred_element_type=f32))
                unit(ys[-1][:M])
            r0, r1 = (0, 48) if par == 0 else (48, 80)
            q_sc[p][r0:r1, :] = jnp.concatenate(ys, axis=1).astype(bf16)

        def proj_kv(p, m, lhs):
            ys = [jnp.dot(lhs, wt(m, 2 * p + t), preferred_element_type=f32)
                  for t in range(2)]
            ring[p // 2][pl.ds(wpos, XR), ring_cols(m, p)] = jnp.concatenate(
                [y[M:] for y in ys], axis=1).astype(bf16)
            unit(ys[0][:M])
            m_sc[2 * p + m] = jnp.concatenate([y[:M] for y in ys], axis=1).astype(bf16)

        def gather(m, p):
            xx = ring[p // 2][pl.ds(rpos, SEG), ring_cols(m, p)]
            mm = jnp.concatenate([m_sc[2 * p + m, :, :DH], m_sc[2 * p + m, :, DH:]], axis=0)
            return jnp.concatenate([mm, xx[:, :DH], xx[:, DH:]], axis=0)

        def qk(p):
            b = q_sc[p]
            q2 = jnp.concatenate([b[m0:m0 + M, :DH], b[m0:m0 + M, DH:],
                                  b[x8:x8 + SEG, :DH], b[x8:x8 + SEG, DH:]], axis=0)
            sc = lax.dot_general(q2, gather(0, p), (((1,), (1,)), ((), ())),
                                 preferred_element_type=f32)
            fill = fill_ref[...]
            sc = jnp.where(fill == 0.0, sc, fill)
            mx = jnp.max(sc, axis=1, keepdims=True)
            e = jnp.exp((sc - mx) * scale)
            l = jnp.sum(e, axis=1, keepdims=True)
            rc = pl.reciprocal(l, approx=True)
            rc = rc * (2.0 - l * rc)
            p_sc[p] = pltpu.bitcast((e * rc).astype(bf16), u32)

        def pv(p):
            o = jnp.dot(_bf(p_sc[p]), gather(1, p), preferred_element_type=f32)
            o_sc[p][m0:m0 + M, :] = jnp.concatenate([o[0:M], o[M:2 * M]], axis=1).astype(bf16)
            o_sc[p][x8:x8 + SEG, :] = jnp.concatenate(
                [o[2 * M:2 * M + SEG], o[2 * M + SEG:]], axis=1).astype(bf16)

        accs = [None] * 8
        odots = [(k, n) for k in range(0, H, OCH) for n in range(8)]
        lcache = {}

        def oproj(cnt):
            r0, r1 = (0, 32) if par == 0 else (32, 80)
            for _ in range(min(cnt, len(odots))):
                k, n = odots.pop(0)
                ke = k + OCH
                if k not in lcache:
                    lcache[k] = jnp.concatenate(
                        [o_sc[p][r0:r1, :] for p in range(k // 2, ke // 2)], axis=1)
                y = jnp.dot(lcache[k], _bf(wo_p[n, k * 64:ke * 64, :]),
                            preferred_element_type=f32)
                accs[n] = y if accs[n] is None else y + accs[n]
                unit(accs[n][:M])

        n1 = s + 7
        pre = dict(u=lambda: s1_u((n1 >> 3) & 1, n1 >> 3, n1 & 7),
                   h=lambda: s1_h(sl1, j),
                   y=lambda: s3(sl1, b3, slot3, j))
        for key in cfg['border'][u4]:
            pre[key]()
        if after_pre is not None:
            after_pre()

        if par == 0:
            lq = jnp.concatenate([mem, x_buf[pl.ds(rbase, 40), :]], axis=0)
        else:
            lq = jnp.concatenate([x_buf[pl.ds(rbase + 40, 24), :], mem], axis=0)
        for p in range(NPAIR):
            proj_q(p, lq)

        lhs = jnp.concatenate([mem, x_buf[pl.ds(x0, XR), :]], axis=0)
        a0, a1 = cfg['att'][u4]
        att = {4 + a0: ([], [0, 1, 2, 3]), 18 + a1: ([12, 13, 14, 15], []),
               **{t + a0: ([t - 6, t - 5], [t - 2, t - 1]) for t in range(6, 18, 2)}}
        for t in range(max(att) + 1):
            if t < NPAIR:
                for m in range(2):
                    proj_kv(t, m, lhs)
            else:
                oproj(cfg['op_per'][u4])
            pvs, qks = att.get(t, ((), ()))
            for p in pvs:
                pv(p)
            for p in qks:
                qk(p)
        oproj(len(odots))
        out = jnp.concatenate(accs, axis=1).astype(bf16)
        if par == 0:
            outb[pl.ds(rbase, 24), :] = out[M:]
            return out[:M]
        outb[pl.ds(rbase + 24, 40), :] = out[:40]
        return out[40:]

    def four_steps(it, carry):
        cb, jj = it >> 1, it & 1

        @pl.when(cb + 1 < NB)
        def _():
            for cp in kvh_copies(cb + 1, jj):
                cp.wait()

        @pl.when(cb >= 1)
        def _():
            q_copy(cb - 1, jj).wait()

        @pl.when(it == 1)
        def _():
            x_copy(1).wait()

        @pl.when(it >= 1)
        def _():
            outa_copy(jnp.maximum(((it - 1) >> 1) - 1, 0), (it - 1) & 1).wait()
            outb_copy(2 * it - 1).start()

        mem = mem_ref[...]
        for u in range(4):
            after = (lambda: outa_copy(jnp.maximum(cb - 1, 0), jj).start()) if u == 3 else None
            mem = step(cb, jj * 4 + u, mem, u, after)
            if u == 1:
                outb_copy(2 * it).start()
        mem_ref[...] = mem

        @pl.when(it + 1 < 2 * NB)
        def _():
            q_copy((it + 1) >> 1, (it + 1) & 1).start()

        @pl.when(cb + 2 < NB)
        def _():
            for cp in kvh_copies(cb + 2, jj):
                cp.start()
        return carry
    q_copy(0, 0).start()
    with jax.named_scope('main'):
        lax.fori_loop(0, 2 * NB, four_steps, 0)

    outb_copy(NSEG // 2 - 1).start()
    q_copy(NB - 1, 0).wait()
    q_copy(NB - 1, 1).wait()
    with jax.named_scope('epi'):
        for j in range(8):
            s3((NB - 1) % 2, NB - 1, NB - 1, j)
            if j % 2 == 1:
                outa_piece(NB - 1, (j - 1) * 2 * C, 4 * C).start()

    outa_copy(NB - 2, 1).wait()
    for pr in range(NSEG // 2):
        outb_copy(pr).wait()
    for j in range(4):
        outa_piece(NB - 1, j * 4 * C, 4 * C).wait()


@jax.jit
def pallas_concat_heads__ssm_conv_h3__memory_aug_recurrent_mem_tr__prompt_kernel(
    A_q, A_k, A_v, A_shift_k, A_ssm_k, A_ssm_D, B_x, B_mem0, B_Wq, B_Wk, B_Wv, B_Wo,
    B_seg_len,
):
    del B_seg_len
    assert A_q.shape == (1, S, D) and B_x.shape == (1, S, D)
    assert B_Wq.shape == (D, H, DH) and B_mem0.shape == (1, M, D)
    vm = pltpu.VMEM
    dma = pltpu.SemaphoreType.DMA
    scratch = [
        vm((D + 4, 16, DH), bf16), vm((D + 4, 16, DH), bf16),
        vm((D + 4, 16, DH), bf16),
        vm((2048 + 4, 16, 128), bf16),
        vm((8, H * DH // 2, 128), u32),
        vm((S, D), bf16),
        vm((M, D), bf16),
        vm((S, D), bf16),
        vm((NB + 1, 32, 128), f32),
        vm((2, S + 64, 128), bf16),
        vm((2, S, 128), bf16), vm((2, S, 128), bf16),
        vm((2, 128, S), bf16),
        vm((NB + 1, S, 128), bf16),
        vm((4 * NC + 1, 2 * C, 128), f32),
        vm((2, 8, 8, 32, 128), u32),
        vm((8, 32 + KPAD, 128), f32),
        vm((C, C), u32), vm((C // 2, C), u32),
        vm((PRE // 2, 256), u32),
        dma((40,)),
        pltpu.SMEM((1,), i32),
    ]
    scratch += [vm((16 * HS, 128), u32)] * 6
    scratch += [vm((RING, 8 * DH), bf16)] * 8
    scratch += [vm((L2, 2 * DH), bf16)] * (2 * NPAIR)
    scratch += [vm((NPAIR, L2 // 2, L2), u32)]
    scratch += [vm((2 * NPAIR, M, 2 * DH), bf16)]
    scratch += [vm((L2, L2), f32), vm((KS, D), bf16), vm((NB, 128), bf16)]

    out = pl.pallas_call(
        _kernel,
        out_shape=jax.ShapeDtypeStruct((S, 2 * D), bf16),
        in_specs=[pl.BlockSpec(memory_space=pl.ANY)] * 12,
        out_specs=pl.BlockSpec(memory_space=pl.ANY),
        scratch_shapes=scratch,
        compiler_params=pltpu.CompilerParams(vmem_limit_bytes=120 * 1024 * 1024,
                                             disable_bounds_checks=True,
                                             disable_semaphore_checks=True),
        name="ssm_memtr",
    )(A_q.reshape(S, D), A_k.reshape(S, D), A_v.reshape(S, D), A_shift_k.T, A_ssm_k,
      A_ssm_D.reshape(NB, 128), B_x.reshape(S, D), B_mem0.reshape(M, D),
      B_Wq, B_Wk, B_Wv, B_Wo.reshape(H * DH // 16, 16, D))
    return out.reshape(1, S, 2 * D)
```

```python
import math

import jax
import jax.numpy as jnp
from jax import lax
import jax.experimental.pallas as pl
import jax.experimental.pallas.tpu as pltpu

bf16, f32, u32, i32 = jnp.bfloat16, jnp.float32, jnp.uint32, jnp.int32

S = 2048
D = 1024
H, DH = 32, 128
M, SEG = 8, 32
NSEG = S // SEG
KS = 4

XR = 24
PRE = S - NSEG * XR
RING = 576
QOFF = 64
HS = 514
NPAIR = H // 2
L2 = 2 * (M + SEG)
OCH = 8
WOP = 76

C = 128
NC = S // C
NB = D // 128
KPAD = 16

CFG = dict(
    att=[(0, 0), (0, 0), (0, 0), (1, 1)], op_per=[4, 3, 4, 4],
    s2_at=[0, 62, 0, 62], s0_at=[17, 78, 17, 78],
    border=['uyh'] * 4, nopro=False,
)


def _bf(x):
    return pltpu.bitcast(x, bf16)


def _kernel(q_hbm, k_hbm, v_hbm, skt_hbm, h_hbm, dd_hbm, x_hbm, mem0_hbm,
            wq_hbm, wk_hbm, wv_hbm, wo_hbm, out_hbm,
            st0, st1, st2, wo_st, wo_p, x_buf, mem_ref, outb,
            coef, k_buf, v_buf, q_buf, h_buf, kvo,
            uh, y_buf, kf, f_p, g_p, xp, sems, zero,
            *bufs):
    wp = bufs[0:6]
    ring = bufs[6:14]
    o_sc = bufs[14:30]
    q_sc = bufs[30:46]
    p_sc, m_sc, fill_ref, skt_buf, dd_buf = bufs[46:51]
    stage = (st0, st1, st2)
    w_hbm = (wk_hbm, wv_hbm, wq_hbm)
    scale = DH ** -0.5
    cfg = CFG
    SW, SWO, SX, SSM, SKVH, SQ, SOUT = 0, 12, 20, 26, 29, 33, 37

    def w_copy(g, c):
        r0 = c * 256
        return pltpu.make_async_copy(
            w_hbm[g // 2].at[pl.ds(r0, 256), pl.ds(16 * (g % 2), 16), :],
            stage[g % 3].at[pl.ds(r0, 256)],
            sems.at[SW + (g % 3) * 4 + c])

    def wo_copy(part, n=WOP):
        rows = pl.ds(part * WOP, n)
        return pltpu.make_async_copy(wo_hbm.at[rows], wo_st.at[rows], sems.at[SWO + part])

    def xc_copy(c):
        cols = pl.ds(pl.multiple_of(c * 256, 256), 256)
        return pltpu.make_async_copy(x_hbm.at[pl.ds(0, PRE), cols],
                                     x_buf.at[pl.ds(0, PRE), cols], sems.at[SX + c])

    def x_copy(part):
        r0, n = ((PRE, 128), (PRE + 128, S - PRE - 128))[part]
        return pltpu.make_async_copy(
            x_hbm.at[pl.ds(r0, n)], x_buf.at[pl.ds(r0, n)], sems.at[SX + 4 + part])

    def small_copies():
        return [pltpu.make_async_copy(skt_hbm, skt_buf, sems.at[SSM + 0]),
                pltpu.make_async_copy(dd_hbm, dd_buf, sems.at[SSM + 1]),
                pltpu.make_async_copy(mem0_hbm, mem_ref, sems.at[SSM + 2])]

    def col(b):
        return pl.ds(pl.multiple_of(b * 128, 128), 128)

    HALF = S // 2

    def half_rows(half, off=0):
        return pl.ds(pl.multiple_of(half * HALF, HALF) + off, HALF)

    def kvh_copies(b, half):
        sl, t = b & 1, half_rows(half)
        sem = sems.at[SKVH + 2 * sl + half]
        return [pltpu.make_async_copy(k_hbm.at[t, col(b)],
                                      k_buf.at[sl, half_rows(half, KPAD)], sem),
                pltpu.make_async_copy(v_hbm.at[t, col(b)], v_buf.at[sl, t], sem),
                pltpu.make_async_copy(h_hbm.at[col(b), t], h_buf.at[sl, :, t], sem)]

    def q_copy(b, half):
        sl, t = b & 1, half_rows(half)
        return pltpu.make_async_copy(q_hbm.at[t, col(b)], q_buf.at[sl, t],
                                     sems.at[SQ + 2 * sl + half])

    def outa_copy(b, half):
        t = half_rows(half)
        return pltpu.make_async_copy(kvo.at[b, t], out_hbm.at[t, col(b)], sems.at[SOUT])

    def outa_piece(b, r0, n):
        return pltpu.make_async_copy(kvo.at[b, pl.ds(r0, n)],
                                     out_hbm.at[pl.ds(r0, n), col(b)], sems.at[SOUT + 1])

    def outb_copy(pr):
        rows = pl.ds(pl.multiple_of(pr * 2 * SEG, 2 * SEG), 2 * SEG)
        return pltpu.make_async_copy(outb.at[rows], out_hbm.at[rows, pl.ds(D, D)],
                                     sems.at[SOUT + 2])

    def relayout(g, c, lo_i=0, hi_i=128):
        src, dst = stage[g % 3], wp[g]
        d0 = c * 256
        for i in range(lo_i, hi_i):
            a = pltpu.bitcast(src[d0 + 2 * i], u32)
            b = pltpu.bitcast(src[d0 + 2 * i + 1], u32)
            lo = (a & jnp.uint32(0xFFFF)) | (b << 16)
            hi = (a >> 16) | (b & jnp.uint32(0xFFFF0000))
            row = c * 128 + i
            dst[pl.ds(row, 8, stride=2 * HS), :] = lo
            dst[pl.ds(row + HS, 8, stride=2 * HS), :] = hi

    def wo_pack(part, r0, r1):
        for r in range(r0, r1):
            blk = pltpu.bitcast(wo_st[part * WOP + r], u32)
            rows = pl.ds(pl.multiple_of((part * WOP + r) * 8, 8), 8)
            for n in range(8):
                wo_p[n, rows, :] = blk[:, n * 128:(n + 1) * 128]

    def wt(m, h):
        g, hh = 2 * m + h // 16, h % 16
        return _bf(wp[g][hh * HS:hh * HS + D // 2, :])

    def ring_cols(m, p):
        c0 = 512 * m + 256 * (p % 2)
        return slice(c0, c0 + 256)

    def s0_kv(sl, b, slot, j, i):
        t0 = pl.multiple_of(j * 2 * C, 2 * C)
        kw = k_buf.at[sl, pl.ds(t0, 2 * C + KPAD)]
        vw = v_buf.at[sl, pl.ds(t0, 2 * C)]
        ow = kvo.at[slot, pl.ds(t0, 2 * C)]
        kf[i] = kw[32 * i:32 * i + 32 + KPAD, :].astype(f32)
        acc = None
        for tap in range(KS):
            term = kf[i, KPAD - tap:KPAD - tap + 32, :] * coef[b, tap:tap + 1, :]
            acc = term if acc is None else acc + term
        ow[32 * i:32 * i + 32, :] = (acc * vw[32 * i:32 * i + 32, :].astype(f32)).astype(bf16)

    def s1_h(sl, j):
        for t in range(2):
            a = 2 * j + t
            hh = h_buf[sl, :, pl.ds(pl.multiple_of(a * C, C), C)]
            for half in range(2):
                fm = _bf(f_p[half * 64:(half + 1) * 64, :])
                uh[sl * 2 * NC + NC + a, half * C:(half + 1) * C, :] = lax.dot_general(
                    fm, hh, (((1,), (1,)), ((), ())), preferred_element_type=f32)

    def s1_u(sl, slot, j):
        for t in range(2):
            a = 2 * j + t
            kv = kvo[slot, pl.ds(pl.multiple_of(a * C, C), C), :]
            for half in range(2):
                fm = _bf(f_p[half * 64:(half + 1) * 64, :])
                uh[sl * 2 * NC + a, half * C:(half + 1) * C, :] = jnp.dot(
                    fm, kv, preferred_element_type=f32)

    def s2_parts(sl, j):
        u0 = sl * 2 * NC
        h0 = u0 + NC
        r0 = pl.multiple_of(j * 32, 32)
        prev = []

        def one(idx, pace):
            grp, a = divmod(idx, NC)
            re, im = pl.ds(r0 + 16 * grp, 8), pl.ds(r0 + 16 * grp + 8, 8)
            yr = yi = None
            for b in range(a + 1):
                if b == a:
                    uh[4 * NC + zero[0], 0:8, :] = pace
                ur, ui = uh[u0 + b, re, :], uh[u0 + b, im, :]
                hr, hi = uh[h0 + a - b, re, :], uh[h0 + a - b, im, :]
                yr = ur * hr if yr is None else yr + ur * hr
                yi = ur * hi if yi is None else yi + ur * hi
                yr = yr - ui * hi
                yi = yi + ui * hr
            pp, qq = yr - yi, yr + yi
            if a > 0:
                zp, zq = pp - prev[1], qq + prev[0]
            else:
                zp, zq = pp, qq
            prev[:] = [pp, qq]
            z = pltpu.bitcast(jnp.concatenate([zp, zq], axis=0).astype(bf16), u32)
            r = (a % 2) * 16 + 4 * grp
            y_buf[sl, j, a // 2, r:r + 4, :] = z[0:4]
            y_buf[sl, j, a // 2, r + 8:r + 12, :] = z[4:8]
        return one

    def s3(sl, b, slot, j):
        rev = 7 - lax.broadcasted_iota(i32, (8, 128), 0)
        for t in range(2):
            a = 2 * j + t
            rows = pl.ds(pl.multiple_of(a * C, C), C)
            eo = []
            for part in range(2):
                r = 16 * t + 8 * part
                yp = y_buf[sl, :, j, r:r + 8, :].reshape(C // 2, 128)
                eo.append(jnp.dot(_bf(g_p[part * 32:(part + 1) * 32, :]), _bf(yp),
                                  preferred_element_type=f32))
            lo, hi = eo[0] + eo[1], eo[0] - eo[1]
            hi = [jnp.take_along_axis(hi[8 * i:8 * i + 8], rev, axis=0) for i in range(7, -1, -1)]
            y = jnp.concatenate([lo] + hi, axis=0)
            y = y + kvo[slot, rows, :].astype(f32) * coef[b, KS:KS + 1, :]
            kvo[slot, rows, :] = (q_buf[sl, rows, :].astype(f32) * y).astype(bf16)

    zero[0] = 0
    for c in range(4):
        w_copy(0, c).start()
        xc_copy(c).start()
        if c == 0:
            for cp in small_copies():
                cp.start()
        else:
            w_copy(1, c - 1).start()

    r = lax.broadcasted_iota(i32, (L2, L2), 0)
    c_ = lax.broadcasted_iota(i32, (L2, L2), 1)
    head = lambda i: jnp.where(i < 2 * M, i // M, (i - 2 * M) // SEG)
    ok = (r < 2 * M) | (c_ < 2 * M) | (c_ <= r)
    fill_ref[...] = jnp.where(head(r) == head(c_),
                              jnp.where(ok, 0.0, -1e9 / scale), -jnp.inf).astype(f32)

    rr = lax.broadcasted_iota(i32, (2 * C, C), 0)
    nn = lax.broadcasted_iota(i32, (2 * C, C), 1)
    kk = 8 * (rr // 16) + rr % 8
    mm = (2 * kk + 1) * (4 * nn + 1) + 4 * C * ((rr // 8) % 2) * (1 + 2 * (kk % 2))
    fm = jnp.cos((mm % (16 * C)).astype(f32) * (math.pi / (8 * C)))
    f_p[...] = pltpu.bitcast(fm.astype(bf16), u32)
    rr = lax.broadcasted_iota(i32, (C, C), 0)
    kk = lax.broadcasted_iota(i32, (C, C), 1)
    mm = (2 * kk + 1) * (2 * (rr % (C // 2)) + 1) + C * (7 - 6 * ((kk + rr // (C // 2)) % 2))
    gm = jnp.cos((mm % (8 * C)).astype(f32) * (math.pi / (4 * C))) * (2 ** -0.5 / C)
    g_p[...] = pltpu.bitcast(gm.astype(bf16), u32)
    for sl in range(2):
        k_buf[sl, 0:KPAD, :] = jnp.zeros((KPAD, 128), bf16)
    uh[0:32] = jnp.zeros((32, 2 * C, 128), f32)

    def pro_body(g, i, tasks):
        r0 = pl.multiple_of(i * 128, 128)
        x = x_buf[pl.ds(r0, 128), :]
        for p in range(8):
            ys = []
            for t in range(2):
                y = jnp.dot(x, wt(g // 2, 16 * (g % 2) + 2 * p + t),
                            preferred_element_type=f32)
                ys.append(y)
                for fn in tasks.get(2 * p + t, ()):
                    fn(y)
            pp = 8 * (g % 2) + p
            ring[pp // 2][pl.ds(pl.multiple_of(QOFF + r0, 64), 128),
                          ring_cols(g // 2, pp)] = jnp.concatenate(ys, axis=1).astype(bf16)

    def add_relayout(tasks, g, c, r):
        for u in range(15):
            def fn(y, u=u):
                stage[g % 3][D + zero[0]] = y[r:r + 16].astype(bf16)
                relayout(g, c, (128 * u) // 15, (128 * (u + 1)) // 15)
            tasks.setdefault(u, []).append(fn)

    def add_wo(tasks, part):
        for u in range(15):
            def fn(y, u=u):
                wo_st[256 + zero[0], :, 0:128] = y[96:112].astype(bf16)
                wo_pack(part, (WOP * u) // 15, (WOP * (u + 1)) // 15)
            tasks.setdefault(u, []).append(fn)

    def add_s01(tasks, j):
        for k in range(8):
            def fn(y, k=k):
                coef[NB + zero[0], 0:8, :] = y[48:56]
                s0_kv(0, 0, 0, j, k)
            tasks.setdefault(k, []).append(fn)
        tasks.setdefault(3, []).append(lambda y: s1_h(0, j))
        tasks.setdefault(11, []).append(lambda y: s1_u(0, 0, j))

    def period(g, body):
        if cfg['nopro']:
            return
        with jax.named_scope('pro%d' % g):
            lax.fori_loop(0, 4, lambda i, c: (body(i), c)[1], 0)

    def p0(c):
        @pl.when(c > 0)
        def _():
            w_copy(1, c - 1).wait()
        w_copy(0, c).wait()
        relayout(0, c)
        xc_copy(c).wait()
        xp[...] = pltpu.bitcast(
            x_buf[0:PRE, pl.ds(pl.multiple_of(c * 256, 256), 256)], u32)
        tasks = {}
        add_relayout(tasks, 1, (c + 3) % 4, 0)
        k0 = pl.multiple_of(c * 128, 128)
        for p in range(8):
            ys = []
            for t in range(2):
                hh = 2 * p + t
                w = _bf(wp[0][pl.ds(k0 + hh * HS, 128), :])
                y = (jnp.dot(_bf(xp[...]), w, preferred_element_type=f32)
                     + uh[2 * hh:2 * hh + 2].reshape(PRE, 128))
                uh[2 * hh:2 * hh + 2] = y.reshape(2, 2 * C, 128)
                ys.append(y)
                for fn in tasks.get(hh, ()):
                    fn(y[256 * t:])
            ring[p // 2][QOFF:QOFF + PRE, ring_cols(0, p)] = (
                jnp.concatenate(ys, axis=1).astype(bf16))

        @pl.when(c == 0)
        def _():
            w_copy(1, 3).start()
            for i in range(4):
                w_copy(2, i).start()
    period(0, p0)
    w_copy(1, 3).wait()
    relayout(1, 3)
    for cp in small_copies():
        cp.wait()
    w_copy(3, 0).start()
    w_copy(3, 1).start()
    for cp in kvh_copies(0, 0) + kvh_copies(0, 1):
        cp.start()
    w_copy(4, 0).start()
    w_copy(4, 1).start()
    for c in range(2, 4):
        w_copy(3, c).start()
        w_copy(4, c).start()
    skt = skt_buf[...].astype(f32)
    ddv = dd_buf[...].astype(f32)
    for b in range(NB):
        coef[b, 0:KS, :] = skt[:, b * 128:(b + 1) * 128]
        coef[b, KS:KS + 1, :] = ddv[b:b + 1, :]

    def p1(i):
        w_copy(2, i).wait()
        tasks = {}
        add_relayout(tasks, 2, i, 0)
        pro_body(1, i, tasks)
    period(1, p1)
    w_copy(5, 0).start()
    for c in range(2):
        w_copy(5, c + 1).start()
        wo_copy(c).start()
    w_copy(5, 3).start()
    for cp in kvh_copies(0, 0) + kvh_copies(0, 1):
        cp.wait()

    def p2(i):
        w_copy(3, i).wait()
        w_copy(4, i).wait()
        tasks = {}
        add_relayout(tasks, 3, i, 0)
        add_relayout(tasks, 4, i, 96)
        add_s01(tasks, i)
        pro_body(2, i, tasks)
    period(2, p2)

    def p3(i):
        @pl.when(i > 0)
        def _():
            wo_copy(i - 1).wait()
        w_copy(5, i).wait()
        tasks = {}
        add_relayout(tasks, 5, i, 0)
        add_wo(tasks, jnp.where(i == 0, 2, i - 1))
        add_s01(tasks, 4 + i)
        pro_body(3, i, tasks)

        @pl.when(i == 0)
        def _():
            wo_copy(2).start()
            wo_copy(3, 256 - 3 * WOP).start()
            x_copy(0).start()
            for cp in kvh_copies(1, 0) + kvh_copies(1, 1):
                cp.start()
            x_copy(1).start()
    period(3, p3)
    wo_copy(3, 256 - 3 * WOP).wait()
    wo_pack(3, 0, 256 - 3 * WOP)
    x_copy(0).wait()

    def step(cb, j, mem, u4, after_pre):
        par = u4 % 2
        s = cb * 8 + j
        x0 = pl.multiple_of(PRE + XR * s, 8)
        wpos = pl.multiple_of(lax.rem(s, RING // XR) * XR, 8)
        rpos = pl.multiple_of(lax.rem(s + QOFF // SEG, RING // SEG) * SEG, 32)
        rbase = pl.multiple_of((s - par) * SEG, 64)
        m0 = 0 if par == 0 else 72
        x8 = 8 + SEG * par

        sl1 = (cb + 1) & 1
        b1 = jnp.minimum(cb + 1, NB - 1)
        slot1 = cb + 1
        b3 = jnp.maximum(cb - 1, 0)
        slot3 = jnp.where(cb == 0, NB, cb - 1)
        s2 = s2_parts(cb & 1, j)
        nu = [0]

        def unit(pace):
            u = nu[0]
            nu[0] += 1
            if 0 <= u - cfg['s0_at'][u4] < 8:
                coef[NB + zero[0], 0:8, :] = pace
                s0_kv(sl1, b1, slot1, j, u - cfg['s0_at'][u4])
            if 0 <= u - cfg['s2_at'][u4] < 2 * NC:
                s2(u - cfg['s2_at'][u4], pace)

        def proj_q(p, lq):
            ys = []
            for t in range(2):
                ys.append(jnp.dot(lq, wt(2, 2 * p + t), preferred_element_type=f32))
                unit(ys[-1][:M])
            r0, r1 = (0, 48) if par == 0 else (48, 80)
            q_sc[p][r0:r1, :] = jnp.concatenate(ys, axis=1).astype(bf16)

        def proj_kv(p, m, lhs):
            ys = [jnp.dot(lhs, wt(m, 2 * p + t), preferred_element_type=f32)
                  for t in range(2)]
            ring[p // 2][pl.ds(wpos, XR), ring_cols(m, p)] = jnp.concatenate(
                [y[M:] for y in ys], axis=1).astype(bf16)
            unit(ys[0][:M])
            m_sc[2 * p + m] = jnp.concatenate([y[:M] for y in ys], axis=1).astype(bf16)

        def gather(m, p):
            xx = ring[p // 2][pl.ds(rpos, SEG), ring_cols(m, p)]
            mm = jnp.concatenate([m_sc[2 * p + m, :, :DH], m_sc[2 * p + m, :, DH:]], axis=0)
            return jnp.concatenate([mm, xx[:, :DH], xx[:, DH:]], axis=0)

        def qk(p):
            b = q_sc[p]
            q2 = jnp.concatenate([b[m0:m0 + M, :DH], b[m0:m0 + M, DH:],
                                  b[x8:x8 + SEG, :DH], b[x8:x8 + SEG, DH:]], axis=0)
            sc = lax.dot_general(q2, gather(0, p), (((1,), (1,)), ((), ())),
                                 preferred_element_type=f32)
            fill = fill_ref[...]
            sc = jnp.where(fill == 0.0, sc, fill)
            mx = jnp.max(sc, axis=1, keepdims=True)
            e = jnp.exp((sc - mx) * scale)
            l = jnp.sum(e, axis=1, keepdims=True)
            rc = pl.reciprocal(l, approx=True)
            rc = rc * (2.0 - l * rc)
            p_sc[p] = pltpu.bitcast((e * rc).astype(bf16), u32)

        def pv(p):
            o = jnp.dot(_bf(p_sc[p]), gather(1, p), preferred_element_type=f32)
            o_sc[p][m0:m0 + M, :] = jnp.concatenate([o[0:M], o[M:2 * M]], axis=1).astype(bf16)
            o_sc[p][x8:x8 + SEG, :] = jnp.concatenate(
                [o[2 * M:2 * M + SEG], o[2 * M + SEG:]], axis=1).astype(bf16)

        accs = [None] * 8
        odots = [(k, n) for k in range(0, H, OCH) for n in range(8)]
        lcache = {}

        def oproj(cnt):
            r0, r1 = (0, 32) if par == 0 else (32, 80)
            for _ in range(min(cnt, len(odots))):
                k, n = odots.pop(0)
                ke = k + OCH
                if k not in lcache:
                    lcache[k] = jnp.concatenate(
                        [o_sc[p][r0:r1, :] for p in range(k // 2, ke // 2)], axis=1)
                y = jnp.dot(lcache[k], _bf(wo_p[n, k * 64:ke * 64, :]),
                            preferred_element_type=f32)
                accs[n] = y if accs[n] is None else y + accs[n]
                unit(accs[n][:M])

        n1 = s + 7
        pre = dict(u=lambda: s1_u((n1 >> 3) & 1, n1 >> 3, n1 & 7),
                   h=lambda: s1_h(sl1, j),
                   y=lambda: s3(sl1, b3, slot3, j))
        for key in cfg['border'][u4]:
            pre[key]()
        if after_pre is not None:
            after_pre()

        if par == 0:
            lq = jnp.concatenate([mem, x_buf[pl.ds(rbase, 40), :]], axis=0)
        else:
            lq = jnp.concatenate([x_buf[pl.ds(rbase + 40, 24), :], mem], axis=0)
        for p in range(NPAIR):
            proj_q(p, lq)

        lhs = jnp.concatenate([mem, x_buf[pl.ds(x0, XR), :]], axis=0)
        a0, a1 = cfg['att'][u4]
        att = {4 + a0: ([], [0, 1, 2, 3]), 18 + a1: ([12, 13, 14, 15], []),
               **{t + a0: ([t - 6, t - 5], [t - 2, t - 1]) for t in range(6, 18, 2)}}
        for t in range(max(att) + 1):
            if t < NPAIR:
                for m in range(2):
                    proj_kv(t, m, lhs)
            else:
                oproj(cfg['op_per'][u4])
            pvs, qks = att.get(t, ((), ()))
            for p in pvs:
                pv(p)
            for p in qks:
                qk(p)
        oproj(len(odots))
        out = jnp.concatenate(accs, axis=1).astype(bf16)
        if par == 0:
            outb[pl.ds(rbase, 24), :] = out[M:]
            return out[:M]
        outb[pl.ds(rbase + 24, 40), :] = out[:40]
        return out[40:]

    def four_steps(it, carry):
        cb, jj = it >> 1, it & 1

        @pl.when(cb + 1 < NB)
        def _():
            for cp in kvh_copies(cb + 1, jj):
                cp.wait()

        @pl.when(cb >= 1)
        def _():
            q_copy(cb - 1, jj).wait()

        @pl.when(it == 1)
        def _():
            x_copy(1).wait()

        @pl.when(it >= 1)
        def _():
            outa_copy(jnp.maximum(((it - 1) >> 1) - 1, 0), (it - 1) & 1).wait()
            outb_copy(2 * it - 1).start()

        mem = mem_ref[...]
        for u in range(4):
            after = (lambda: outa_copy(jnp.maximum(cb - 1, 0), jj).start()) if u == 3 else None
            mem = step(cb, jj * 4 + u, mem, u, after)
            if u == 1:
                outb_copy(2 * it).start()
        mem_ref[...] = mem

        @pl.when(it + 1 < 2 * NB)
        def _():
            q_copy((it + 1) >> 1, (it + 1) & 1).start()

        @pl.when(cb + 2 < NB)
        def _():
            for cp in kvh_copies(cb + 2, jj):
                cp.start()
        return carry
    q_copy(0, 0).start()
    with jax.named_scope('main'):
        lax.fori_loop(0, 2 * NB, four_steps, 0)

    outb_copy(NSEG // 2 - 1).start()
    q_copy(NB - 1, 0).wait()
    q_copy(NB - 1, 1).wait()
    with jax.named_scope('epi'):
        for j in range(8):
            s3((NB - 1) % 2, NB - 1, NB - 1, j)
            if j % 2 == 1:
                outa_piece(NB - 1, (j - 1) * 2 * C, 4 * C).start()

    outa_copy(NB - 2, 1).wait()
    for pr in range(NSEG // 2):
        outb_copy(pr).wait()
    for j in range(4):
        outa_piece(NB - 1, j * 4 * C, 4 * C).wait()


@jax.jit
def pallas_concat_heads__ssm_conv_h3__memory_aug_recurrent_mem_tr__prompt_kernel(
    A_q, A_k, A_v, A_shift_k, A_ssm_k, A_ssm_D, B_x, B_mem0, B_Wq, B_Wk, B_Wv, B_Wo,
    B_seg_len,
):
    del B_seg_len
    assert A_q.shape == (1, S, D) and B_x.shape == (1, S, D)
    assert B_Wq.shape == (D, H, DH) and B_mem0.shape == (1, M, D)
    vm = pltpu.VMEM
    dma = pltpu.SemaphoreType.DMA
    scratch = [
        vm((D + 4, 16, DH), bf16), vm((D + 4, 16, DH), bf16),
        vm((D + 4, 16, DH), bf16),
        vm((256 + 1, 16, D), bf16),
        vm((8, H * DH // 2, 128), u32),
        vm((S, D), bf16),
        vm((M, D), bf16),
        vm((S, D), bf16),
        vm((NB + 1, 32, 128), f32),
        vm((2, S + 64, 128), bf16),
        vm((2, S, 128), bf16), vm((2, S, 128), bf16),
        vm((2, 128, S), bf16),
        vm((NB + 1, S, 128), bf16),
        vm((4 * NC + 1, 2 * C, 128), f32),
        vm((2, 8, 8, 32, 128), u32),
        vm((8, 32 + KPAD, 128), f32),
        vm((C, C), u32), vm((C // 2, C), u32),
        vm((PRE // 2, 256), u32),
        dma((40,)),
        pltpu.SMEM((1,), i32),
    ]
    scratch += [vm((16 * HS, 128), u32)] * 6
    scratch += [vm((RING, 8 * DH), bf16)] * 8
    scratch += [vm((L2, 2 * DH), bf16)] * (2 * NPAIR)
    scratch += [vm((NPAIR, L2 // 2, L2), u32)]
    scratch += [vm((2 * NPAIR, M, 2 * DH), bf16)]
    scratch += [vm((L2, L2), f32), vm((KS, D), bf16), vm((NB, 128), bf16)]

    out = pl.pallas_call(
        _kernel,
        out_shape=jax.ShapeDtypeStruct((S, 2 * D), bf16),
        in_specs=[pl.BlockSpec(memory_space=pl.ANY)] * 12,
        out_specs=pl.BlockSpec(memory_space=pl.ANY),
        scratch_shapes=scratch,
        compiler_params=pltpu.CompilerParams(vmem_limit_bytes=120 * 1024 * 1024,
                                             disable_bounds_checks=True,
                                             disable_semaphore_checks=True),
        name="ssm_memtr",
    )(A_q.reshape(S, D), A_k.reshape(S, D), A_v.reshape(S, D), A_shift_k.T, A_ssm_k,
      A_ssm_D.reshape(NB, 128), B_x.reshape(S, D), B_mem0.reshape(M, D),
      B_Wq, B_Wk, B_Wv, B_Wo.reshape(H * DH // 16, 16, D))
    return out.reshape(1, S, 2 * D)
```

```python
import math

import jax
import jax.numpy as jnp
from jax import lax
import jax.experimental.pallas as pl
import jax.experimental.pallas.tpu as pltpu

bf16, f32, u32, i32 = jnp.bfloat16, jnp.float32, jnp.uint32, jnp.int32

S = 2048
D = 1024
H, DH = 32, 128
M, SEG = 8, 32
NSEG = S // SEG
KS = 4

XR = 24
PRE = S - NSEG * XR
RING = 576
QOFF = 64
HS = 514
NPAIR = H // 2
L2 = 2 * (M + SEG)
OCH = 8
WOP = 76

C = 128
NC = S // C
NB = D // 128
KPAD = 16

CFG = dict(
    att=[(0, 0), (0, 0), (0, 0), (1, 1)], op_per=[4, 3, 4, 4],
    s2_at=[0, 62, 0, 62], s0_at=[17, 78, 17, 78],
    border=['uyh'] * 4, nopro=False,
)


def _bf(x):
    return pltpu.bitcast(x, bf16)


def _kernel(q_hbm, k_hbm, v_hbm, skt_hbm, h_hbm, dd_hbm, x_hbm, mem0_hbm,
            wq_hbm, wk_hbm, wv_hbm, wo_hbm, out_hbm,
            st0, st1, st2, wo_st, wo_p, x_buf, mem_ref, outb,
            coef, k_buf, v_buf, q_buf, h_buf, kvo,
            uh, y_buf, kf, f_p, g_p, xp, sems, zero,
            *bufs):
    wp = bufs[0:6]
    ring = bufs[6:14]
    o_sc = bufs[14:30]
    q_sc = bufs[30:46]
    p_sc, m_sc, fill_ref, skt_buf, dd_buf = bufs[46:51]
    stage = (st0, st1, st2)
    w_hbm = (wk_hbm, wv_hbm, wq_hbm)
    scale = DH ** -0.5
    cfg = CFG
    SW, SWO, SX, SSM, SKVH, SQ, SOUT = 0, 12, 20, 26, 29, 33, 37

    def w_copy(g, c):
        r0 = c * 256
        return pltpu.make_async_copy(
            w_hbm[g // 2].at[pl.ds(r0, 256), pl.ds(16 * (g % 2), 16), :],
            stage[g % 3].at[pl.ds(r0, 256)],
            sems.at[SW + (g % 3) * 4 + c])

    def wo_copy(part, n=WOP):
        rows = pl.ds(part * WOP, n)
        return pltpu.make_async_copy(wo_hbm.at[rows], wo_st.at[rows], sems.at[SWO + part])

    def xc_copy(c):
        cols = pl.ds(pl.multiple_of(c * 256, 256), 256)
        return pltpu.make_async_copy(x_hbm.at[pl.ds(0, PRE), cols],
                                     x_buf.at[pl.ds(0, PRE), cols], sems.at[SX + c])

    def x_copy(part):
        r0, n = ((PRE, 128), (PRE + 128, S - PRE - 128))[part]
        return pltpu.make_async_copy(
            x_hbm.at[pl.ds(r0, n)], x_buf.at[pl.ds(r0, n)], sems.at[SX + 4 + part])

    def small_copies():
        return [pltpu.make_async_copy(skt_hbm, skt_buf, sems.at[SSM + 0]),
                pltpu.make_async_copy(dd_hbm, dd_buf, sems.at[SSM + 1]),
                pltpu.make_async_copy(mem0_hbm, mem_ref, sems.at[SSM + 2])]

    def col(b):
        return pl.ds(pl.multiple_of(b * 128, 128), 128)

    HALF = S // 2

    def half_rows(half, off=0):
        return pl.ds(pl.multiple_of(half * HALF, HALF) + off, HALF)

    def kvh_copies(b, half):
        sl, t = b & 1, half_rows(half)
        sem = sems.at[SKVH + 2 * sl + half]
        return [pltpu.make_async_copy(k_hbm.at[t, col(b)],
                                      k_buf.at[sl, half_rows(half, KPAD)], sem),
                pltpu.make_async_copy(v_hbm.at[t, col(b)], v_buf.at[sl, t], sem),
                pltpu.make_async_copy(h_hbm.at[col(b), t], h_buf.at[sl, :, t], sem)]

    def q_copy(b, half):
        sl, t = b & 1, half_rows(half)
        return pltpu.make_async_copy(q_hbm.at[t, col(b)], q_buf.at[sl, t],
                                     sems.at[SQ + 2 * sl + half])

    def outa_copy(b, half):
        t = half_rows(half)
        return pltpu.make_async_copy(kvo.at[b, t], out_hbm.at[t, col(b)], sems.at[SOUT])

    def outa_piece(b, r0, n):
        return pltpu.make_async_copy(kvo.at[b, pl.ds(r0, n)],
                                     out_hbm.at[pl.ds(r0, n), col(b)], sems.at[SOUT + 1])

    def outb_copy(pr):
        rows = pl.ds(pl.multiple_of(pr * 2 * SEG, 2 * SEG), 2 * SEG)
        return pltpu.make_async_copy(outb.at[rows], out_hbm.at[rows, pl.ds(D, D)],
                                     sems.at[SOUT + 2])

    def relayout(g, c, lo_i=0, hi_i=128):
        src, dst = stage[g % 3], wp[g]
        d0 = c * 256
        for i in range(lo_i, hi_i):
            a = pltpu.bitcast(src[d0 + 2 * i], u32)
            b = pltpu.bitcast(src[d0 + 2 * i + 1], u32)
            lo = (a & jnp.uint32(0xFFFF)) | (b << 16)
            hi = (a >> 16) | (b & jnp.uint32(0xFFFF0000))
            row = c * 128 + i
            dst[pl.ds(row, 8, stride=2 * HS), :] = lo
            dst[pl.ds(row + HS, 8, stride=2 * HS), :] = hi

    def wo_pack(part, r0, r1):
        for r in range(r0, r1):
            blk = pltpu.bitcast(wo_st[part * WOP + r], u32)
            rows = pl.ds(pl.multiple_of((part * WOP + r) * 8, 8), 8)
            for n in range(8):
                wo_p[n, rows, :] = blk[:, n * 128:(n + 1) * 128]

    def wt(m, h):
        g, hh = 2 * m + h // 16, h % 16
        return _bf(wp[g][hh * HS:hh * HS + D // 2, :])

    def ring_cols(m, p):
        c0 = 512 * m + 256 * (p % 2)
        return slice(c0, c0 + 256)

    def s0_kv(sl, b, slot, j, i):
        t0 = pl.multiple_of(j * 2 * C, 2 * C)
        kw = k_buf.at[sl, pl.ds(t0, 2 * C + KPAD)]
        vw = v_buf.at[sl, pl.ds(t0, 2 * C)]
        ow = kvo.at[slot, pl.ds(t0, 2 * C)]
        kf[i] = kw[32 * i:32 * i + 32 + KPAD, :].astype(f32)
        acc = None
        for tap in range(KS):
            term = kf[i, KPAD - tap:KPAD - tap + 32, :] * coef[b, tap:tap + 1, :]
            acc = term if acc is None else acc + term
        ow[32 * i:32 * i + 32, :] = (acc * vw[32 * i:32 * i + 32, :].astype(f32)).astype(bf16)

    def s1_h(sl, j):
        for t in range(2):
            a = 2 * j + t
            hh = h_buf[sl, :, pl.ds(pl.multiple_of(a * C, C), C)]
            for half in range(2):
                fm = _bf(f_p[half * 64:(half + 1) * 64, :])
                uh[sl * 2 * NC + NC + a, half * C:(half + 1) * C, :] = lax.dot_general(
                    fm, hh, (((1,), (1,)), ((), ())), preferred_element_type=f32)

    def s1_u(sl, slot, j):
        for t in range(2):
            a = 2 * j + t
            kv = kvo[slot, pl.ds(pl.multiple_of(a * C, C), C), :]
            for half in range(2):
                fm = _bf(f_p[half * 64:(half + 1) * 64, :])
                uh[sl * 2 * NC + a, half * C:(half + 1) * C, :] = jnp.dot(
                    fm, kv, preferred_element_type=f32)

    def s2_parts(sl, j):
        u0 = sl * 2 * NC
        h0 = u0 + NC
        r0 = pl.multiple_of(j * 32, 32)
        prev = []

        def one(idx, pace):
            grp, a = divmod(idx, NC)
            re, im = pl.ds(r0 + 16 * grp, 8), pl.ds(r0 + 16 * grp + 8, 8)
            yr = yi = None
            for b in range(a + 1):
                if b == a:
                    uh[4 * NC + zero[0], 0:8, :] = pace
                ur, ui = uh[u0 + b, re, :], uh[u0 + b, im, :]
                hr, hi = uh[h0 + a - b, re, :], uh[h0 + a - b, im, :]
                yr = ur * hr if yr is None else yr + ur * hr
                yi = ur * hi if yi is None else yi + ur * hi
                yr = yr - ui * hi
                yi = yi + ui * hr
            pp, qq = yr - yi, yr + yi
            if a > 0:
                zp, zq = pp - prev[1], qq + prev[0]
            else:
                zp, zq = pp, qq
            prev[:] = [pp, qq]
            z = pltpu.bitcast(jnp.concatenate([zp, zq], axis=0).astype(bf16), u32)
            r = (a % 2) * 16 + 4 * grp
            y_buf[sl, j, a // 2, r:r + 4, :] = z[0:4]
            y_buf[sl, j, a // 2, r + 8:r + 12, :] = z[4:8]
        return one

    def s3(sl, b, slot, j):
        rev = 7 - lax.broadcasted_iota(i32, (8, 128), 0)
        for t in range(2):
            a = 2 * j + t
            rows = pl.ds(pl.multiple_of(a * C, C), C)
            eo = []
            for part in range(2):
                r = 16 * t + 8 * part
                yp = y_buf[sl, :, j, r:r + 8, :].reshape(C // 2, 128)
                eo.append(jnp.dot(_bf(g_p[part * 32:(part + 1) * 32, :]), _bf(yp),
                                  preferred_element_type=f32))
            lo, hi = eo[0] + eo[1], eo[0] - eo[1]
            hi = [jnp.take_along_axis(hi[8 * i:8 * i + 8], rev, axis=0) for i in range(7, -1, -1)]
            y = jnp.concatenate([lo] + hi, axis=0)
            y = y + kvo[slot, rows, :].astype(f32) * coef[b, KS:KS + 1, :]
            kvo[slot, rows, :] = (q_buf[sl, rows, :].astype(f32) * y).astype(bf16)

    zero[0] = 0
    for c in range(4):
        w_copy(0, c).start()
        xc_copy(c).start()
        if c == 0:
            for cp in small_copies():
                cp.start()
        else:
            w_copy(1, c - 1).start()

    r = lax.broadcasted_iota(i32, (L2, L2), 0)
    c_ = lax.broadcasted_iota(i32, (L2, L2), 1)
    head = lambda i: jnp.where(i < 2 * M, i // M, (i - 2 * M) // SEG)
    ok = (r < 2 * M) | (c_ < 2 * M) | (c_ <= r)
    fill_ref[...] = jnp.where(head(r) == head(c_),
                              jnp.where(ok, 0.0, -1e9 / scale), -jnp.inf).astype(f32)

    rr = lax.broadcasted_iota(i32, (2 * C, C), 0)
    nn = lax.broadcasted_iota(i32, (2 * C, C), 1)
    kk = 8 * (rr // 16) + rr % 8
    mm = (2 * kk + 1) * (4 * nn + 1) + 4 * C * ((rr // 8) % 2) * (1 + 2 * (kk % 2))
    fm = jnp.cos((mm % (16 * C)).astype(f32) * (math.pi / (8 * C)))
    f_p[...] = pltpu.bitcast(fm.astype(bf16), u32)
    rr = lax.broadcasted_iota(i32, (C, C), 0)
    kk = lax.broadcasted_iota(i32, (C, C), 1)
    mm = (2 * kk + 1) * (2 * (rr % (C // 2)) + 1) + C * (7 - 6 * ((kk + rr // (C // 2)) % 2))
    gm = jnp.cos((mm % (8 * C)).astype(f32) * (math.pi / (4 * C))) * (2 ** -0.5 / C)
    g_p[...] = pltpu.bitcast(gm.astype(bf16), u32)
    for sl in range(2):
        k_buf[sl, 0:KPAD, :] = jnp.zeros((KPAD, 128), bf16)
    uh[0:32] = jnp.zeros((32, 2 * C, 128), f32)

    def pro_body(g, i, tasks):
        r0 = pl.multiple_of(i * 128, 128)
        x = x_buf[pl.ds(r0, 128), :]
        for p in range(8):
            ys = []
            for t in range(2):
                y = jnp.dot(x, wt(g // 2, 16 * (g % 2) + 2 * p + t),
                            preferred_element_type=f32)
                ys.append(y)
                for fn in tasks.get(2 * p + t, ()):
                    fn(y)
            pp = 8 * (g % 2) + p
            ring[pp // 2][pl.ds(pl.multiple_of(QOFF + r0, 64), 128),
                          ring_cols(g // 2, pp)] = jnp.concatenate(ys, axis=1).astype(bf16)

    def add_relayout(tasks, g, c, r):
        for u in range(15):
            def fn(y, u=u):
                stage[g % 3][D + zero[0]] = y[r:r + 16].astype(bf16)
                relayout(g, c, (128 * u) // 15, (128 * (u + 1)) // 15)
            tasks.setdefault(u, []).append(fn)

    def add_wo(tasks, part):
        for u in range(15):
            def fn(y, u=u):
                wo_st[256 + zero[0], :, 0:128] = y[96:112].astype(bf16)
                wo_pack(part, (WOP * u) // 15, (WOP * (u + 1)) // 15)
            tasks.setdefault(u, []).append(fn)

    def add_s01(tasks, j, with_u=True):
        for k in range(8):
            def fn(y, k=k):
                coef[NB + zero[0], 0:8, :] = y[48:56]
                s0_kv(0, 0, 0, j, k)
            tasks.setdefault(k, []).append(fn)
        tasks.setdefault(3, []).append(lambda y: s1_h(0, j))
        if with_u:
            tasks.setdefault(11, []).append(lambda y: s1_u(0, 0, j))

    def period(g, body):
        if cfg['nopro']:
            return
        with jax.named_scope('pro%d' % g):
            lax.fori_loop(0, 4, lambda i, c: (body(i), c)[1], 0)

    def p0(c):
        @pl.when(c > 0)
        def _():
            w_copy(1, c - 1).wait()
        w_copy(0, c).wait()
        relayout(0, c)
        xc_copy(c).wait()
        xp[...] = pltpu.bitcast(
            x_buf[0:PRE, pl.ds(pl.multiple_of(c * 256, 256), 256)], u32)
        tasks = {}
        add_relayout(tasks, 1, (c + 3) % 4, 0)
        k0 = pl.multiple_of(c * 128, 128)
        for p in range(8):
            ys = []
            for t in range(2):
                hh = 2 * p + t
                w = _bf(wp[0][pl.ds(k0 + hh * HS, 128), :])
                y = (jnp.dot(_bf(xp[...]), w, preferred_element_type=f32)
                     + uh[2 * hh:2 * hh + 2].reshape(PRE, 128))
                uh[2 * hh:2 * hh + 2] = y.reshape(2, 2 * C, 128)
                ys.append(y)
                for fn in tasks.get(hh, ()):
                    fn(y[256 * t:])
            ring[p // 2][QOFF:QOFF + PRE, ring_cols(0, p)] = (
                jnp.concatenate(ys, axis=1).astype(bf16))

        @pl.when(c == 0)
        def _():
            w_copy(1, 3).start()
            for i in range(4):
                w_copy(2, i).start()
    period(0, p0)
    w_copy(1, 3).wait()
    relayout(1, 3)
    for cp in small_copies():
        cp.wait()
    w_copy(3, 0).start()
    w_copy(3, 1).start()
    for cp in kvh_copies(0, 0) + kvh_copies(0, 1):
        cp.start()
    w_copy(4, 0).start()
    w_copy(4, 1).start()
    for c in range(2, 4):
        w_copy(3, c).start()
        w_copy(4, c).start()
    skt = skt_buf[...].astype(f32)
    ddv = dd_buf[...].astype(f32)
    for b in range(NB):
        coef[b, 0:KS, :] = skt[:, b * 128:(b + 1) * 128]
        coef[b, KS:KS + 1, :] = ddv[b:b + 1, :]

    def p1(i):
        w_copy(2, i).wait()
        tasks = {}
        add_relayout(tasks, 2, i, 0)
        pro_body(1, i, tasks)
    period(1, p1)
    w_copy(5, 0).start()
    for c in range(2):
        w_copy(5, c + 1).start()
        wo_copy(c).start()
    w_copy(5, 3).start()
    for cp in kvh_copies(0, 0) + kvh_copies(0, 1):
        cp.wait()

    def p2(i):
        w_copy(3, i).wait()
        w_copy(4, i).wait()
        tasks = {}
        add_relayout(tasks, 3, i, 0)
        add_relayout(tasks, 4, i, 96)
        add_s01(tasks, i)
        pro_body(2, i, tasks)
    period(2, p2)

    def p3(i):
        @pl.when(i > 0)
        def _():
            wo_copy(i - 1).wait()
        w_copy(5, i).wait()
        tasks = {}
        add_relayout(tasks, 5, i, 0)
        add_wo(tasks, jnp.where(i == 0, 2, i - 1))
        add_s01(tasks, 4 + i, False)
        pro_body(3, i, tasks)

        @pl.when(i == 0)
        def _():
            wo_copy(2).start()
            wo_copy(3, 256 - 3 * WOP).start()
            x_copy(0).start()
            for cp in kvh_copies(1, 0) + kvh_copies(1, 1):
                cp.start()
            x_copy(1).start()
    period(3, p3)
    wo_copy(3, 256 - 3 * WOP).wait()
    wo_pack(3, 0, 256 - 3 * WOP)
    x_copy(0).wait()

    def step(cb, j, mem, u4, after_pre):
        par = u4 % 2
        s = cb * 8 + j
        x0 = pl.multiple_of(PRE + XR * s, 8)
        wpos = pl.multiple_of(lax.rem(s, RING // XR) * XR, 8)
        rpos = pl.multiple_of(lax.rem(s + QOFF // SEG, RING // SEG) * SEG, 32)
        rbase = pl.multiple_of((s - par) * SEG, 64)
        m0 = 0 if par == 0 else 72
        x8 = 8 + SEG * par

        sl1 = (cb + 1) & 1
        b1 = jnp.minimum(cb + 1, NB - 1)
        slot1 = cb + 1
        b3 = jnp.maximum(cb - 1, 0)
        slot3 = jnp.where(cb == 0, NB, cb - 1)
        s2 = s2_parts(cb & 1, j)
        nu = [0]

        def unit(pace):
            u = nu[0]
            nu[0] += 1
            if 0 <= u - cfg['s0_at'][u4] < 8:
                coef[NB + zero[0], 0:8, :] = pace
                s0_kv(sl1, b1, slot1, j, u - cfg['s0_at'][u4])
            if 0 <= u - cfg['s2_at'][u4] < 2 * NC:
                s2(u - cfg['s2_at'][u4], pace)

        def proj_q(p, lq):
            ys = []
            for t in range(2):
                ys.append(jnp.dot(lq, wt(2, 2 * p + t), preferred_element_type=f32))
                unit(ys[-1][:M])
            r0, r1 = (0, 48) if par == 0 else (48, 80)
            q_sc[p][r0:r1, :] = jnp.concatenate(ys, axis=1).astype(bf16)

        def proj_kv(p, m, lhs):
            ys = [jnp.dot(lhs, wt(m, 2 * p + t), preferred_element_type=f32)
                  for t in range(2)]
            ring[p // 2][pl.ds(wpos, XR), ring_cols(m, p)] = jnp.concatenate(
                [y[M:] for y in ys], axis=1).astype(bf16)
            unit(ys[0][:M])
            m_sc[2 * p + m] = jnp.concatenate([y[:M] for y in ys], axis=1).astype(bf16)

        def gather(m, p):
            xx = ring[p // 2][pl.ds(rpos, SEG), ring_cols(m, p)]
            mm = jnp.concatenate([m_sc[2 * p + m, :, :DH], m_sc[2 * p + m, :, DH:]], axis=0)
            return jnp.concatenate([mm, xx[:, :DH], xx[:, DH:]], axis=0)

        def qk(p):
            b = q_sc[p]
            q2 = jnp.concatenate([b[m0:m0 + M, :DH], b[m0:m0 + M, DH:],
                                  b[x8:x8 + SEG, :DH], b[x8:x8 + SEG, DH:]], axis=0)
            sc = lax.dot_general(q2, gather(0, p), (((1,), (1,)), ((), ())),
                                 preferred_element_type=f32)
            fill = fill_ref[...]
            sc = jnp.where(fill == 0.0, sc, fill)
            mx = jnp.max(sc, axis=1, keepdims=True)
            e = jnp.exp((sc - mx) * scale)
            l = jnp.sum(e, axis=1, keepdims=True)
            rc = pl.reciprocal(l, approx=True)
            rc = rc * (2.0 - l * rc)
            p_sc[p] = pltpu.bitcast((e * rc).astype(bf16), u32)

        def pv(p):
            o = jnp.dot(_bf(p_sc[p]), gather(1, p), preferred_element_type=f32)
            o_sc[p][m0:m0 + M, :] = jnp.concatenate([o[0:M], o[M:2 * M]], axis=1).astype(bf16)
            o_sc[p][x8:x8 + SEG, :] = jnp.concatenate(
                [o[2 * M:2 * M + SEG], o[2 * M + SEG:]], axis=1).astype(bf16)

        accs = [None] * 8
        odots = [(k, n) for k in range(0, H, OCH) for n in range(8)]
        lcache = {}

        def oproj(cnt):
            r0, r1 = (0, 32) if par == 0 else (32, 80)
            for _ in range(min(cnt, len(odots))):
                k, n = odots.pop(0)
                ke = k + OCH
                if k not in lcache:
                    lcache[k] = jnp.concatenate(
                        [o_sc[p][r0:r1, :] for p in range(k // 2, ke // 2)], axis=1)
                y = jnp.dot(lcache[k], _bf(wo_p[n, k * 64:ke * 64, :]),
                            preferred_element_type=f32)
                accs[n] = y if accs[n] is None else y + accs[n]
                unit(accs[n][:M])

        def pre_u():
            if u4 == 0:
                n1 = s + 4
                for k in range(4):
                    s1_u((n1 >> 3) & 1, n1 >> 3, (n1 & 7) + k)
        pre = dict(u=pre_u,
                   h=lambda: s1_h(sl1, j),
                   y=lambda: s3(sl1, b3, slot3, j))
        for key in cfg['border'][u4]:
            pre[key]()
        if after_pre is not None:
            after_pre()

        if par == 0:
            lq = jnp.concatenate([mem, x_buf[pl.ds(rbase, 40), :]], axis=0)
        else:
            lq = jnp.concatenate([x_buf[pl.ds(rbase + 40, 24), :], mem], axis=0)
        for p in range(NPAIR):
            proj_q(p, lq)

        lhs = jnp.concatenate([mem, x_buf[pl.ds(x0, XR), :]], axis=0)
        a0, a1 = cfg['att'][u4]
        att = {4 + a0: ([], [0, 1, 2, 3]), 18 + a1: ([12, 13, 14, 15], []),
               **{t + a0: ([t - 6, t - 5], [t - 2, t - 1]) for t in range(6, 18, 2)}}
        for t in range(max(att) + 1):
            if t < NPAIR:
                for m in range(2):
                    proj_kv(t, m, lhs)
            else:
                oproj(cfg['op_per'][u4])
            pvs, qks = att.get(t, ((), ()))
            for p in pvs:
                pv(p)
            for p in qks:
                qk(p)
        oproj(len(odots))
        out = jnp.concatenate(accs, axis=1).astype(bf16)
        if par == 0:
            outb[pl.ds(rbase, 24), :] = out[M:]
            return out[:M]
        outb[pl.ds(rbase + 24, 40), :] = out[:40]
        return out[40:]

    def four_steps(it, carry):
        cb, jj = it >> 1, it & 1

        @pl.when(cb + 1 < NB)
        def _():
            for cp in kvh_copies(cb + 1, jj):
                cp.wait()

        @pl.when(cb >= 1)
        def _():
            q_copy(cb - 1, jj).wait()

        @pl.when(it == 1)
        def _():
            x_copy(1).wait()

        @pl.when(it >= 1)
        def _():
            outa_copy(jnp.maximum(((it - 1) >> 1) - 1, 0), (it - 1) & 1).wait()
            outb_copy(2 * it - 1).start()

        mem = mem_ref[...]
        for u in range(4):
            after = (lambda: outa_copy(jnp.maximum(cb - 1, 0), jj).start()) if u == 3 else None
            mem = step(cb, jj * 4 + u, mem, u, after)
            if u == 1:
                outb_copy(2 * it).start()
        mem_ref[...] = mem

        @pl.when(it + 1 < 2 * NB)
        def _():
            q_copy((it + 1) >> 1, (it + 1) & 1).start()

        @pl.when(cb + 2 < NB)
        def _():
            for cp in kvh_copies(cb + 2, jj):
                cp.start()
        return carry
    q_copy(0, 0).start()
    with jax.named_scope('main'):
        lax.fori_loop(0, 2 * NB, four_steps, 0)

    outb_copy(NSEG // 2 - 1).start()
    q_copy(NB - 1, 0).wait()
    q_copy(NB - 1, 1).wait()
    with jax.named_scope('epi'):
        for j in range(8):
            s3((NB - 1) % 2, NB - 1, NB - 1, j)
            if j % 2 == 1:
                outa_piece(NB - 1, (j - 1) * 2 * C, 4 * C).start()

    outa_copy(NB - 2, 1).wait()
    for pr in range(NSEG // 2):
        outb_copy(pr).wait()
    for j in range(4):
        outa_piece(NB - 1, j * 4 * C, 4 * C).wait()


@jax.jit
def pallas_concat_heads__ssm_conv_h3__memory_aug_recurrent_mem_tr__prompt_kernel(
    A_q, A_k, A_v, A_shift_k, A_ssm_k, A_ssm_D, B_x, B_mem0, B_Wq, B_Wk, B_Wv, B_Wo,
    B_seg_len,
):
    del B_seg_len
    assert A_q.shape == (1, S, D) and B_x.shape == (1, S, D)
    assert B_Wq.shape == (D, H, DH) and B_mem0.shape == (1, M, D)
    vm = pltpu.VMEM
    dma = pltpu.SemaphoreType.DMA
    scratch = [
        vm((D + 4, 16, DH), bf16), vm((D + 4, 16, DH), bf16),
        vm((D + 4, 16, DH), bf16),
        vm((256 + 1, 16, D), bf16),
        vm((8, H * DH // 2, 128), u32),
        vm((S, D), bf16),
        vm((M, D), bf16),
        vm((S, D), bf16),
        vm((NB + 1, 32, 128), f32),
        vm((2, S + 64, 128), bf16),
        vm((2, S, 128), bf16), vm((2, S, 128), bf16),
        vm((2, 128, S), bf16),
        vm((NB + 1, S, 128), bf16),
        vm((4 * NC + 1, 2 * C, 128), f32),
        vm((2, 8, 8, 32, 128), u32),
        vm((8, 32 + KPAD, 128), f32),
        vm((C, C), u32), vm((C // 2, C), u32),
        vm((PRE // 2, 256), u32),
        dma((40,)),
        pltpu.SMEM((1,), i32),
    ]
    scratch += [vm((16 * HS, 128), u32)] * 6
    scratch += [vm((RING, 8 * DH), bf16)] * 8
    scratch += [vm((L2, 2 * DH), bf16)] * (2 * NPAIR)
    scratch += [vm((NPAIR, L2 // 2, L2), u32)]
    scratch += [vm((2 * NPAIR, M, 2 * DH), bf16)]
    scratch += [vm((L2, L2), f32), vm((KS, D), bf16), vm((NB, 128), bf16)]

    out = pl.pallas_call(
        _kernel,
        out_shape=jax.ShapeDtypeStruct((S, 2 * D), bf16),
        in_specs=[pl.BlockSpec(memory_space=pl.ANY)] * 12,
        out_specs=pl.BlockSpec(memory_space=pl.ANY),
        scratch_shapes=scratch,
        compiler_params=pltpu.CompilerParams(vmem_limit_bytes=120 * 1024 * 1024,
                                             disable_bounds_checks=True,
                                             disable_semaphore_checks=True),
        name="ssm_memtr",
    )(A_q.reshape(S, D), A_k.reshape(S, D), A_v.reshape(S, D), A_shift_k.T, A_ssm_k,
      A_ssm_D.reshape(NB, 128), B_x.reshape(S, D), B_mem0.reshape(M, D),
      B_Wq, B_Wk, B_Wv, B_Wo.reshape(H * DH // 16, 16, D))
    return out.reshape(1, S, 2 * D)
```

```python
import math

import jax
import jax.numpy as jnp
from jax import lax
import jax.experimental.pallas as pl
import jax.experimental.pallas.tpu as pltpu

bf16, f32, u32, i32 = jnp.bfloat16, jnp.float32, jnp.uint32, jnp.int32

S = 2048
D = 1024
H, DH = 32, 128
M, SEG = 8, 32
NSEG = S // SEG
KS = 4

XR = 24
PRE = S - NSEG * XR
RING = 576
QOFF = 64
HS = 514
NPAIR = H // 2
L2 = 2 * (M + SEG)
OCH = 8
WOP = 76

C = 128
NC = S // C
NB = D // 128
KPAD = 16

CFG = dict(
    att=[(0, 0), (0, 0), (0, 0), (1, 1)], op_per=[4, 3, 4, 4],
    s2_at=[0, 62, 0, 62], s0_at=[17, 78, 17, 78],
    border=['uyh'] * 4, nopro=False,
)


def _bf(x):
    return pltpu.bitcast(x, bf16)


def _kernel(q_hbm, k_hbm, v_hbm, skt_hbm, h_hbm, dd_hbm, x_hbm, mem0_hbm,
            wq_hbm, wk_hbm, wv_hbm, wo_hbm, out_hbm,
            st0, st1, st2, wo_st, wo_p, x_buf, mem_ref, outb,
            coef, k_buf, v_buf, q_buf, h_buf, kvo,
            uh, y_buf, kf, f_p, g_p, xp, sems, zero,
            *bufs):
    wp = bufs[0:6]
    ring = bufs[6:14]
    o_sc = bufs[14:30]
    q_sc = bufs[30:46]
    p_sc, m_sc, fill_ref, skt_buf, dd_buf = bufs[46:51]
    stage = (st0, st1, st2)
    w_hbm = (wk_hbm, wv_hbm, wq_hbm)
    scale = DH ** -0.5
    cfg = CFG
    SW, SWO, SX, SSM, SKVH, SQ, SOUT = 0, 12, 20, 26, 29, 33, 37

    def w_copy(g, c):
        r0 = c * 256
        return pltpu.make_async_copy(
            w_hbm[g // 2].at[pl.ds(r0, 256), pl.ds(16 * (g % 2), 16), :],
            stage[g % 3].at[pl.ds(r0, 256)],
            sems.at[SW + (g % 3) * 4 + c])

    def wo_copy(part, n=WOP):
        rows = pl.ds(part * WOP, n)
        return pltpu.make_async_copy(wo_hbm.at[rows], wo_st.at[rows], sems.at[SWO + part])

    def xc_copy(c):
        cols = pl.ds(pl.multiple_of(c * 256, 256), 256)
        return pltpu.make_async_copy(x_hbm.at[pl.ds(0, PRE), cols],
                                     x_buf.at[pl.ds(0, PRE), cols], sems.at[SX + c])

    def x_copy(part):
        r0, n = ((PRE, 128), (PRE + 128, S - PRE - 128))[part]
        return pltpu.make_async_copy(
            x_hbm.at[pl.ds(r0, n)], x_buf.at[pl.ds(r0, n)], sems.at[SX + 4 + part])

    def small_copies():
        return [pltpu.make_async_copy(skt_hbm, skt_buf, sems.at[SSM + 0]),
                pltpu.make_async_copy(dd_hbm, dd_buf, sems.at[SSM + 1]),
                pltpu.make_async_copy(mem0_hbm, mem_ref, sems.at[SSM + 2])]

    def col(b):
        return pl.ds(pl.multiple_of(b * 128, 128), 128)

    HALF = S // 2

    def half_rows(half, off=0):
        return pl.ds(pl.multiple_of(half * HALF, HALF) + off, HALF)

    def kvh_copies(b, half):
        sl, t = b & 1, half_rows(half)
        sem = sems.at[SKVH + 2 * sl + half]
        return [pltpu.make_async_copy(k_hbm.at[t, col(b)],
                                      k_buf.at[sl, half_rows(half, KPAD)], sem),
                pltpu.make_async_copy(v_hbm.at[t, col(b)], v_buf.at[sl, t], sem),
                pltpu.make_async_copy(h_hbm.at[col(b), t], h_buf.at[sl, :, t], sem)]

    def q_copy(b, half):
        sl, t = b & 1, half_rows(half)
        return pltpu.make_async_copy(q_hbm.at[t, col(b)], q_buf.at[sl, t],
                                     sems.at[SQ + 2 * sl + half])

    def outa_copy(b, half):
        t = half_rows(half)
        return pltpu.make_async_copy(kvo.at[b, t], out_hbm.at[t, col(b)], sems.at[SOUT])

    def outa_piece(b, r0, n):
        return pltpu.make_async_copy(kvo.at[b, pl.ds(r0, n)],
                                     out_hbm.at[pl.ds(r0, n), col(b)], sems.at[SOUT + 1])

    def outb_copy(pr):
        rows = pl.ds(pl.multiple_of(pr * 2 * SEG, 2 * SEG), 2 * SEG)
        return pltpu.make_async_copy(outb.at[rows], out_hbm.at[rows, pl.ds(D, D)],
                                     sems.at[SOUT + 2])

    def relayout(g, c, lo_i=0, hi_i=128):
        src, dst = stage[g % 3], wp[g]
        d0 = c * 256
        for i in range(lo_i, hi_i):
            a = pltpu.bitcast(src[d0 + 2 * i], u32)
            b = pltpu.bitcast(src[d0 + 2 * i + 1], u32)
            lo = (a & jnp.uint32(0xFFFF)) | (b << 16)
            hi = (a >> 16) | (b & jnp.uint32(0xFFFF0000))
            row = c * 128 + i
            dst[pl.ds(row, 8, stride=2 * HS), :] = lo
            dst[pl.ds(row + HS, 8, stride=2 * HS), :] = hi

    def wo_pack(part, r0, r1):
        for r in range(r0, r1):
            blk = pltpu.bitcast(wo_st[part * WOP + r], u32)
            rows = pl.ds(pl.multiple_of((part * WOP + r) * 8, 8), 8)
            for n in range(8):
                wo_p[n, rows, :] = blk[:, n * 128:(n + 1) * 128]

    def wt(m, h):
        g, hh = 2 * m + h // 16, h % 16
        return _bf(wp[g][hh * HS:hh * HS + D // 2, :])

    def ring_cols(m, p):
        c0 = 512 * m + 256 * (p % 2)
        return slice(c0, c0 + 256)

    def s0_kv(sl, b, slot, j, i):
        t0 = pl.multiple_of(j * 2 * C, 2 * C)
        kw = k_buf.at[sl, pl.ds(t0, 2 * C + KPAD)]
        vw = v_buf.at[sl, pl.ds(t0, 2 * C)]
        ow = kvo.at[slot, pl.ds(t0, 2 * C)]
        kf[i] = kw[32 * i:32 * i + 32 + KPAD, :].astype(f32)
        acc = None
        for tap in range(KS):
            term = kf[i, KPAD - tap:KPAD - tap + 32, :] * coef[b, tap:tap + 1, :]
            acc = term if acc is None else acc + term
        ow[32 * i:32 * i + 32, :] = (acc * vw[32 * i:32 * i + 32, :].astype(f32)).astype(bf16)

    def s1_h(sl, j):
        for t in range(2):
            a = 2 * j + t
            hh = h_buf[sl, :, pl.ds(pl.multiple_of(a * C, C), C)]
            for half in range(2):
                fm = _bf(f_p[half * 64:(half + 1) * 64, :])
                uh[sl * 2 * NC + NC + a, half * C:(half + 1) * C, :] = lax.dot_general(
                    fm, hh, (((1,), (1,)), ((), ())), preferred_element_type=f32)

    def s1_u(sl, slot, j):
        for t in range(2):
            a = 2 * j + t
            kv = kvo[slot, pl.ds(pl.multiple_of(a * C, C), C), :]
            for half in range(2):
                fm = _bf(f_p[half * 64:(half + 1) * 64, :])
                uh[sl * 2 * NC + a, half * C:(half + 1) * C, :] = jnp.dot(
                    fm, kv, preferred_element_type=f32)

    def s2_parts(sl, j):
        u0 = sl * 2 * NC
        h0 = u0 + NC
        r0 = pl.multiple_of(j * 32, 32)
        prev = []

        def one(idx, pace):
            grp, a = divmod(idx, NC)
            re, im = pl.ds(r0 + 16 * grp, 8), pl.ds(r0 + 16 * grp + 8, 8)
            yr = yi = None
            for b in range(a + 1):
                if b == a:
                    uh[4 * NC + zero[0], 0:8, :] = pace
                ur, ui = uh[u0 + b, re, :], uh[u0 + b, im, :]
                hr, hi = uh[h0 + a - b, re, :], uh[h0 + a - b, im, :]
                yr = ur * hr if yr is None else yr + ur * hr
                yi = ur * hi if yi is None else yi + ur * hi
                yr = yr - ui * hi
                yi = yi + ui * hr
            pp, qq = yr - yi, yr + yi
            if a > 0:
                zp, zq = pp - prev[1], qq + prev[0]
            else:
                zp, zq = pp, qq
            prev[:] = [pp, qq]
            z = pltpu.bitcast(jnp.concatenate([zp, zq], axis=0).astype(bf16), u32)
            r = (a % 2) * 16 + 4 * grp
            y_buf[sl, j, a // 2, r:r + 4, :] = z[0:4]
            y_buf[sl, j, a // 2, r + 8:r + 12, :] = z[4:8]
        return one

    def s3(sl, b, slot, j):
        rev = 7 - lax.broadcasted_iota(i32, (8, 128), 0)
        for t in range(2):
            a = 2 * j + t
            rows = pl.ds(pl.multiple_of(a * C, C), C)
            eo = []
            for part in range(2):
                r = 16 * t + 8 * part
                yp = y_buf[sl, :, j, r:r + 8, :].reshape(C // 2, 128)
                eo.append(jnp.dot(_bf(g_p[part * 32:(part + 1) * 32, :]), _bf(yp),
                                  preferred_element_type=f32))
            lo, hi = eo[0] + eo[1], eo[0] - eo[1]
            hi = [jnp.take_along_axis(hi[8 * i:8 * i + 8], rev, axis=0) for i in range(7, -1, -1)]
            y = jnp.concatenate([lo] + hi, axis=0)
            y = y + kvo[slot, rows, :].astype(f32) * coef[b, KS:KS + 1, :]
            kvo[slot, rows, :] = (q_buf[sl, rows, :].astype(f32) * y).astype(bf16)

    zero[0] = 0
    for c in range(4):
        w_copy(0, c).start()
        xc_copy(c).start()
        if c == 0:
            for cp in small_copies():
                cp.start()
        else:
            w_copy(1, c - 1).start()

    r = lax.broadcasted_iota(i32, (L2, L2), 0)
    c_ = lax.broadcasted_iota(i32, (L2, L2), 1)
    head = lambda i: jnp.where(i < 2 * M, i // M, (i - 2 * M) // SEG)
    ok = (r < 2 * M) | (c_ < 2 * M) | (c_ <= r)
    fill_ref[...] = jnp.where(head(r) == head(c_),
                              jnp.where(ok, 0.0, -1e9 / scale), -jnp.inf).astype(f32)

    def tables(t, carry):
        rr = lax.broadcasted_iota(i32, (32, C), 0) + 32 * t
        nn = lax.broadcasted_iota(i32, (32, C), 1)
        kk = 8 * (rr >> 4) + (rr & 7)
        mm = (2 * kk + 1) * (4 * nn + 1) + 4 * C * ((rr >> 3) & 1) * (1 + 2 * (kk & 1))
        fm = jnp.cos((mm & (16 * C - 1)).astype(f32) * (math.pi / (8 * C)))
        f_p[pl.ds(pl.multiple_of(16 * t, 16), 16), :] = pltpu.bitcast(fm.astype(bf16), u32)
        rr = lax.broadcasted_iota(i32, (16, C), 0) + 16 * t
        kk = lax.broadcasted_iota(i32, (16, C), 1)
        mm = (2 * kk + 1) * (2 * (rr & (C // 2 - 1)) + 1) + C * (7 - 6 * ((kk + (rr >> 6)) & 1))
        gm = jnp.cos((mm & (8 * C - 1)).astype(f32) * (math.pi / (4 * C))) * (2 ** -0.5 / C)
        g_p[pl.ds(pl.multiple_of(8 * t, 8), 8), :] = pltpu.bitcast(gm.astype(bf16), u32)
        uh[pl.ds(4 * t, 4)] = jnp.zeros((4, 2 * C, 128), f32)
        return carry
    lax.fori_loop(0, 8, tables, 0)
    for sl in range(2):
        k_buf[sl, 0:KPAD, :] = jnp.zeros((KPAD, 128), bf16)

    def pro_body(g, i, tasks):
        r0 = pl.multiple_of(i * 128, 128)
        x = x_buf[pl.ds(r0, 128), :]
        for p in range(8):
            ys = []
            for t in range(2):
                y = jnp.dot(x, wt(g // 2, 16 * (g % 2) + 2 * p + t),
                            preferred_element_type=f32)
                ys.append(y)
                for fn in tasks.get(2 * p + t, ()):
                    fn(y)
            pp = 8 * (g % 2) + p
            ring[pp // 2][pl.ds(pl.multiple_of(QOFF + r0, 64), 128),
                          ring_cols(g // 2, pp)] = jnp.concatenate(ys, axis=1).astype(bf16)

    def add_relayout(tasks, g, c, r):
        for u in range(15):
            def fn(y, u=u):
                stage[g % 3][D + zero[0]] = y[r:r + 16].astype(bf16)
                relayout(g, c, (128 * u) // 15, (128 * (u + 1)) // 15)
            tasks.setdefault(u, []).append(fn)

    def add_wo(tasks, part):
        for u in range(15):
            def fn(y, u=u):
                wo_st[256 + zero[0], :, 0:128] = y[96:112].astype(bf16)
                wo_pack(part, (WOP * u) // 15, (WOP * (u + 1)) // 15)
            tasks.setdefault(u, []).append(fn)

    def add_s01(tasks, j, with_u=True):
        for k in range(8):
            def fn(y, k=k):
                coef[NB + zero[0], 0:8, :] = y[48:56]
                s0_kv(0, 0, 0, j, k)
            tasks.setdefault(k, []).append(fn)
        tasks.setdefault(3, []).append(lambda y: s1_h(0, j))
        if with_u:
            tasks.setdefault(11, []).append(lambda y: s1_u(0, 0, j))

    def period(g, body, n=4):
        if cfg['nopro']:
            return
        with jax.named_scope('pro%d' % g):
            lax.fori_loop(0, n, lambda i, c: (body(i), c)[1], 0)

    def p0(c):
        @pl.when(c > 0)
        def _():
            w_copy(1, c - 1).wait()
        w_copy(0, c).wait()
        relayout(0, c)
        xc_copy(c).wait()
        xp[...] = pltpu.bitcast(
            x_buf[0:PRE, pl.ds(pl.multiple_of(c * 256, 256), 256)], u32)
        tasks = {}
        add_relayout(tasks, 1, (c + 3) % 4, 0)
        k0 = pl.multiple_of(c * 128, 128)
        for p in range(8):
            ys = []
            for t in range(2):
                hh = 2 * p + t
                w = _bf(wp[0][pl.ds(k0 + hh * HS, 128), :])
                y = (jnp.dot(_bf(xp[...]), w, preferred_element_type=f32)
                     + uh[2 * hh:2 * hh + 2].reshape(PRE, 128))
                uh[2 * hh:2 * hh + 2] = y.reshape(2, 2 * C, 128)
                ys.append(y)
                for fn in tasks.get(hh, ()):
                    fn(y[256 * t:])
            ring[p // 2][QOFF:QOFF + PRE, ring_cols(0, p)] = (
                jnp.concatenate(ys, axis=1).astype(bf16))

        @pl.when(c == 0)
        def _():
            w_copy(1, 3).start()
            for i in range(4):
                w_copy(2, i).start()
    period(0, p0)
    w_copy(1, 3).wait()
    relayout(1, 3)
    for cp in small_copies():
        cp.wait()
    w_copy(3, 0).start()
    w_copy(3, 1).start()
    for cp in kvh_copies(0, 0):
        cp.start()
    w_copy(4, 0).start()
    w_copy(4, 1).start()
    for c in range(2, 4):
        w_copy(3, c).start()
        w_copy(4, c).start()
    for cp in kvh_copies(0, 1):
        cp.start()
    skt = skt_buf[...].astype(f32)
    ddv = dd_buf[...].astype(f32)
    for b in range(NB):
        coef[b, 0:KS, :] = skt[:, b * 128:(b + 1) * 128]
        coef[b, KS:KS + 1, :] = ddv[b:b + 1, :]

    def p1(i):
        w_copy(2, i).wait()
        tasks = {}
        add_relayout(tasks, 2, i, 0)
        pro_body(1, i, tasks)
    period(1, p1)
    w_copy(5, 0).start()
    for c in range(2):
        w_copy(5, c + 1).start()
        wo_copy(c).start()
    w_copy(5, 3).start()
    for cp in kvh_copies(0, 0):
        cp.wait()

    def p2(i2):
        for i in (2 * i2, 2 * i2 + 1):
            w_copy(3, i).wait()
            w_copy(4, i).wait()
        for i in (2 * i2, 2 * i2 + 1):
            tasks = {}
            add_relayout(tasks, 3, i, 0)
            add_relayout(tasks, 4, i, 96)
            add_s01(tasks, i)
            pro_body(2, i, tasks)
    period(2, p2, 2)
    for cp in kvh_copies(0, 1):
        cp.wait()

    def p3(i):
        @pl.when(i > 0)
        def _():
            wo_copy(i - 1).wait()
        w_copy(5, i).wait()
        tasks = {}
        add_relayout(tasks, 5, i, 0)
        add_wo(tasks, jnp.where(i == 0, 2, i - 1))
        add_s01(tasks, 4 + i, False)
        pro_body(3, i, tasks)

        @pl.when(i == 0)
        def _():
            wo_copy(2).start()
            wo_copy(3, 256 - 3 * WOP).start()
            x_copy(0).start()
            for cp in kvh_copies(1, 0) + kvh_copies(1, 1):
                cp.start()
            x_copy(1).start()
    period(3, p3)
    wo_copy(3, 256 - 3 * WOP).wait()
    wo_pack(3, 0, 256 - 3 * WOP)
    x_copy(0).wait()

    def step(cb, j, mem, u4, after_pre):
        par = u4 % 2
        s = cb * 8 + j
        x0 = pl.multiple_of(PRE + XR * s, 8)
        wpos = pl.multiple_of(lax.rem(s, RING // XR) * XR, 8)
        rpos = pl.multiple_of(lax.rem(s + QOFF // SEG, RING // SEG) * SEG, 32)
        rbase = pl.multiple_of((s - par) * SEG, 64)
        m0 = 0 if par == 0 else 72
        x8 = 8 + SEG * par

        sl1 = (cb + 1) & 1
        b1 = jnp.minimum(cb + 1, NB - 1)
        slot1 = cb + 1
        b3 = jnp.maximum(cb - 1, 0)
        slot3 = jnp.where(cb == 0, NB, cb - 1)
        s2 = s2_parts(cb & 1, j)
        nu = [0]

        def unit(pace):
            u = nu[0]
            nu[0] += 1
            if 0 <= u - cfg['s0_at'][u4] < 8:
                coef[NB + zero[0], 0:8, :] = pace
                s0_kv(sl1, b1, slot1, j, u - cfg['s0_at'][u4])
            if 0 <= u - cfg['s2_at'][u4] < 2 * NC:
                s2(u - cfg['s2_at'][u4], pace)

        def proj_q(p, lq):
            ys = []
            for t in range(2):
                ys.append(jnp.dot(lq, wt(2, 2 * p + t), preferred_element_type=f32))
                unit(ys[-1][:M])
            r0, r1 = (0, 48) if par == 0 else (48, 80)
            q_sc[p][r0:r1, :] = jnp.concatenate(ys, axis=1).astype(bf16)

        def proj_kv(p, m, lhs):
            ys = [jnp.dot(lhs, wt(m, 2 * p + t), preferred_element_type=f32)
                  for t in range(2)]
            ring[p // 2][pl.ds(wpos, XR), ring_cols(m, p)] = jnp.concatenate(
                [y[M:] for y in ys], axis=1).astype(bf16)
            unit(ys[0][:M])
            m_sc[2 * p + m] = jnp.concatenate([y[:M] for y in ys], axis=1).astype(bf16)

        def gather(m, p):
            xx = ring[p // 2][pl.ds(rpos, SEG), ring_cols(m, p)]
            mm = jnp.concatenate([m_sc[2 * p + m, :, :DH], m_sc[2 * p + m, :, DH:]], axis=0)
            return jnp.concatenate([mm, xx[:, :DH], xx[:, DH:]], axis=0)

        def qk(p):
            b = q_sc[p]
            q2 = jnp.concatenate([b[m0:m0 + M, :DH], b[m0:m0 + M, DH:],
                                  b[x8:x8 + SEG, :DH], b[x8:x8 + SEG, DH:]], axis=0)
            sc = lax.dot_general(q2, gather(0, p), (((1,), (1,)), ((), ())),
                                 preferred_element_type=f32)
            fill = fill_ref[...]
            sc = jnp.where(fill == 0.0, sc, fill)
            mx = jnp.max(sc, axis=1, keepdims=True)
            e = jnp.exp((sc - mx) * scale)
            l = jnp.sum(e, axis=1, keepdims=True)
            rc = pl.reciprocal(l, approx=True)
            rc = rc * (2.0 - l * rc)
            p_sc[p] = pltpu.bitcast((e * rc).astype(bf16), u32)

        def pv(p):
            o = jnp.dot(_bf(p_sc[p]), gather(1, p), preferred_element_type=f32)
            o_sc[p][m0:m0 + M, :] = jnp.concatenate([o[0:M], o[M:2 * M]], axis=1).astype(bf16)
            o_sc[p][x8:x8 + SEG, :] = jnp.concatenate(
                [o[2 * M:2 * M + SEG], o[2 * M + SEG:]], axis=1).astype(bf16)

        accs = [None] * 8
        odots = [(k, n) for k in range(0, H, OCH) for n in range(8)]
        lcache = {}

        def oproj(cnt):
            r0, r1 = (0, 32) if par == 0 else (32, 80)
            for _ in range(min(cnt, len(odots))):
                k, n = odots.pop(0)
                ke = k + OCH
                if k not in lcache:
                    lcache[k] = jnp.concatenate(
                        [o_sc[p][r0:r1, :] for p in range(k // 2, ke // 2)], axis=1)
                y = jnp.dot(lcache[k], _bf(wo_p[n, k * 64:ke * 64, :]),
                            preferred_element_type=f32)
                accs[n] = y if accs[n] is None else y + accs[n]
                unit(accs[n][:M])

        def pre_u():
            if u4 == 0:
                n1 = s + 4
                for k in range(4):
                    s1_u((n1 >> 3) & 1, n1 >> 3, (n1 & 7) + k)
        pre = dict(u=pre_u,
                   h=lambda: s1_h(sl1, j),
                   y=lambda: s3(sl1, b3, slot3, j))
        for key in cfg['border'][u4]:
            pre[key]()
        if after_pre is not None:
            after_pre()

        if par == 0:
            lq = jnp.concatenate([mem, x_buf[pl.ds(rbase, 40), :]], axis=0)
        else:
            lq = jnp.concatenate([x_buf[pl.ds(rbase + 40, 24), :], mem], axis=0)
        for p in range(NPAIR):
            proj_q(p, lq)

        lhs = jnp.concatenate([mem, x_buf[pl.ds(x0, XR), :]], axis=0)
        a0, a1 = cfg['att'][u4]
        att = {4 + a0: ([], [0, 1, 2, 3]), 18 + a1: ([12, 13, 14, 15], []),
               **{t + a0: ([t - 6, t - 5], [t - 2, t - 1]) for t in range(6, 18, 2)}}
        for t in range(max(att) + 1):
            if t < NPAIR:
                for m in range(2):
                    proj_kv(t, m, lhs)
            else:
                oproj(cfg['op_per'][u4])
            pvs, qks = att.get(t, ((), ()))
            for p in pvs:
                pv(p)
            for p in qks:
                qk(p)
        oproj(len(odots))
        out = jnp.concatenate(accs, axis=1).astype(bf16)
        if par == 0:
            outb[pl.ds(rbase, 24), :] = out[M:]
            return out[:M]
        outb[pl.ds(rbase + 24, 40), :] = out[:40]
        return out[40:]

    def four_steps(it, carry):
        cb, jj = it >> 1, it & 1

        @pl.when(cb + 1 < NB)
        def _():
            for cp in kvh_copies(cb + 1, jj):
                cp.wait()

        @pl.when(cb >= 1)
        def _():
            q_copy(cb - 1, jj).wait()

        @pl.when(it == 1)
        def _():
            x_copy(1).wait()

        @pl.when(it >= 1)
        def _():
            outa_copy(jnp.maximum(((it - 1) >> 1) - 1, 0), (it - 1) & 1).wait()
            outb_copy(2 * it - 1).start()

        mem = mem_ref[...]
        for u in range(4):
            after = (lambda: outa_copy(jnp.maximum(cb - 1, 0), jj).start()) if u == 3 else None
            mem = step(cb, jj * 4 + u, mem, u, after)
            if u == 1:
                outb_copy(2 * it).start()
        mem_ref[...] = mem

        @pl.when(it + 1 < 2 * NB)
        def _():
            q_copy((it + 1) >> 1, (it + 1) & 1).start()

        @pl.when(cb + 2 < NB)
        def _():
            for cp in kvh_copies(cb + 2, jj):
                cp.start()
        return carry
    q_copy(0, 0).start()
    with jax.named_scope('main'):
        lax.fori_loop(0, 2 * NB, four_steps, 0)

    outb_copy(NSEG // 2 - 1).start()
    q_copy(NB - 1, 0).wait()
    q_copy(NB - 1, 1).wait()
    with jax.named_scope('epi'):
        for j in range(8):
            s3((NB - 1) % 2, NB - 1, NB - 1, j)
            if j % 2 == 1:
                outa_piece(NB - 1, (j - 1) * 2 * C, 4 * C).start()

    outa_copy(NB - 2, 1).wait()
    for pr in range(NSEG // 2):
        outb_copy(pr).wait()
    for j in range(4):
        outa_piece(NB - 1, j * 4 * C, 4 * C).wait()


@jax.jit
def pallas_concat_heads__ssm_conv_h3__memory_aug_recurrent_mem_tr__prompt_kernel(
    A_q, A_k, A_v, A_shift_k, A_ssm_k, A_ssm_D, B_x, B_mem0, B_Wq, B_Wk, B_Wv, B_Wo,
    B_seg_len,
):
    del B_seg_len
    assert A_q.shape == (1, S, D) and B_x.shape == (1, S, D)
    assert B_Wq.shape == (D, H, DH) and B_mem0.shape == (1, M, D)
    vm = pltpu.VMEM
    dma = pltpu.SemaphoreType.DMA
    scratch = [
        vm((D + 4, 16, DH), bf16), vm((D + 4, 16, DH), bf16),
        vm((D + 4, 16, DH), bf16),
        vm((256 + 1, 16, D), bf16),
        vm((8, H * DH // 2, 128), u32),
        vm((S, D), bf16),
        vm((M, D), bf16),
        vm((S, D), bf16),
        vm((NB + 1, 32, 128), f32),
        vm((2, S + 64, 128), bf16),
        vm((2, S, 128), bf16), vm((2, S, 128), bf16),
        vm((2, 128, S), bf16),
        vm((NB + 1, S, 128), bf16),
        vm((4 * NC + 1, 2 * C, 128), f32),
        vm((2, 8, 8, 32, 128), u32),
        vm((8, 32 + KPAD, 128), f32),
        vm((C, C), u32), vm((C // 2, C), u32),
        vm((PRE // 2, 256), u32),
        dma((40,)),
        pltpu.SMEM((1,), i32),
    ]
    scratch += [vm((16 * HS, 128), u32)] * 6
    scratch += [vm((RING, 8 * DH), bf16)] * 8
    scratch += [vm((L2, 2 * DH), bf16)] * (2 * NPAIR)
    scratch += [vm((NPAIR, L2 // 2, L2), u32)]
    scratch += [vm((2 * NPAIR, M, 2 * DH), bf16)]
    scratch += [vm((L2, L2), f32), vm((KS, D), bf16), vm((NB, 128), bf16)]

    out = pl.pallas_call(
        _kernel,
        out_shape=jax.ShapeDtypeStruct((S, 2 * D), bf16),
        in_specs=[pl.BlockSpec(memory_space=pl.ANY)] * 12,
        out_specs=pl.BlockSpec(memory_space=pl.ANY),
        scratch_shapes=scratch,
        compiler_params=pltpu.CompilerParams(vmem_limit_bytes=120 * 1024 * 1024,
                                             disable_bounds_checks=True,
                                             disable_semaphore_checks=True),
        name="ssm_memtr",
    )(A_q.reshape(S, D), A_k.reshape(S, D), A_v.reshape(S, D), A_shift_k.T, A_ssm_k,
      A_ssm_D.reshape(NB, 128), B_x.reshape(S, D), B_mem0.reshape(M, D),
      B_Wq, B_Wk, B_Wv, B_Wo.reshape(H * DH // 16, 16, D))
    return out.reshape(1, S, 2 * D)
```

```python
import math

import jax
import jax.numpy as jnp
from jax import lax
import jax.experimental.pallas as pl
import jax.experimental.pallas.tpu as pltpu

bf16, f32, u32, i32 = jnp.bfloat16, jnp.float32, jnp.uint32, jnp.int32

S = 2048
D = 1024
H, DH = 32, 128
M, SEG = 8, 32
NSEG = S // SEG
KS = 4

XR = 24
PRE = S - NSEG * XR
RING = 576
QOFF = 64
HS = 514
NPAIR = H // 2
L2 = 2 * (M + SEG)
OCH = 8
Q1 = 224
WOP = 72

C = 128
NC = S // C
NB = D // 128
KPAD = 16

CFG = dict(
    att=[(0, 0), (0, 0), (0, 0), (1, 1)], op_per=[4, 3, 4, 4],
    s2_at=[0, 62, 0, 62], s0_at=[17, 78, 17, 78],
    border=['uyh'] * 4, nopro=False,
)


def _bf(x):
    return pltpu.bitcast(x, bf16)


def _kernel(q_hbm, k_hbm, v_hbm, skt_hbm, h_hbm, dd_hbm, x_hbm, mem0_hbm,
            wq_hbm, wk_hbm, wv_hbm, wo_hbm, out_hbm,
            st0, st1, st2, wo_st, wo_p, x_buf, mem_ref, outb,
            coef, k_buf, v_buf, q_buf, h_buf, kvo,
            uh, y_buf, kf, f_p, g_p, xp, sems, zero,
            *bufs):
    wp = bufs[0:6]
    ring = bufs[6:14]
    o_sc = bufs[14:30]
    q_sc = bufs[30:46]
    p_sc, m_sc, fill_ref, skt_buf, dd_buf = bufs[46:51]
    stage = (st0, st1, st2)
    w_hbm = (wk_hbm, wv_hbm, wq_hbm)
    scale = DH ** -0.5
    cfg = CFG
    SW, SWO, SX, SSM, SKVH, SQ, SOUT = 0, 12, 20, 26, 29, 33, 37

    def w_copy(g, c, q=256, n=None):
        rows = pl.ds(c * q, q if n is None else n)
        return pltpu.make_async_copy(
            w_hbm[g // 2].at[rows, pl.ds(16 * (g % 2), 16), :], stage[g % 3].at[rows],
            sems.at[SW + (g % 3) * 4 + c])

    def wo_copy(part, n=WOP):
        rows = pl.ds(part * WOP, n)
        return pltpu.make_async_copy(wo_hbm.at[rows], wo_st.at[rows], sems.at[SWO + part])

    def xc_copy(c):
        cols = pl.ds(pl.multiple_of(c * 256, 256), 256)
        return pltpu.make_async_copy(x_hbm.at[pl.ds(0, PRE), cols],
                                     x_buf.at[pl.ds(0, PRE), cols], sems.at[SX + c])

    def x_copy(part):
        r0, n = ((PRE, 96), (PRE + 96, S - PRE - 96))[part]
        return pltpu.make_async_copy(
            x_hbm.at[pl.ds(r0, n)], x_buf.at[pl.ds(r0, n)], sems.at[SX + 4 + part])

    def small_copies():
        return [pltpu.make_async_copy(skt_hbm, skt_buf, sems.at[SSM + 0]),
                pltpu.make_async_copy(dd_hbm, dd_buf, sems.at[SSM + 1]),
                pltpu.make_async_copy(mem0_hbm, mem_ref, sems.at[SSM + 2])]

    def col(b):
        return pl.ds(pl.multiple_of(b * 128, 128), 128)

    HALF = S // 2

    def half_rows(half, off=0):
        return pl.ds(pl.multiple_of(half * HALF, HALF) + off, HALF)

    def kvh_copies(b, half):
        sl, t = b & 1, half_rows(half)
        sem = sems.at[SKVH + 2 * sl + half]
        return [pltpu.make_async_copy(k_hbm.at[t, col(b)],
                                      k_buf.at[sl, half_rows(half, KPAD)], sem),
                pltpu.make_async_copy(v_hbm.at[t, col(b)], v_buf.at[sl, t], sem),
                pltpu.make_async_copy(h_hbm.at[col(b), t], h_buf.at[sl, :, t], sem)]

    def q_copy(b, half):
        sl, t = b & 1, half_rows(half)
        return pltpu.make_async_copy(q_hbm.at[t, col(b)], q_buf.at[sl, t],
                                     sems.at[SQ + 2 * sl + half])

    def outa_copy(b, half):
        t = half_rows(half)
        return pltpu.make_async_copy(kvo.at[b, t], out_hbm.at[t, col(b)], sems.at[SOUT])

    def outa_piece(b, r0, n):
        return pltpu.make_async_copy(kvo.at[b, pl.ds(r0, n)],
                                     out_hbm.at[pl.ds(r0, n), col(b)], sems.at[SOUT + 1])

    def outb_copy(pr):
        rows = pl.ds(pl.multiple_of(pr * 2 * SEG, 2 * SEG), 2 * SEG)
        return pltpu.make_async_copy(outb.at[rows], out_hbm.at[rows, pl.ds(D, D)],
                                     sems.at[SOUT + 2])

    def relayout(g, c, lo_i=0, hi_i=128, q=256):
        src, dst = stage[g % 3], wp[g]
        d0 = c * q
        for i in range(lo_i, hi_i):
            a = pltpu.bitcast(src[d0 + 2 * i], u32)
            b = pltpu.bitcast(src[d0 + 2 * i + 1], u32)
            lo = (a & jnp.uint32(0xFFFF)) | (b << 16)
            hi = (a >> 16) | (b & jnp.uint32(0xFFFF0000))
            row = c * (q // 2) + i
            dst[pl.ds(row, 8, stride=2 * HS), :] = lo
            dst[pl.ds(row + HS, 8, stride=2 * HS), :] = hi

    def wo_pack(part, r0, r1):
        for r in range(r0, r1):
            blk = pltpu.bitcast(wo_st[part * WOP + r], u32)
            rows = pl.ds(pl.multiple_of((part * WOP + r) * 8, 8), 8)
            for n in range(8):
                wo_p[n, rows, :] = blk[:, n * 128:(n + 1) * 128]

    def wt(m, h):
        g, hh = 2 * m + h // 16, h % 16
        return _bf(wp[g][hh * HS:hh * HS + D // 2, :])

    def ring_cols(m, p):
        c0 = 512 * m + 256 * (p % 2)
        return slice(c0, c0 + 256)

    def s0_kv(sl, b, slot, j, i):
        t0 = pl.multiple_of(j * 2 * C, 2 * C)
        kw = k_buf.at[sl, pl.ds(t0, 2 * C + KPAD)]
        vw = v_buf.at[sl, pl.ds(t0, 2 * C)]
        ow = kvo.at[slot, pl.ds(t0, 2 * C)]
        kf[i] = kw[32 * i:32 * i + 32 + KPAD, :].astype(f32)
        acc = None
        for tap in range(KS):
            term = kf[i, KPAD - tap:KPAD - tap + 32, :] * coef[b, tap:tap + 1, :]
            acc = term if acc is None else acc + term
        ow[32 * i:32 * i + 32, :] = (acc * vw[32 * i:32 * i + 32, :].astype(f32)).astype(bf16)

    def s1_h(sl, j):
        for t in range(2):
            a = 2 * j + t
            hh = h_buf[sl, :, pl.ds(pl.multiple_of(a * C, C), C)]
            for half in range(2):
                fm = _bf(f_p[half * 64:(half + 1) * 64, :])
                uh[sl * 2 * NC + NC + a, half * C:(half + 1) * C, :] = lax.dot_general(
                    fm, hh, (((1,), (1,)), ((), ())), preferred_element_type=f32)

    def s1_u(sl, slot, j):
        for t in range(2):
            a = 2 * j + t
            kv = kvo[slot, pl.ds(pl.multiple_of(a * C, C), C), :]
            for half in range(2):
                fm = _bf(f_p[half * 64:(half + 1) * 64, :])
                uh[sl * 2 * NC + a, half * C:(half + 1) * C, :] = jnp.dot(
                    fm, kv, preferred_element_type=f32)

    def s2_parts(sl, j):
        u0 = sl * 2 * NC
        h0 = u0 + NC
        r0 = pl.multiple_of(j * 32, 32)
        prev = []

        def one(idx, pace):
            grp, a = divmod(idx, NC)
            re, im = pl.ds(r0 + 16 * grp, 8), pl.ds(r0 + 16 * grp + 8, 8)
            yr = yi = None
            for b in range(a + 1):
                if b == a:
                    uh[4 * NC + zero[0], 0:8, :] = pace
                ur, ui = uh[u0 + b, re, :], uh[u0 + b, im, :]
                hr, hi = uh[h0 + a - b, re, :], uh[h0 + a - b, im, :]
                yr = ur * hr if yr is None else yr + ur * hr
                yi = ur * hi if yi is None else yi + ur * hi
                yr = yr - ui * hi
                yi = yi + ui * hr
            pp, qq = yr - yi, yr + yi
            if a > 0:
                zp, zq = pp - prev[1], qq + prev[0]
            else:
                zp, zq = pp, qq
            prev[:] = [pp, qq]
            z = pltpu.bitcast(jnp.concatenate([zp, zq], axis=0).astype(bf16), u32)
            r = (a % 2) * 16 + 4 * grp
            y_buf[sl, j, a // 2, r:r + 4, :] = z[0:4]
            y_buf[sl, j, a // 2, r + 8:r + 12, :] = z[4:8]
        return one

    def s3(sl, b, slot, j):
        rev = 7 - lax.broadcasted_iota(i32, (8, 128), 0)
        for t in range(2):
            a = 2 * j + t
            rows = pl.ds(pl.multiple_of(a * C, C), C)
            eo = []
            for part in range(2):
                r = 16 * t + 8 * part
                yp = y_buf[sl, :, j, r:r + 8, :].reshape(C // 2, 128)
                eo.append(jnp.dot(_bf(g_p[part * 32:(part + 1) * 32, :]), _bf(yp),
                                  preferred_element_type=f32))
            lo, hi = eo[0] + eo[1], eo[0] - eo[1]
            hi = [jnp.take_along_axis(hi[8 * i:8 * i + 8], rev, axis=0) for i in range(7, -1, -1)]
            y = jnp.concatenate([lo] + hi, axis=0)
            y = y + kvo[slot, rows, :].astype(f32) * coef[b, KS:KS + 1, :]
            kvo[slot, rows, :] = (q_buf[sl, rows, :].astype(f32) * y).astype(bf16)

    zero[0] = 0
    for c in range(4):
        w_copy(0, c).start()
        if c > 0:
            w_copy(1, c - 1, Q1).start()
        xc_copy(c).start()
    for cp in small_copies():
        cp.start()

    r = lax.broadcasted_iota(i32, (L2, L2), 0)
    c_ = lax.broadcasted_iota(i32, (L2, L2), 1)
    head = lambda i: jnp.where(i < 2 * M, i // M, (i - 2 * M) // SEG)
    ok = (r < 2 * M) | (c_ < 2 * M) | (c_ <= r)
    const = lambda v: jnp.full((L2, L2), v, f32)
    fill_ref[...] = jnp.where(head(r) == head(c_),
                              jnp.where(ok, const(0.0), const(-1e9 / scale)), const(-jnp.inf))

    def tables(t, carry):
        rr = lax.broadcasted_iota(i32, (32, C), 0) + 32 * t
        nn = lax.broadcasted_iota(i32, (32, C), 1)
        kk = 8 * (rr >> 4) + (rr & 7)
        mm = (2 * kk + 1) * (4 * nn + 1) + 4 * C * ((rr >> 3) & 1) * (1 + 2 * (kk & 1))
        fm = jnp.cos((mm & (16 * C - 1)).astype(f32) * (math.pi / (8 * C)))
        f_p[pl.ds(pl.multiple_of(16 * t, 16), 16), :] = pltpu.bitcast(fm.astype(bf16), u32)
        rr = lax.broadcasted_iota(i32, (16, C), 0) + 16 * t
        kk = lax.broadcasted_iota(i32, (16, C), 1)
        mm = (2 * kk + 1) * (2 * (rr & (C // 2 - 1)) + 1) + C * (7 - 6 * ((kk + (rr >> 6)) & 1))
        gm = jnp.cos((mm & (8 * C - 1)).astype(f32) * (math.pi / (4 * C))) * (2 ** -0.5 / C)
        g_p[pl.ds(pl.multiple_of(8 * t, 8), 8), :] = pltpu.bitcast(gm.astype(bf16), u32)
        uh[pl.ds(4 * t, 4)] = jnp.zeros((4, 2 * C, 128), f32)
        return carry
    lax.fori_loop(0, 8, tables, 0)
    for sl in range(2):
        k_buf[sl, 0:KPAD, :] = jnp.zeros((KPAD, 128), bf16)

    def pro_body(g, i, tasks):
        r0 = pl.multiple_of(i * 128, 128)
        x = x_buf[pl.ds(r0, 128), :]
        for p in range(8):
            ys = []
            for t in range(2):
                y = jnp.dot(x, wt(g // 2, 16 * (g % 2) + 2 * p + t),
                            preferred_element_type=f32)
                ys.append(y)
                for fn in tasks.get(2 * p + t, ()):
                    fn(y)
            pp = 8 * (g % 2) + p
            ring[pp // 2][pl.ds(pl.multiple_of(QOFF + r0, 64), 128),
                          ring_cols(g // 2, pp)] = jnp.concatenate(ys, axis=1).astype(bf16)

    def add_relayout(tasks, g, c, r, q=256):
        for u in range(15):
            def fn(y, u=u):
                stage[g % 3][D + zero[0]] = y[r:r + 16].astype(bf16)
                relayout(g, c, (q // 2 * u) // 15, (q // 2 * (u + 1)) // 15, q)
            tasks.setdefault(u, []).append(fn)

    def add_wo(tasks, part):
        for u in range(15):
            def fn(y, u=u):
                wo_st[256 + zero[0], :, 0:128] = y[96:112].astype(bf16)
                wo_pack(part, (WOP * u) // 15, (WOP * (u + 1)) // 15)
            tasks.setdefault(u, []).append(fn)

    def add_s01(tasks, j, with_u=True):
        for k in range(8):
            def fn(y, k=k):
                coef[NB + zero[0], 0:8, :] = y[48:56]
                s0_kv(0, 0, 0, j, k)
            tasks.setdefault(k, []).append(fn)
        tasks.setdefault(3, []).append(lambda y: s1_h(0, j))
        if with_u:
            tasks.setdefault(11, []).append(lambda y: s1_u(0, 0, j))

    def period(g, body, n=4):
        if cfg['nopro']:
            return
        with jax.named_scope('pro%d' % g):
            lax.fori_loop(0, n, lambda i, c: (body(i), c)[1], 0)

    def p0(c):
        @pl.when(c > 0)
        def _():
            w_copy(1, c - 1, Q1).wait()
        w_copy(0, c).wait()
        relayout(0, c)
        xc_copy(c).wait()
        xp[...] = pltpu.bitcast(
            x_buf[0:PRE, pl.ds(pl.multiple_of(c * 256, 256), 256)], u32)
        tasks = {}
        add_relayout(tasks, 1, (c + 3) & 3, 0, Q1)
        k0 = pl.multiple_of(c * 128, 128)
        for p in range(8):
            ys = []
            for t in range(2):
                hh = 2 * p + t
                w = _bf(wp[0][pl.ds(k0 + hh * HS, 128), :])
                y = (jnp.dot(_bf(xp[...]), w, preferred_element_type=f32)
                     + uh[2 * hh:2 * hh + 2].reshape(PRE, 128))
                uh[2 * hh:2 * hh + 2] = y.reshape(2, 2 * C, 128)
                ys.append(y)
                for fn in tasks.get(hh, ()):
                    fn(y[256 * t:])
            ring[p // 2][QOFF:QOFF + PRE, ring_cols(0, p)] = (
                jnp.concatenate(ys, axis=1).astype(bf16))

        @pl.when(c == 0)
        def _():
            w_copy(1, 3, Q1, D - 3 * Q1).start()
            for i in range(4):
                w_copy(2, i).start()
    period(0, p0)
    w_copy(1, 3, Q1, D - 3 * Q1).wait()
    relayout(1, 3, 0, (D - 3 * Q1) // 2, Q1)
    for cp in small_copies():
        cp.wait()
    w_copy(3, 0).start()
    w_copy(3, 1).start()
    for cp in kvh_copies(0, 0):
        cp.start()
    w_copy(4, 0).start()
    w_copy(4, 1).start()
    for c in range(2, 4):
        w_copy(3, c).start()
        w_copy(4, c).start()
    for cp in kvh_copies(0, 1):
        cp.start()
    skt = skt_buf[...].astype(f32)
    ddv = dd_buf[...].astype(f32)
    for b in range(NB):
        coef[b, 0:KS, :] = skt[:, b * 128:(b + 1) * 128]
        coef[b, KS:KS + 1, :] = ddv[b:b + 1, :]

    def p1(i):
        w_copy(2, i).wait()
        tasks = {}
        add_relayout(tasks, 2, i, 0)
        pro_body(1, i, tasks)
    period(1, p1)
    w_copy(5, 0).start()
    for c in range(2):
        w_copy(5, c + 1).start()
        wo_copy(c).start()
    w_copy(5, 3).start()
    for cp in kvh_copies(0, 0):
        cp.wait()

    def p2(i2):
        for i in (2 * i2, 2 * i2 + 1):
            w_copy(3, i).wait()
            w_copy(4, i).wait()
        for i in (2 * i2, 2 * i2 + 1):
            tasks = {}
            add_relayout(tasks, 3, i, 0)
            add_relayout(tasks, 4, i, 96)
            add_s01(tasks, i)
            pro_body(2, i, tasks)
    period(2, p2, 2)
    for cp in kvh_copies(0, 1):
        cp.wait()

    def p3(i):
        @pl.when(i > 0)
        def _():
            wo_copy(i - 1).wait()
        w_copy(5, i).wait()
        tasks = {}
        add_relayout(tasks, 5, i, 0)
        add_wo(tasks, jnp.where(i == 0, 2, i - 1))
        add_s01(tasks, 4 + i, False)
        pro_body(3, i, tasks)

        @pl.when(i == 0)
        def _():
            wo_copy(2).start()
            wo_copy(3, 256 - 3 * WOP).start()
            x_copy(0).start()
            for cp in kvh_copies(1, 0) + kvh_copies(1, 1):
                cp.start()
            x_copy(1).start()
    period(3, p3)
    wo_copy(3, 256 - 3 * WOP).wait()
    wo_pack(3, 0, 256 - 3 * WOP)
    x_copy(0).wait()

    def step(cb, j, mem, u4, after_pre):
        par = u4 % 2
        s = cb * 8 + j
        x0 = pl.multiple_of(PRE + XR * s, 8)
        wpos = pl.multiple_of(lax.rem(s, RING // XR) * XR, 8)
        rpos = pl.multiple_of(lax.rem(s + QOFF // SEG, RING // SEG) * SEG, 32)
        rbase = pl.multiple_of((s - par) * SEG, 64)
        m0 = 0 if par == 0 else 72
        x8 = 8 + SEG * par

        sl1 = (cb + 1) & 1
        b1 = jnp.minimum(cb + 1, NB - 1)
        slot1 = cb + 1
        b3 = jnp.maximum(cb - 1, 0)
        slot3 = jnp.where(cb == 0, NB, cb - 1)
        s2 = s2_parts(cb & 1, j)
        nu = [0]

        def unit(pace):
            u = nu[0]
            nu[0] += 1
            if 0 <= u - cfg['s0_at'][u4] < 8:
                coef[NB + zero[0], 0:8, :] = pace
                s0_kv(sl1, b1, slot1, j, u - cfg['s0_at'][u4])
            if 0 <= u - cfg['s2_at'][u4] < 2 * NC:
                s2(u - cfg['s2_at'][u4], pace)

        def proj_q(p, lq):
            ys = []
            for t in range(2):
                ys.append(jnp.dot(lq, wt(2, 2 * p + t), preferred_element_type=f32))
                unit(ys[-1][:M])
            r0, r1 = (0, 48) if par == 0 else (48, 80)
            q_sc[p][r0:r1, :] = jnp.concatenate(ys, axis=1).astype(bf16)

        def proj_kv(p, m, lhs):
            ys = [jnp.dot(lhs, wt(m, 2 * p + t), preferred_element_type=f32)
                  for t in range(2)]
            ring[p // 2][pl.ds(wpos, XR), ring_cols(m, p)] = jnp.concatenate(
                [y[M:] for y in ys], axis=1).astype(bf16)
            unit(ys[0][:M])
            m_sc[2 * p + m] = jnp.concatenate([y[:M] for y in ys], axis=1).astype(bf16)

        def gather(m, p):
            xx = ring[p // 2][pl.ds(rpos, SEG), ring_cols(m, p)]
            mm = jnp.concatenate([m_sc[2 * p + m, :, :DH], m_sc[2 * p + m, :, DH:]], axis=0)
            return jnp.concatenate([mm, xx[:, :DH], xx[:, DH:]], axis=0)

        def qk(p):
            b = q_sc[p]
            q2 = jnp.concatenate([b[m0:m0 + M, :DH], b[m0:m0 + M, DH:],
                                  b[x8:x8 + SEG, :DH], b[x8:x8 + SEG, DH:]], axis=0)
            sc = lax.dot_general(q2, gather(0, p), (((1,), (1,)), ((), ())),
                                 preferred_element_type=f32)
            fill = fill_ref[...]
            sc = jnp.where(fill == 0.0, sc, fill)
            mx = jnp.max(sc, axis=1, keepdims=True)
            e = jnp.exp((sc - mx) * scale)
            l = jnp.sum(e, axis=1, keepdims=True)
            rc = pl.reciprocal(l, approx=True)
            rc = rc * (2.0 - l * rc)
            p_sc[p] = pltpu.bitcast((e * rc).astype(bf16), u32)

        def pv(p):
            o = jnp.dot(_bf(p_sc[p]), gather(1, p), preferred_element_type=f32)
            o_sc[p][m0:m0 + M, :] = jnp.concatenate([o[0:M], o[M:2 * M]], axis=1).astype(bf16)
            o_sc[p][x8:x8 + SEG, :] = jnp.concatenate(
                [o[2 * M:2 * M + SEG], o[2 * M + SEG:]], axis=1).astype(bf16)

        accs = [None] * 8
        odots = [(k, n) for k in range(0, H, OCH) for n in range(8)]
        lcache = {}

        def oproj(cnt):
            r0, r1 = (0, 32) if par == 0 else (32, 80)
            for _ in range(min(cnt, len(odots))):
                k, n = odots.pop(0)
                ke = k + OCH
                if k not in lcache:
                    lcache[k] = jnp.concatenate(
                        [o_sc[p][r0:r1, :] for p in range(k // 2, ke // 2)], axis=1)
                y = jnp.dot(lcache[k], _bf(wo_p[n, k * 64:ke * 64, :]),
                            preferred_element_type=f32)
                accs[n] = y if accs[n] is None else y + accs[n]
                unit(accs[n][:M])

        def pre_u():
            if u4 == 0:
                n1 = s + 4
                for k in range(4):
                    s1_u((n1 >> 3) & 1, n1 >> 3, (n1 & 7) + k)
        pre = dict(u=pre_u,
                   h=lambda: s1_h(sl1, j),
                   y=lambda: s3(sl1, b3, slot3, j))
        for key in cfg['border'][u4]:
            pre[key]()
        if after_pre is not None:
            after_pre()

        if par == 0:
            lq = jnp.concatenate([mem, x_buf[pl.ds(rbase, 40), :]], axis=0)
        else:
            lq = jnp.concatenate([x_buf[pl.ds(rbase + 40, 24), :], mem], axis=0)
        for p in range(NPAIR):
            proj_q(p, lq)

        lhs = jnp.concatenate([mem, x_buf[pl.ds(x0, XR), :]], axis=0)
        a0, a1 = cfg['att'][u4]
        att = {4 + a0: ([], [0, 1, 2, 3]), 18 + a1: ([12, 13, 14, 15], []),
               **{t + a0: ([t - 6, t - 5], [t - 2, t - 1]) for t in range(6, 18, 2)}}
        for t in range(max(att) + 1):
            if t < NPAIR:
                for m in range(2):
                    proj_kv(t, m, lhs)
            else:
                oproj(cfg['op_per'][u4])
            pvs, qks = att.get(t, ((), ()))
            for p in pvs:
                pv(p)
            for p in qks:
                qk(p)
        oproj(len(odots))
        out = jnp.concatenate(accs, axis=1).astype(bf16)
        if par == 0:
            outb[pl.ds(rbase, 24), :] = out[M:]
            return out[:M]
        outb[pl.ds(rbase + 24, 40), :] = out[:40]
        return out[40:]

    def four_steps(it, carry):
        cb, jj = it >> 1, it & 1

        @pl.when(cb + 1 < NB)
        def _():
            for cp in kvh_copies(cb + 1, jj):
                cp.wait()

        @pl.when(cb >= 1)
        def _():
            q_copy(cb - 1, jj).wait()

        @pl.when(it == 1)
        def _():
            x_copy(1).wait()

        @pl.when(it >= 1)
        def _():
            outa_copy(jnp.maximum(((it - 1) >> 1) - 1, 0), (it - 1) & 1).wait()
            outb_copy(2 * it - 1).start()

        mem = mem_ref[...]
        for u in range(4):
            after = (lambda: outa_copy(jnp.maximum(cb - 1, 0), jj).start()) if u == 3 else None
            mem = step(cb, jj * 4 + u, mem, u, after)
            if u == 1:
                outb_copy(2 * it).start()
        mem_ref[...] = mem

        @pl.when(it + 1 < 2 * NB)
        def _():
            q_copy((it + 1) >> 1, (it + 1) & 1).start()

        @pl.when(cb + 2 < NB)
        def _():
            for cp in kvh_copies(cb + 2, jj):
                cp.start()
        return carry
    q_copy(0, 0).start()
    with jax.named_scope('main'):
        lax.fori_loop(0, 2 * NB, four_steps, 0)

    outb_copy(NSEG // 2 - 1).start()
    q_copy(NB - 1, 0).wait()
    q_copy(NB - 1, 1).wait()
    with jax.named_scope('epi'):
        for j in range(8):
            s3((NB - 1) % 2, NB - 1, NB - 1, j)
            if j % 2 == 1:
                outa_piece(NB - 1, (j - 1) * 2 * C, 4 * C).start()

    outa_copy(NB - 2, 1).wait()
    for pr in range(NSEG // 2):
        outb_copy(pr).wait()
    for j in range(4):
        outa_piece(NB - 1, j * 4 * C, 4 * C).wait()


@jax.jit
def pallas_concat_heads__ssm_conv_h3__memory_aug_recurrent_mem_tr__prompt_kernel(
    A_q, A_k, A_v, A_shift_k, A_ssm_k, A_ssm_D, B_x, B_mem0, B_Wq, B_Wk, B_Wv, B_Wo,
    B_seg_len,
):
    del B_seg_len
    assert A_q.shape == (1, S, D) and B_x.shape == (1, S, D)
    assert B_Wq.shape == (D, H, DH) and B_mem0.shape == (1, M, D)
    vm = pltpu.VMEM
    dma = pltpu.SemaphoreType.DMA
    scratch = [
        vm((D + 4, 16, DH), bf16), vm((D + 4, 16, DH), bf16),
        vm((D + 4, 16, DH), bf16),
        vm((256 + 1, 16, D), bf16),
        vm((8, H * DH // 2, 128), u32),
        vm((S, D), bf16),
        vm((M, D), bf16),
        vm((S, D), bf16),
        vm((NB + 1, 32, 128), f32),
        vm((2, S + 64, 128), bf16),
        vm((2, S, 128), bf16), vm((2, S, 128), bf16),
        vm((2, 128, S), bf16),
        vm((NB + 1, S, 128), bf16),
        vm((4 * NC + 1, 2 * C, 128), f32),
        vm((2, 8, 8, 32, 128), u32),
        vm((8, 32 + KPAD, 128), f32),
        vm((C, C), u32), vm((C // 2, C), u32),
        vm((PRE // 2, 256), u32),
        dma((40,)),
        pltpu.SMEM((1,), i32),
    ]
    scratch += [vm((16 * HS, 128), u32)] * 6
    scratch += [vm((RING, 8 * DH), bf16)] * 8
    scratch += [vm((L2, 2 * DH), bf16)] * (2 * NPAIR)
    scratch += [vm((NPAIR, L2 // 2, L2), u32)]
    scratch += [vm((2 * NPAIR, M, 2 * DH), bf16)]
    scratch += [vm((L2, L2), f32), vm((KS, D), bf16), vm((NB, 128), bf16)]

    out = pl.pallas_call(
        _kernel,
        out_shape=jax.ShapeDtypeStruct((S, 2 * D), bf16),
        in_specs=[pl.BlockSpec(memory_space=pl.ANY)] * 12,
        out_specs=pl.BlockSpec(memory_space=pl.ANY),
        scratch_shapes=scratch,
        compiler_params=pltpu.CompilerParams(vmem_limit_bytes=120 * 1024 * 1024,
                                             disable_bounds_checks=True,
                                             disable_semaphore_checks=True),
        name="ssm_memtr",
    )(A_q.reshape(S, D), A_k.reshape(S, D), A_v.reshape(S, D), A_shift_k.T, A_ssm_k,
      A_ssm_D.reshape(NB, 128), B_x.reshape(S, D), B_mem0.reshape(M, D),
      B_Wq, B_Wk, B_Wv, B_Wo.reshape(H * DH // 16, 16, D))
    return out.reshape(1, S, 2 * D)
```
